```python
import jax
import jax.numpy as jnp

def _softmax(x, axis=-1):
    return jax.nn.softmax(x, axis=axis)
def _gelu(x):
    return jax.nn.gelu(x, approximate=True)
def _silu(x):
    return jax.nn.silu(x)
def _sigmoid(x):
    return jax.nn.sigmoid(x)
def _layernorm(x, axis=-1, eps=1e-5):
    m = jnp.mean(x, axis=axis, keepdims=True)
    v = jnp.var(x, axis=axis, keepdims=True)
    return (x - m) / jnp.sqrt(v + eps)
def _scatter_add(tgt, idx, src, axis=0):
    return tgt.at[idx].add(src)
def _segment_sum(src, seg, n):
    return jax.ops.segment_sum(src, seg, n)
class _Rng:
    def __init__(self, key):
        self._k = key
    def _next(self):
        self._k, sub = jax.random.split(self._k)
        return sub
    def normal(self, shape):
        return jax.random.normal(self._next(), shape, dtype=jnp.bfloat16)
    def randint(self, lo, hi, shape):
        return jax.random.randint(self._next(), shape, lo, hi, dtype=jnp.int32)
    def uniform(self, shape, lo=0.0, hi=1.0):
        return jax.random.uniform(self._next(), shape, jnp.bfloat16, lo, hi)
    def permutation(self, n):
        return jax.random.permutation(self._next(), n)


kernel_name = 'recurrent_scan__mha_block_cached__moe_arch_mod__prompt'

def setup_inputs():
    _rng = _Rng(jax.random.key(int.from_bytes(__import__("os").urandom(4), "little")))
    _w = (lambda a: (lambda t: t.astype(jnp.bfloat16) if jnp.issubdtype(t.dtype, jnp.floating) else t)(jnp.asarray(a)))
    def _A_setup():
        B, Sq, D = 1, 2048, 640
        H, Sk, Dh = 32, 2048, 128
        return {
            "x": _w((lambda *s: _rng.normal(s) * 0.05)(B, Sq, D)),
            "k_cache": _w((lambda *s: _rng.normal(s) * 0.05)(B, H, Sk, Dh)),
            "v_cache": _w((lambda *s: _rng.normal(s) * 0.05)(B, H, Sk, Dh)),
            "wq": _w((lambda *s: _rng.normal(s) * 0.05)(D, H * Dh) * (D ** -0.5)),
            "wo": _w((lambda *s: _rng.normal(s) * 0.05)(H * Dh, D) * ((H * Dh) ** -0.5)),
        }
    _A_in = _A_setup()

    def _B_setup():
        B, S, D, F, C = 1, 2048, 640, 1728, 8
        return {
            "x": _w((lambda *s: _rng.normal(s) * 0.05)(B, S, D)),
            "w_r": _w((lambda *s: _rng.normal(s) * 0.05)(D)),
            "w_gate": _w((lambda *s: _rng.normal(s) * 0.05)(D, F)),
            "w_up": _w((lambda *s: _rng.normal(s) * 0.05)(D, F)),
            "w_down": _w((lambda *s: _rng.normal(s) * 0.05)(F, D)),
        }
    _B_in = _B_setup()

    return {
        "A_x": _A_in["x"],
        "A_k_cache": _A_in["k_cache"],
        "A_v_cache": _A_in["v_cache"],
        "A_wq": _A_in["wq"],
        "A_wo": _A_in["wo"],
        "B_x": _B_in["x"],
        "B_w_r": _B_in["w_r"],
        "B_w_gate": _B_in["w_gate"],
        "B_w_up": _B_in["w_up"],
        "B_w_down": _B_in["w_down"],
    }

def reference(A_x, A_k_cache, A_v_cache, A_wq, A_wo, B_x, B_w_r, B_w_gate, B_w_up, B_w_down):
    def _A_ref(x, k_cache, v_cache, wq, wo):
        B, Sq, D = x.shape
        H, Dh = 32, 128
        q = (lambda x, *d: x.transpose(*d))((x @ wq).reshape(B, Sq, H, Dh), 0, 2, 1, 3)
        scores = jnp.einsum("bhqd,bhkd->bhqk", q, k_cache) * (Dh ** -0.5)
        p = _softmax(scores, axis=-1)
        o = jnp.einsum("bhqk,bhkd->bhqd", p, v_cache)
        return (lambda x, *d: x.transpose(*d))(o, 0, 2, 1, 3).reshape(B, Sq, H * Dh) @ wo

    def _B_ref(x, w_r, w_gate, w_up, w_down):
        B, S, D = x.shape
        C = 8
        r = x @ w_r
        idx = jnp.argsort(-r, axis=-1)[:, :C]
        idx_e = jnp.repeat(idx.reshape(B, C, 1), D, axis=2)
        x_sel = jnp.take_along_axis(x, idx_e, axis=1)
        g = _silu(x_sel @ w_gate)
        u = x_sel @ w_up
        y = (g * u) @ w_down
        r_sel = _sigmoid(jnp.take_along_axis(r, idx, axis=1))
        y = y * r_sel.reshape(B, C, 1)
        b_off = (jnp.arange(B) * S).reshape(B, 1)
        flat_idx = (idx + b_off).reshape(B * C)
        zero = (x * 0.0).reshape(B * S, D)
        upd = _scatter_add(zero, flat_idx, y.reshape(B * C, D), axis=0)
        return x + upd.reshape(B, S, D)

    x = A_x
    xn = _layernorm(x, axis=-1)
    s = _A_ref(xn, A_k_cache, A_v_cache, A_wq, A_wo)
    g = _silu(_B_ref(xn, B_w_r, B_w_gate, B_w_up, B_w_down))
    return x + s * g
```

```python
import functools
import numpy as np
import jax
import jax.numpy as jnp
from jax import lax
import jax.experimental.pallas as pl
import jax.experimental.pallas.tpu as pltpu

S, D, H, DH, SK, F, C = 2048, 640, 32, 128, 2048, 1728, 8
LOG2E = 1.4426950408889634
EPS = float(np.asarray(1e-5, dtype=jnp.bfloat16))
f32, bf16, i32 = jnp.float32, jnp.bfloat16, jnp.int32
NT = (((1,), (1,)), ((), ()))


def rb(x):
    return x.astype(bf16).astype(f32)


def sigmoid(x):
    return 1.0 / (1.0 + jnp.exp2(x * (-LOG2E)))


def attention_body(t, w_buf, s_bufs, k_buf, v_buf, P):
    BQ, NU, KC, DL = P["BQ"], P["NU"], P["KC"], P["DL"]
    LA, LS, PD, LC, XD, FD, QA = (P[k] for k in "LA LS PD LC XD FD QA".split())
    NB = S // BQ; R = BQ // 16; NC = SK // KC; W = KC // 128; L = NC + DL
    z0 = pl.multiple_of(lax.shift_right_logical(t * t, 24) * 32, 32)
    z1 = pl.multiple_of(lax.shift_right_logical(t * t + t, 25) * 32, 32)

    def s_loc(g, w, r):
        return (g // L) % 2, (((g % L) * R + r) * W + w) * 16
    def ld_s(g, w, r):
        par, o = s_loc(g, w, r)
        return s_bufs[par][pl.ds(z1 + o, 16), :]
    def st_s(g, w, r, v):
        par, o = s_loc(g, w, r)
        s_bufs[par][pl.ds(z0 + o, 16), :] = v
    def st_tok(g, v):
        s_bufs[s_loc(g, 0, 0)[0]][pl.ds(z0 + L * R * W * 16, 8), :] = v
    MX = lambda a: (a % 3) * BQ
    LP = 3 * BQ
    OA = 4 * BQ
    def ld(off, r): return w_buf[pl.ds(z1 + (off + 16 * r), 16), :]
    def st(off, r, v): w_buf[pl.ds(z0 + (off + 16 * r), 16), :] = v
    units = []
    for u in range(NU):
        if NU >= NB: units.append((t * (NU // NB) + u // NB, (u % NB) * (BQ // 2)))
        else:
            per = NB // NU
            units.append((t // per, ((t % per) * NU + u) * (BQ // 2)))
    qrow = [pl.multiple_of(P["QB"] + h * (S // 2) + r0, 32) for h, r0 in units]
    dots = []
    for g in range(NU * NC + L):
        if g < NU * NC: dots.append(("qk", g))
        if g - L >= 0: dots.append(("pv", g - L))
    ev = []; val = {}
    def add(slot, prio, fn): ev.append((slot, prio, len(ev), fn))
    def res(i):
        if ("res", i) not in val:
            kind, g = dots[i]; a, c = divmod(g, NC); h = units[a][0]
            if kind == "qk":
                q = pltpu.bitcast(jnp.concatenate([val.pop(("q", i, r)) for r in range(R)], axis=0), bf16)
                val["res", i] = lax.dot_general(q, k_buf[h, pl.ds(c * KC, KC), :], NT, preferred_element_type=f32)
            else:
                p = jnp.concatenate([val.pop(("p", i, r)) for r in range(R)], axis=0).astype(bf16)
                val["res", i] = jnp.dot(p, v_buf[h, pl.ds(c * KC, KC), :], preferred_element_type=f32)
        return val["res", i]
    for i, (kind, g) in enumerate(dots):
        a, c = divmod(g, NC)
        la = P["LAL"] if i == len(dots) - 1 else LA
        for r in range(R):
            j = i * R + r
            if kind == "qk":
                def l_q(i=i, a=a, r=r):
                    val["q", i, r] = w_buf[pl.ds(z1 + qrow[a] + 8 * r, 8), :]
                add(min(j - QA, i * R + PD - 1), 1, l_q)
                if c > 0:
                    def l_acc(a=a, r=r): val["mx", a, r] = ld(MX(a), r)
                    add(j + PD - LC, 1, l_acc)
                def s_res(i=i, g=g, a=a, c=c, r=r):
                    s = res(i)[16 * r:16 * r + 16]
                    tiles = [s[:, w * 128:(w + 1) * 128] for w in range(W)]
                    for w in range(W): st_s(g, w, r, tiles[w])
                    val["tok"] = tiles[W - 1][:8]
                    mx = functools.reduce(jnp.maximum, tiles)
                    if c > 0: mx = jnp.maximum(mx, val.pop(("mx", a, r)))
                    if c == NC - 1:
                        val["m", a, r] = jnp.broadcast_to(jnp.max(mx, axis=-1, keepdims=True), (16, 128))
                    else: st(MX(a), r, mx)
                add(j + PD, 0, s_res)
                if c == NC - 1:
                    def s_m(a=a, r=r): st(MX(a), r, val.pop(("m", a, r)))
                    add(j + PD + XD, 0, s_m)
            else:
                def l_lhs(i=i, g=g, a=a, c=c, r=r):
                    m = ld(MX(a), r)
                    if "tok" in val: st_tok(g, val.pop("tok"))
                    ps = [jnp.exp2(ld_s(g, w, r) - m) for w in range(W)]
                    lp = functools.reduce(lax.add, ps)
                    if c > 0: lp = lp + ld(LP, r)
                    val["lp", i, r] = lp
                    val["p", i, r] = jnp.concatenate(ps, axis=1)
                add(min(j - la, i * R + PD - 1), 1, l_lhs)
                if c < NC - 1:
                    def s_lp(i=i, r=r): st(LP, r, val.pop(("lp", i, r)))
                    add(j - la + LS, 0, s_lp)
                if c > 0:
                    def l_acc(i=i, r=r): val["o", i, r] = ld(OA, r)
                    add(j + PD - LC, 1, l_acc)
                if c < NC - 1:
                    def s_res(i=i, c=c, r=r):
                        d = res(i)[16 * r:16 * r + 16]
                        if c > 0: d = d + val.pop(("o", i, r))
                        val["tok"] = d[:8]
                        st(OA, r, d)
                    add(j + PD, 0, s_res)
                else:
                    def s_res(i=i, r=r):
                        d = res(i)[16 * r:16 * r + 16] + val.pop(("o", i, r))
                        val["tok"] = d[:8]
                        val["of", i, r] = d
                    add(j + PD, 0, s_res)
                    def s_fin(i=i, a=a, r=r):
                        l = jnp.sum(val.pop(("lp", i, r)), axis=-1, keepdims=True)
                        r0 = pl.reciprocal(l, approx=True)
                        rl = r0 * (2.0 - l * r0)
                        ob = pltpu.bitcast((val.pop(("of", i, r)) * rl).astype(bf16), f32)
                        w_buf[pl.ds(z0 + qrow[a] + 8 * r, 8), :] = ob
                    add(max(j - la + LS + XD + FD, j + PD), 0, s_fin)
    ev.sort(key=lambda e: e[:3])
    for e in ev: e[3]()


def make(flags=None, **kw):
    P = dict(BQ=128, NU=16, KC=512, DL=2, LA=4, LAL=4, LS=3, PD=8, LC=2, XD=9, FD=2, QA=2, BX=256, G=4, BO=256, HA=8, SKIP="")
    P.update(kw)
    BQ, NU, KC, BX, G, BO, HA = (P[k] for k in "BQ NU KC BX G BO HA".split())
    P["QB"] = QB = 5 * BQ
    NB = S // BQ; NX = S // BX; NG = H // G; NO = S // BO
    L = SK // KC + P["DL"]

    def kernel(x_hbm, k_hbm, v_hbm, wq_hbm, wo_hbm, wr_hbm, wg_hbm, wu_hbm, wd_hbm, out_hbm,
               x_buf, xn_buf, w_buf, s_buf0, s_buf1, k_buf, v_buf, wq_buf, wo_buf, wr_buf, wg_buf, wu_buf, wd_buf, out_buf,
               x_sem, wq_sem, kv_sem, misc_sem, out_sem):
        xr = [(0, BX), (BX, 2 * BX), (3 * BX, S - 3 * BX)]
        x_cp = lambda i: pltpu.make_async_copy(x_hbm.at[pl.ds(*xr[i])], x_buf.at[pl.ds(*xr[i])], x_sem.at[i])
        wq_cp = lambda j: pltpu.make_async_copy(wq_hbm.at[:, pl.ds(j * G * DH, G * DH)], wq_buf.at[j], wq_sem.at[j])
        hr = [(0, HA), (HA, H - HA)]
        k_cp = lambda j: pltpu.make_async_copy(k_hbm.at[pl.ds(*hr[j])], k_buf.at[pl.ds(*hr[j])], kv_sem.at[2 * j])
        v_cp = lambda j: pltpu.make_async_copy(v_hbm.at[pl.ds(*hr[j])], v_buf.at[pl.ds(*hr[j])], kv_sem.at[2 * j + 1])
        wr_cp = lambda: pltpu.make_async_copy(wr_hbm, wr_buf, misc_sem.at[0])
        wg_cp = lambda: pltpu.make_async_copy(wg_hbm, wg_buf, misc_sem.at[1])
        wu_cp = lambda: pltpu.make_async_copy(wu_hbm, wu_buf, misc_sem.at[2])
        wd_cp = lambda: pltpu.make_async_copy(wd_hbm, wd_buf, misc_sem.at[3])
        wo_cp = lambda: pltpu.make_async_copy(wo_hbm, wo_buf, misc_sem.at[4])

        x_cp(0).start(); wr_cp().start(); wq_cp(0).start(); x_cp(1).start()

        def qproj(j, i):
            xn = xn_buf[pl.ds(i * BX, BX), :]
            q = jnp.dot(xn, wq_buf[j], preferred_element_type=f32)
            q = (q * (DH ** -0.5 * LOG2E)).astype(bf16)
            for g in range(G):
                r0 = pl.multiple_of(QB + (j * G + g) * (S // 2) + i * (BX // 2), 32)
                w_buf[pl.ds(r0, BX // 2), :] = pltpu.bitcast(q[:, g * DH:(g + 1) * DH], f32)

        lane = lax.broadcasted_iota(i32, (8, 128), 1)
        sub = lax.broadcasted_iota(i32, (8, 128), 0)

        def layernorm(i, rd):
            x = x_buf[pl.ds(i * BX, BX), :].astype(f32)
            m = jnp.sum(x, axis=-1, keepdims=True) * (1.0 / D)
            xc = x - m
            var = jnp.sum(xc * xc, axis=-1, keepdims=True) * (1.0 / D)
            sd = rb(jnp.sqrt(rb(rb(var) + EPS)))
            xn = (rb(x - rb(m)) * (1.0 / sd)).astype(bf16)
            xn_buf[pl.ds(i * BX, BX), :] = xn
            r = jnp.sum(xn.astype(f32) * wr, axis=-1, keepdims=True)
            r = jnp.broadcast_to(r, (BX, 128))
            for t in range(BX // 8):
                pos = i * (BX // 8) + t
                rd[pos // 128] = jnp.where(lane == pos % 128, r[t * 8:(t + 1) * 8], rd[pos // 128])

        x_cp(0).wait(); wr_cp().wait()
        x_cp(2).start()
        wr = wr_buf[...].astype(f32).reshape(1, D)
        rd = [jnp.zeros((8, 128), f32) for _ in range(S // 1024)]
        layernorm(0, rd)
        wq_cp(0).wait(); x_cp(1).wait()
        wq_cp(1).start()
        for i in range(NX):
            if i == 2:
                x_cp(2).wait()
                for j in range(2, NG):
                    wq_cp(j).start()
            if i + 1 < NX:
                layernorm(i + 1, rd)
            qproj(0, i)
        wg_cp().start(); wu_cp().start(); wd_cp().start()
        k_cp(0).start(); v_cp(0).start()

        def p1_body(j, _):
            wq_cp(j).wait()
            for i in range(NX):
                qproj(j, i)
        lax.fori_loop(1, NG - 1, p1_body, None)

        wq_cp(NG - 1).wait(); wg_cp().wait(); wu_cp().wait(); wd_cp().wait()
        k_cp(0).wait(); v_cp(0).wait()
        k_cp(1).start(); v_cp(1).start(); wo_cp().start()
        keys = []
        for t in range(len(rd)):
            r = rb(rd[t])
            r = jnp.where(r == 0.0, 0.0, r)
            b = lax.shift_right_logical(pltpu.bitcast(r, i32), 16)
            k16 = jnp.where(b >= 0x8000, 0xFFFF - b, b + 0x8000)
            k16 = jnp.where(r != r, 0, k16)
            tok = t * 1024 + lane * 8 + sub
            keys.append(pltpu.bitcast(0x20000000 + k16 * 2048 + (2047 - tok), f32))
        idxs = []
        ktop = jnp.zeros((8, 128), i32)
        for c in range(C):
            mx = functools.reduce(jnp.maximum, keys)
            mx = jnp.max(jnp.max(mx, axis=1, keepdims=True), axis=0, keepdims=True)
            mxb = jnp.broadcast_to(mx, (8, 128))
            keys = [jnp.where(kk == mxb, 0.0, kk) for kk in keys]
            mi = pltpu.bitcast(mxb, i32)
            ktop = jnp.where(sub == c, mi, ktop)
            idxs.append(2047 - (mi[0, 0] & 2047))
        k16 = lax.shift_right_logical(ktop - 0x20000000, 11)
        b = jnp.where(k16 >= 0x8000, k16 - 0x8000, 0xFFFF - k16)
        r_sel = pltpu.bitcast(lax.shift_left(b, 16), f32)[:, :1]
        row16 = lax.broadcasted_iota(i32, (16, D), 0)
        row8 = lax.broadcasted_iota(i32, (8, D), 0)
        x_sel = jnp.zeros((8, D), f32)
        bases = [pl.multiple_of(ix & -16, 16) for ix in idxs]
        for c in range(C):
            blk = xn_buf[pl.ds(bases[c], 16), :].astype(f32)
            rowv = jnp.sum(jnp.where(row16 == idxs[c] - bases[c], blk, 0.0), axis=0, keepdims=True)
            x_sel = jnp.where(row8 == c, rowv, x_sel)
        F1, F2 = P.get("F1", 5), P.get("F2", 6)
        for i in range(F1):
            qproj(NG - 1, i)
        xs = x_sel.astype(bf16)
        a = rb(lax.dot_general(xs, wg_buf[...], NT, preferred_element_type=f32))
        u = rb(lax.dot_general(xs, wu_buf[...], NT, preferred_element_type=f32))
        hid = (rb(a * sigmoid(a)) * u).astype(bf16)
        for i in range(F1, F2):
            qproj(NG - 1, i)
        y = rb(jnp.dot(hid, wd_buf[...], preferred_element_type=f32))
        z = rb(x_sel + rb(y * rb(sigmoid(r_sel))))
        for i in range(F2, NX):
            qproj(NG - 1, i)
        for c in range(C):
            blk = xn_buf[pl.ds(bases[c], 16), :].astype(f32)
            xn_buf[pl.ds(bases[c], 16), :] = jnp.where(row16 == idxs[c] - bases[c], z[c:c + 1, :], blk).astype(bf16)

        TA = HA * NB // NU
        def att_body(t, _):
            @pl.when(t == TA)
            def _():
                k_cp(1).wait(); v_cp(1).wait(); wo_cp().wait()
            if "a" not in P["SKIP"]:
                attention_body(t, w_buf, (s_buf0, s_buf1), k_buf, v_buf, P)
        lax.fori_loop(0, H * NB // NU, att_body, None)

        out_cp = lambda i: pltpu.make_async_copy(out_buf.at[pl.ds(i * BO, BO)], out_hbm.at[pl.ds(i * BO, BO)], out_sem.at[i])
        def p3_body(i, _):
            r0 = pl.multiple_of(i * BO, BO)
            o = jnp.concatenate([pltpu.bitcast(w_buf[pl.ds(pl.multiple_of(QB + h * (S // 2) + i * (BO // 2), 32), BO // 2), :], bf16) for h in range(H)], axis=-1)
            s = jnp.dot(o, wo_buf[...], preferred_element_type=f32)
            xn = xn_buf[pl.ds(r0, BO), :].astype(f32)
            out_buf[pl.ds(r0, BO), :] = (x_buf[pl.ds(r0, BO), :].astype(f32) + s * (xn * sigmoid(xn))).astype(bf16)
            out_cp(i).start()
        lax.fori_loop(0, NO, p3_body, None)
        for i in range(NO):
            out_cp(i).wait()

    @jax.jit
    def fn(A_x, A_k_cache, A_v_cache, A_wq, A_wo, B_x, B_w_r, B_w_gate, B_w_up, B_w_down):
        any_spec = pl.BlockSpec(memory_space=pl.ANY)
        s_shape = pltpu.VMEM((L * BQ * (KC // 128) + 32, 128), f32)
        out = pl.pallas_call(
            kernel,
            in_specs=[any_spec] * 9,
            out_specs=any_spec,
            out_shape=jax.ShapeDtypeStruct((S, D), bf16),
            scratch_shapes=[
                pltpu.VMEM((S, D), bf16), pltpu.VMEM((S, D), bf16),
                pltpu.VMEM((QB + H * S // 2, DH), f32), s_shape, s_shape,
                pltpu.VMEM((H, SK, DH), bf16), pltpu.VMEM((H, SK, DH), bf16),
                pltpu.VMEM((NG, D, G * DH), bf16), pltpu.VMEM((H * DH, D), bf16),
                pltpu.VMEM((D,), bf16), pltpu.VMEM((F, D), bf16), pltpu.VMEM((F, D), bf16), pltpu.VMEM((F, D), bf16),
                pltpu.VMEM((S, D), bf16),
                pltpu.SemaphoreType.DMA((3,)), pltpu.SemaphoreType.DMA((NG,)), pltpu.SemaphoreType.DMA((4,)),
                pltpu.SemaphoreType.DMA((5,)), pltpu.SemaphoreType.DMA((NO,)),
            ],
            compiler_params=pltpu.CompilerParams(vmem_limit_bytes=120 * 1024 * 1024, flags=flags),
            name="fused_kernel",
        )(A_x.reshape(S, D), A_k_cache.reshape(H, SK, DH), A_v_cache.reshape(H, SK, DH), A_wq, A_wo,
          B_w_r, B_w_gate.T, B_w_up.T, B_w_down)
        return out.reshape(1, S, D)
    return fn


_impl = make(NU=16)


@jax.jit
def pallas_recurrent_scan__mha_block_cached__moe_arch_mod__prompt_kernel(
    A_x, A_k_cache, A_v_cache, A_wq, A_wo, B_x, B_w_r, B_w_gate, B_w_up, B_w_down
):
    return _impl(A_x, A_k_cache, A_v_cache, A_wq, A_wo, B_x, B_w_r, B_w_gate, B_w_up, B_w_down)
```

```python
import functools
import numpy as np
import jax
import jax.numpy as jnp
from jax import lax
import jax.experimental.pallas as pl
import jax.experimental.pallas.tpu as pltpu

S, D, H, DH, SK, F, C = 2048, 640, 32, 128, 2048, 1728, 8
LOG2E = 1.4426950408889634
EPS = float(np.asarray(1e-5, dtype=jnp.bfloat16))
f32, bf16, i32 = jnp.float32, jnp.bfloat16, jnp.int32
NT = (((1,), (1,)), ((), ()))


def rb(x):
    return x.astype(bf16).astype(f32)


def sigmoid(x):
    return 1.0 / (1.0 + jnp.exp2(x * (-LOG2E)))


def attention_body(n0, NU, g0, NGR, z0, z1, w_buf, s_bufs, k_buf, v_buf, xn_buf, P):
    BQ, KC, DL = P["BQ"], P["KC"], P["DL"]
    LA, LS, PD, LC, XD, FD, QA = (P[k] for k in "LA LS PD LC XD FD QA".split())
    NB = S // BQ; R = BQ // 16; NC = SK // KC; W = KC // 128; L = NC + DL
    def s_loc(g, w, r):
        return (g // L) % 2, (((g % L) * R + r) * W + w) * 16
    def ld_s(g, w, r):
        par, o = s_loc(g, w, r)
        return s_bufs[par][pl.ds(z1 + o, 16), :]
    def st_s(g, w, r, v):
        par, o = s_loc(g, w, r)
        s_bufs[par][pl.ds(z0 + o, 16), :] = v
    def st_tok(g, v):
        s_bufs[s_loc(g, 0, 0)[0]][pl.ds(z0 + L * R * W * 16, 8), :] = v
    MX = lambda a: (a % 3) * BQ
    LP = 3 * BQ
    OA = 4 * BQ
    def ld(off, r): return w_buf[pl.ds(z1 + (off + 16 * r), 16), :]
    def st(off, r, v): w_buf[pl.ds(z0 + (off + 16 * r), 16), :] = v
    heads = [(n0 + u) // NB if isinstance(n0, int) else lax.shift_right_logical(n0 + u, NB.bit_length() - 1) for u in range(NU)]
    qbase = P["QB"] + n0 * (BQ // 2)
    if not isinstance(n0, int): qbase = pl.multiple_of(qbase, 32)
    qrow = [qbase + u * (BQ // 2) for u in range(NU)]
    dots = []
    for g in range(NU * NC + L):
        if g < NU * NC: dots.append(("qk", g))
        if g - L >= 0: dots.append(("pv", g - L))
    ev = []; val = {}
    def add(slot, prio, fn): ev.append((slot, prio, len(ev), fn))
    def res(i):
        if ("res", i) not in val:
            kind, g = dots[i]; a, c = divmod(g, NC); h = heads[a]
            if kind == "qk":
                q = pltpu.bitcast(jnp.concatenate([val.pop(("q", i, r)) for r in range(R)], axis=0), bf16)
                val["res", i] = lax.dot_general(q, k_buf[h, pl.ds(c * KC, KC), :], NT, preferred_element_type=f32)
            else:
                p = jnp.concatenate([val.pop(("p", i, r)) for r in range(R)], axis=0).astype(bf16)
                val["res", i] = jnp.dot(p, v_buf[h, pl.ds(c * KC, KC), :], preferred_element_type=f32)
        return val["res", i]
    for i, (kind, g) in enumerate(dots):
        a, c = divmod(g, NC)
        la = P["LAL"] if i == len(dots) - 1 else LA
        for r in range(R):
            j = i * R + r
            if kind == "qk":
                def l_q(i=i, a=a, r=r):
                    val["q", i, r] = w_buf[pl.ds(z1 + qrow[a] + 8 * r, 8), :]
                add(min(j - QA, i * R + PD - 1), 1, l_q)
                if c > 0:
                    def l_acc(a=a, r=r): val["mx", a, r] = ld(MX(a), r)
                    add(j + PD - LC, 1, l_acc)
                def s_res(i=i, g=g, a=a, c=c, r=r):
                    s = res(i)[16 * r:16 * r + 16]
                    tiles = [s[:, w * 128:(w + 1) * 128] for w in range(W)]
                    for w in range(W): st_s(g, w, r, tiles[w])
                    val["tok"] = tiles[W - 1][:8]
                    mx = functools.reduce(jnp.maximum, tiles)
                    if c > 0: mx = jnp.maximum(mx, val.pop(("mx", a, r)))
                    if c == NC - 1:
                        val["m", a, r] = jnp.broadcast_to(jnp.max(mx, axis=-1, keepdims=True), (16, 128))
                    else: st(MX(a), r, mx)
                add(j + PD, 0, s_res)
                if c == NC - 1:
                    def s_m(a=a, r=r): st(MX(a), r, val.pop(("m", a, r)))
                    add(j + PD + XD, 0, s_m)
            else:
                def l_lhs(i=i, g=g, a=a, c=c, r=r):
                    m = ld(MX(a), r)
                    if "tok" in val: st_tok(g, val.pop("tok"))
                    ps = [jnp.exp2(ld_s(g, w, r) - m) for w in range(W)]
                    lp = functools.reduce(lax.add, ps)
                    if c > 0: lp = lp + ld(LP, r)
                    val["lp", i, r] = lp
                    val["p", i, r] = jnp.concatenate(ps, axis=1)
                add(min(j - la, i * R + PD - 1), 1, l_lhs)
                if c < NC - 1:
                    def s_lp(i=i, r=r): st(LP, r, val.pop(("lp", i, r)))
                    add(j - la + LS, 0, s_lp)
                if c > 0:
                    def l_acc(i=i, r=r): val["o", i, r] = ld(OA, r)
                    add(j + PD - LC, 1, l_acc)
                if c < NC - 1:
                    def s_res(i=i, c=c, r=r):
                        d = res(i)[16 * r:16 * r + 16]
                        if c > 0: d = d + val.pop(("o", i, r))
                        val["tok"] = d[:8]
                        st(OA, r, d)
                    add(j + PD, 0, s_res)
                else:
                    def s_res(i=i, r=r):
                        d = res(i)[16 * r:16 * r + 16] + val.pop(("o", i, r))
                        val["tok"] = d[:8]
                        val["of", i, r] = d
                    add(j + PD, 0, s_res)
                    def s_fin(i=i, a=a, r=r):
                        l = jnp.sum(val.pop(("lp", i, r)), axis=-1, keepdims=True)
                        r0 = pl.reciprocal(l, approx=True)
                        rl = r0 * (2.0 - l * r0)
                        ob = pltpu.bitcast((val.pop(("of", i, r)) * rl).astype(bf16), f32)
                        w_buf[pl.ds(z0 + qrow[a] + 8 * r, 8), :] = ob
                    add(max(j - la + LS + XD + FD, j + PD), 0, s_fin)
    items = [(rg, w) for rg in range(NGR) for w in range(D // 128)]
    gx = g0 * 16 if isinstance(g0, int) else pl.multiple_of(g0 * 16, 16)
    gw = g0 * 8 if isinstance(g0, int) else pl.multiple_of(g0 * 8, 8)
    for n_, (rg, w) in enumerate(items):
        def gate(rg=rg, w=w):
            xn = xn_buf[pl.ds(gx + 16 * rg, 16), pl.ds(w * 128, 128)].astype(f32)
            w_buf[pl.ds(z0 + gw + (P["GB"] + w * (S // 2) + 8 * rg), 8), :] = pltpu.bitcast((xn * sigmoid(xn)).astype(bf16), f32)
        add(P["GS"] + n_ * P["GD"], 0, gate)
    ev.sort(key=lambda e: e[:3])
    for e in ev: e[3]()


def make(flags=None, **kw):
    P = dict(BQ=128, NU=16, KC=512, DL=2, LA=4, LAL=4, LS=3, PD=8, LC=2, XD=9, FD=2, QA=2, BX=256, G=4, BO=256, HA=8, SKIP="",
             DS=('x0 wr q0 x1', 'x2', '', 'x3', '', 'q1', 'qr'), GS=50, GD=2, UO=2, UJ=2, F0=19, FG=8, XB=1, DENSE=1, LN=64, XA=(0, 1, 2, 4, 8))
    P.update(kw)
    BQ, NU, KC, BX, G, BO, HA = (P[k] for k in "BQ NU KC BX G BO HA".split())
    P["QB"] = QB = 5 * BQ
    P["GB"] = GB = QB + H * S // 2
    NB = S // BQ; NX = S // BX; NG = H // G; NO = S // BO
    L = SK // KC + P["DL"]

    def kernel(x_hbm, k_hbm, v_hbm, wq_hbm, wo_hbm, wr_hbm, wg_hbm, wu_hbm, wd_hbm, out_hbm,
               x_buf, xn_buf, w_buf, s_buf0, s_buf1, k_buf, v_buf, wq_buf, wo_buf, wr_buf, wg_buf, wu_buf, wd_buf, out_buf, z_ref,
               x_sem, wq_sem, kv_sem, misc_sem, out_sem):
        XA = P["XA"]; LN = P["LN"]
        xr = [(a_ * BX, (b_ - a_) * BX) for a_, b_ in zip(XA[:-1], XA[1:])]
        x_cp = lambda i: pltpu.make_async_copy(x_hbm.at[pl.ds(*xr[i])], x_buf.at[pl.ds(*xr[i])], x_sem.at[i])
        wq_cp = lambda j: pltpu.make_async_copy(wq_hbm.at[:, pl.ds(j * G * DH, G * DH)], wq_buf.at[j], wq_sem.at[j])
        hr = [(0, HA), (HA, H - HA)]
        k_cp = lambda j: pltpu.make_async_copy(k_hbm.at[pl.ds(*hr[j])], k_buf.at[pl.ds(*hr[j])], kv_sem.at[2 * j])
        v_cp = lambda j: pltpu.make_async_copy(v_hbm.at[pl.ds(*hr[j])], v_buf.at[pl.ds(*hr[j])], kv_sem.at[2 * j + 1])
        wr_cp = lambda: pltpu.make_async_copy(wr_hbm, wr_buf, misc_sem.at[0])
        wg_cp = lambda: pltpu.make_async_copy(wg_hbm, wg_buf, misc_sem.at[1])
        wu_cp = lambda: pltpu.make_async_copy(wu_hbm, wu_buf, misc_sem.at[2])
        wd_cp = lambda: pltpu.make_async_copy(wd_hbm, wd_buf, misc_sem.at[3])
        wo_cp = lambda: pltpu.make_async_copy(wo_hbm, wo_buf, misc_sem.at[4])

        cur = []
        def mark(name):
            if not P.get("PROF"): return
            if cur: cur.pop().__exit__(None, None, None)
            if name:
                cm = jax.named_scope(name); cm.__enter__(); cur.append(cm)
        mark("p0_wait_x0")
        cps = dict(x0=lambda: x_cp(0), x1=lambda: x_cp(1), x2=lambda: x_cp(2), x3=lambda: x_cp(3), wr=wr_cp,
                   q0=lambda: wq_cp(0), q1=lambda: wq_cp(1))
        def start(stage):
            for nm in P["DS"][stage].split():
                if nm == "qr":
                    for j in range(2, NG): wq_cp(j).start()
                else: cps[nm]().start()
        start(0)
        z_ref[0] = 0
        z_ref[1] = 0

        def store_q(j, g, i, q):
            q = (q * (DH ** -0.5 * LOG2E)).astype(bf16)
            r0 = pl.multiple_of(QB + (j * G + g) * (S // 2) + i * (BX // 2), 32)
            w_buf[pl.ds(r0, BX // 2), :] = pltpu.bitcast(q, f32)
            return q

        def qproj(j, i):
            q = jnp.dot(xn_buf[pl.ds(i * BX, BX), :], wq_buf[j], preferred_element_type=f32)
            return [store_q(j, g, i, q[:, g * DH:(g + 1) * DH]) for g in range(G)]

        lane = lax.broadcasted_iota(i32, (8, 128), 1)
        sub = lax.broadcasted_iota(i32, (8, 128), 0)

        def layernorm(r0, n):
            x = x_buf[pl.ds(r0, n), :].astype(f32)
            m = jnp.sum(x, axis=-1, keepdims=True)
            yield
            m = m * (1.0 / D)
            mb = rb(m)
            xc = x - mb
            dm = m - mb
            var = jnp.sum(xc * xc, axis=-1, keepdims=True)
            if P["XB"]: xb = xc.astype(bf16)
            yield
            var = jnp.broadcast_to(var * (1.0 / D) - dm * dm, (n, 128))
            if P["DENSE"]:
                dense = var[:8]
                for t in range(1, n // 8):
                    dense = jnp.where(lane == t, var[t * 8:(t + 1) * 8], dense)
                inv = 1.0 / rb(jnp.sqrt(rb(rb(jnp.maximum(dense, 0.0)) + EPS)))
                inv = jnp.concatenate([jnp.broadcast_to(inv[:, t:t + 1], (8, 128)) for t in range(n // 8)], axis=0)
                yield
            else:
                inv = 1.0 / rb(jnp.sqrt(rb(rb(jnp.maximum(var, 0.0)) + EPS)))
            xr_ = xb.astype(f32) if P["XB"] else rb(xc)
            xn = jnp.concatenate([xr_[:, w * 128:(w + 1) * 128] * inv for w in range(D // 128)], axis=1).astype(bf16)
            xn_buf[pl.ds(r0, n), :] = xn
            r = jnp.broadcast_to(jnp.sum(xn.astype(f32) * wr, axis=-1, keepdims=True), (n, 128))
            yield "stored"
            for t in range(n // 8):
                pos = r0 // 8 + t
                rd[pos // 128] = jnp.where(lane == pos % 128, r[t * 8:(t + 1) * 8], rd[pos // 128])

        ln = dict(next=0, done=0, live=[])
        def layernorm_upto(row, avail):
            while ln["done"] < row:
                for gen in list(ln["live"]):
                    st_ = next(gen, "end")
                    if st_ == "stored": ln["done"] += LN
                    if st_ == "end": ln["live"].remove(gen)
                if ln["next"] < avail:
                    gen = layernorm(ln["next"], LN); next(gen)
                    ln["live"].append(gen); ln["next"] += LN

        x_cp(0).wait()
        start(1)
        wr_cp().wait()
        mark('p1_ln0')
        wr = wr_buf[...].astype(f32).reshape(1, D)
        rd = [jnp.zeros((8, 128), f32) for _ in range(S // 1024)]
        layernorm_upto(BX, BX)
        mark('p2_wait_wq0')
        wq_cp(0).wait()
        start(2)
        starts = [r[0] // BX for r in xr]
        for i in range(NX):
            if i + 1 in starts:
                n_ = starts.index(i + 1)
                mark(f'p3_wait_x{n_}')
                start(2 + n_)
                x_cp(n_).wait()
                avail = xr[n_][0] + xr[n_][1]
            if i + 1 in starts: mark(f'p3_q{i}')
            qproj(0, i)
            if i + 1 < NX:
                layernorm_upto((i + 2) * BX, avail)
        for gen in ln["live"]:
            for _ in gen: pass
        start(6)
        mark('p35_wait_q1')
        wq_cp(1).wait()
        mark('p36_j1')
        for i in range(NX):
            qproj(1, i)

        mark('p4_wait_wq')
        for j in range(2, NG):
            if j == NG - 1:
                wg_cp().start(); wu_cp().start(); wd_cp().start(); k_cp(0).start(); v_cp(0).start()
            wq_cp(j).wait()
        mark('p5_1b')
        UJ = P["UJ"]
        if UJ:
            def p1_body(jj, _):
                for u in range(UJ):
                    for i in range(NX):
                        qproj(2 + jj * UJ + u, i)
            lax.fori_loop(0, (NG - 4) // UJ, p1_body, None)
        else:
            for j in range(2, NG - 2):
                for i in range(NX):
                    qproj(j, i)

        mark('p6_wait')
        wg_cp().wait(); wu_cp().wait(); wd_cp().wait()
        k_cp(1).start(); v_cp(1).start(); wo_cp().start()
        k_cp(0).wait(); v_cp(0).wait()
        mark('p7_1c')
        keys = []
        for t in range(len(rd)):
            r = rb(rd[t])
            r = jnp.where(r == 0.0, 0.0, r)
            b = lax.shift_right_logical(pltpu.bitcast(r, i32), 16)
            k16 = jnp.where(b >= 0x8000, 0xFFFF - b, b + 0x8000)
            k16 = jnp.where(r != r, 0, k16)
            tok = t * 1024 + lane * 8 + sub
            keys.append(pltpu.bitcast(0x20000000 + k16 * 2048 + (2047 - tok), f32))
        idxs = []
        ktop = jnp.zeros((8, 128), i32)
        for c in range(C):
            mx = functools.reduce(jnp.maximum, keys)
            mx = jnp.max(jnp.max(mx, axis=0, keepdims=True), axis=1, keepdims=True)
            mxb = jnp.broadcast_to(mx, (8, 128))
            keys = [jnp.where(kk == mxb, 0.0, kk) for kk in keys]
            mi = pltpu.bitcast(mxb, i32)
            ktop = jnp.where(sub == c, mi, ktop)
            idxs.append(2047 - (mi[0, 0] & 2047))
        k16 = lax.shift_right_logical(ktop - 0x20000000, 11)
        b = jnp.where(k16 >= 0x8000, k16 - 0x8000, 0xFFFF - k16)
        r_sel = pltpu.bitcast(lax.shift_left(b, 16), f32)[:, :1]
        row16 = lax.broadcasted_iota(i32, (16, D), 0)
        row8 = lax.broadcasted_iota(i32, (8, D), 0)
        x_sel = jnp.zeros((8, D), f32)
        bases = [pl.multiple_of(ix & -16, 16) for ix in idxs]
        for c in range(C):
            blk = xn_buf[pl.ds(bases[c], 16), :].astype(f32)
            rowv = jnp.sum(jnp.where(row16 == idxs[c] - bases[c], blk, 0.0), axis=0, keepdims=True)
            x_sel = jnp.where(row8 == c, rowv, x_sel)
        xs = x_sel.astype(bf16)
        KT = D // 128
        acc = {}
        def accum(key, d):
            acc[key] = acc[key] + d if key in acc else d
        def q_tile(j, i, g, k):
            accum((j, i, g), jnp.dot(xn_buf[pl.ds(i * BX, BX), pl.ds(k * 128, 128)], wq_buf[j, pl.ds(k * 128, 128), pl.ds(g * DH, DH)], preferred_element_type=f32))
            if k == KT - 1:
                store_q(j, g, i, acc.pop((j, i, g)))
        fr = [(f0, min(128, F - f0)) for f0 in range(0, F, 128)]
        def up_tile(name, w, f, k):
            accum((name, f), lax.dot_general(xs[:, k * 128:(k + 1) * 128], w[pl.ds(*fr[f]), pl.ds(k * 128, 128)], NT, preferred_element_type=f32))
        def down_tile(f, n):
            if n == 0:
                a = rb(acc.pop(("g", f)))
                acc["h"] = (rb(a * sigmoid(a)) * rb(acc.pop(("u", f)))).astype(bf16)
            accum(("y", n), jnp.dot(acc["h"], wd_buf[pl.ds(*fr[f]), pl.ds(n * 128, 128)], preferred_element_type=f32))
        part = functools.partial
        q_tiles = [part(q_tile, j, i, g, k) for j in (NG - 2, NG - 1) for i in range(NX) for g in range(G) for k in range(KT)]
        f_tiles = [part(up_tile, nm, w, f, k) for f in range(len(fr)) for nm, w in (("g", wg_buf), ("u", wu_buf)) for k in range(KT)]
        f_tiles += [None] * (4 * P["FG"])
        f_tiles += [part(down_tile, f, n) for f in range(len(fr)) for n in range(KT)]
        for rnd in range(len(q_tiles) // 4):
            for fn_ in q_tiles[4 * rnd:4 * rnd + 4]:
                fn_()
            if rnd >= P["F0"]:
                for fn_ in f_tiles[:4]:
                    if fn_ is not None: fn_()
                f_tiles = f_tiles[4:]
        assert not f_tiles
        y = rb(jnp.concatenate([acc.pop(("y", n)) for n in range(KT)], axis=1))
        z = rb(x_sel + rb(y * rb(sigmoid(r_sel))))
        for c in range(C):
            blk = xn_buf[pl.ds(bases[c], 16), :].astype(f32)
            xn_buf[pl.ds(bases[c], 16), :] = jnp.where(row16 == idxs[c] - bases[c], z[c:c + 1, :], blk).astype(bf16)

        mark('p8_att')
        NIT, N0 = divmod(H * NB, NU)
        GPI, G0 = divmod(S // 16, NIT)
        opaque = lambda i: pl.multiple_of(z_ref[i], 32)
        if N0 and "a" not in P["SKIP"]:
            attention_body(0, N0, 0, G0, opaque(0), opaque(1), w_buf, (s_buf0, s_buf1), k_buf, v_buf, xn_buf, P)
        TA = (HA * NB - N0) // NU
        z0, z1 = opaque(0), opaque(1)
        def att_body(t, _):
            @pl.when(t == TA)
            def _():
                k_cp(1).wait(); v_cp(1).wait(); wo_cp().wait()
            if "a" not in P["SKIP"]:
                attention_body(N0 + t * NU, NU, G0 + t * GPI, GPI, z0, z1, w_buf, (s_buf0, s_buf1), k_buf, v_buf, xn_buf, P)
        lax.fori_loop(0, NIT, att_body, None)

        out_cp = lambda i: pltpu.make_async_copy(out_buf.at[pl.ds(i * BO, BO)], out_hbm.at[pl.ds(i * BO, BO)], out_sem.at[i])
        mark('p9_out')
        UO = P["UO"]
        def p3_body(ii, _):
            for u in range(UO):
                i = ii * UO + u
                r0 = pl.multiple_of(i * BO, BO)
                packed = lambda base, n: jnp.concatenate([pltpu.bitcast(w_buf[pl.ds(pl.multiple_of(base + h * (S // 2) + i * (BO // 2), 32), BO // 2), :], bf16) for h in range(n)], axis=-1)
                s = jnp.dot(packed(QB, H), wo_buf[...], preferred_element_type=f32)
                out_buf[pl.ds(r0, BO), :] = (x_buf[pl.ds(r0, BO), :].astype(f32) + s * packed(GB, D // 128).astype(f32)).astype(bf16)
                out_cp(i).start()
        if UO == NO:
            p3_body(0, None)
        else:
            lax.fori_loop(0, NO // UO, p3_body, None)
        mark('pa_wait_out')
        for i in range(NO):
            out_cp(i).wait()
        mark(None)

    @jax.jit
    def fn(A_x, A_k_cache, A_v_cache, A_wq, A_wo, B_x, B_w_r, B_w_gate, B_w_up, B_w_down):
        any_spec = pl.BlockSpec(memory_space=pl.ANY)
        s_shape = pltpu.VMEM((L * BQ * (KC // 128) + 32, 128), f32)
        out = pl.pallas_call(
            kernel,
            in_specs=[any_spec] * 9,
            out_specs=any_spec,
            out_shape=jax.ShapeDtypeStruct((S, D), bf16),
            scratch_shapes=[
                pltpu.VMEM((S, D), bf16), pltpu.VMEM((S, D), bf16),
                pltpu.VMEM((GB + D // 128 * S // 2, DH), f32), s_shape, s_shape,
                pltpu.VMEM((H, SK, DH), bf16), pltpu.VMEM((H, SK, DH), bf16),
                pltpu.VMEM((NG, D, G * DH), bf16), pltpu.VMEM((H * DH, D), bf16),
                pltpu.VMEM((D,), bf16), pltpu.VMEM((F, D), bf16), pltpu.VMEM((F, D), bf16), pltpu.VMEM((F, D), bf16),
                pltpu.VMEM((S, D), bf16), pltpu.SMEM((2,), i32),
                pltpu.SemaphoreType.DMA((len(P['XA']) - 1,)), pltpu.SemaphoreType.DMA((NG,)), pltpu.SemaphoreType.DMA((4,)),
                pltpu.SemaphoreType.DMA((5,)), pltpu.SemaphoreType.DMA((NO,)),
            ],
            compiler_params=pltpu.CompilerParams(vmem_limit_bytes=120 * 1024 * 1024, flags=flags),
            name="fused_kernel",
        )(A_x.reshape(S, D), A_k_cache.reshape(H, SK, DH), A_v_cache.reshape(H, SK, DH), A_wq, A_wo,
          B_w_r, B_w_gate.T, B_w_up.T, B_w_down)
        return out.reshape(1, S, D)
    return fn


_impl = make(NU=21)


@jax.jit
def pallas_recurrent_scan__mha_block_cached__moe_arch_mod__prompt_kernel(
    A_x, A_k_cache, A_v_cache, A_wq, A_wo, B_x, B_w_r, B_w_gate, B_w_up, B_w_down
):
    return _impl(A_x, A_k_cache, A_v_cache, A_wq, A_wo, B_x, B_w_r, B_w_gate, B_w_up, B_w_down)
```

```python
import functools
import numpy as np
import jax
import jax.numpy as jnp
from jax import lax
import jax.experimental.pallas as pl
import jax.experimental.pallas.tpu as pltpu

S, D, H, DH, SK, F, C = 2048, 640, 32, 128, 2048, 1728, 8
LOG2E = 1.4426950408889634
EPS = float(np.asarray(1e-5, dtype=jnp.bfloat16))
f32, bf16, i32 = jnp.float32, jnp.bfloat16, jnp.int32
NT = (((1,), (1,)), ((), ()))


def rb(x):
    return x.astype(bf16).astype(f32)


def sigmoid(x):
    return 1.0 / (1.0 + jnp.exp2(x * (-LOG2E)))


def attention_body(n0, NU, g0, NGR, z0, z1, w_buf, s_bufs, a_bufs, k_buf, v_buf, xn_buf, P):
    BQ, KC, DL = P["BQ"], P["KC"], P["DL"]
    LA, LS, PD, LC, XD, FD, QA = (P[k] for k in "LA LS PD LC XD FD QA".split())
    NB = S // BQ; R = BQ // 16; NC = SK // KC; W = KC // 128; L = NC + DL
    def s_loc(g, w, r):
        return (g // L) % len(s_bufs), (((g % L) * R + r) * W + w) * 16
    def ld_s(g, w, r):
        par, o = s_loc(g, w, r)
        return s_bufs[par][pl.ds(z1 + o, 16), :]
    def st_s(g, w, r, v):
        par, o = s_loc(g, w, r)
        s_bufs[par][pl.ds(z0 + o, 16), :] = v
    def st_tok(g, v):
        s_bufs[s_loc(g, 0, 0)[0]][pl.ds(z0 + L * R * W * 16, 8), :] = v
    MX, LP, OA = 0, BQ, 2 * BQ
    def ld(a, off, r): return a_bufs[a % len(a_bufs)][pl.ds(z1 + (off + 16 * r), 16), :]
    def st(a, off, r, v): a_bufs[a % len(a_bufs)][pl.ds(z0 + (off + 16 * r), 16), :] = v
    heads = [(n0 + u) // NB if isinstance(n0, int) else lax.shift_right_logical(n0 + u, NB.bit_length() - 1) for u in range(NU)]
    qbase = P["QB"] + n0 * (BQ // 2)
    if not isinstance(n0, int): qbase = pl.multiple_of(qbase, 32)
    qrow = [qbase + u * (BQ // 2) for u in range(NU)]
    dots = []
    for g in range(NU * NC + L):
        if g < NU * NC: dots.append(("qk", g))
        if g - L >= 0: dots.append(("pv", g - L))
    ev = []; val = {}
    def add(slot, prio, fn): ev.append((slot, prio, len(ev), fn))
    def res(i):
        if ("res", i) not in val:
            kind, g = dots[i]; a, c = divmod(g, NC); h = heads[a]
            if kind == "qk":
                q = pltpu.bitcast(jnp.concatenate([val.pop(("q", i, r)) for r in range(R)], axis=0), bf16)
                val["res", i] = lax.dot_general(q, k_buf[h, pl.ds(c * KC, KC), :], NT, preferred_element_type=f32)
            else:
                p = jnp.concatenate([val.pop(("p", i, r)) for r in range(R)], axis=0).astype(bf16)
                val["res", i] = jnp.dot(p, v_buf[h, pl.ds(c * KC, KC), :], preferred_element_type=f32)
        return val["res", i]
    for i, (kind, g) in enumerate(dots):
        a, c = divmod(g, NC)
        la = P["LAL"] if i == len(dots) - 1 else LA
        for r in range(R):
            j = i * R + r
            if kind == "qk":
                def l_q(i=i, a=a, r=r):
                    if "tok" in val and r % P["QT"] == 0: w_buf[pl.ds(z0, 8), :] = val["tok"]
                    val["q", i, r] = w_buf[pl.ds(z1 + qrow[a] + 8 * r, 8), :]
                add(min(j - QA, i * R + PD - 1), 1, l_q)
                if c > 0:
                    def l_acc(a=a, r=r): val["mx", a, r] = ld(a, MX, r)
                    add(j + PD - LC, 1, l_acc)
                def s_res(i=i, g=g, a=a, c=c, r=r):
                    s = res(i)[16 * r:16 * r + 16]
                    tiles = [s[:, w * 128:(w + 1) * 128] for w in range(W)]
                    for w in range(W): st_s(g, w, r, tiles[w])
                    val["tok"] = tiles[W - 1][:8]
                    mx = functools.reduce(jnp.maximum, tiles)
                    if c > 0: mx = jnp.maximum(mx, val.pop(("mx", a, r)))
                    if c == NC - 1:
                        val["m", a, r] = jnp.broadcast_to(jnp.max(mx, axis=-1, keepdims=True), (16, 128))
                    else: st(a, MX, r, mx)
                add(j + PD, 0, s_res)
                if c == NC - 1:
                    def s_m(a=a, r=r): st(a, MX, r, val.pop(("m", a, r)))
                    add(j + PD + XD, 0, s_m)
            else:
                def l_lhs(i=i, g=g, a=a, c=c, r=r):
                    m = ld(a, MX, r)
                    if "tok" in val: st_tok(g, val["tok"])
                    ps = [jnp.exp2(ld_s(g, w, r) - m) for w in range(W)]
                    lp = functools.reduce(lax.add, ps)
                    if c > 0: lp = lp + ld(a, LP, r)
                    val["lp", i, r] = lp
                    val["p", i, r] = jnp.concatenate(ps, axis=1)
                add(min(j - la, i * R + PD - 1), 1, l_lhs)
                if c < NC - 1:
                    def s_lp(i=i, a=a, r=r): st(a, LP, r, val.pop(("lp", i, r)))
                    add(j - la + LS, 0, s_lp)
                if c > 0:
                    def l_acc(i=i, a=a, r=r): val["o", i, r] = ld(a, OA, r)
                    add(j + PD - LC, 1, l_acc)
                if c < NC - 1:
                    def s_res(i=i, a=a, c=c, r=r):
                        d = res(i)[16 * r:16 * r + 16]
                        if c > 0: d = d + val.pop(("o", i, r))
                        val["tok"] = d[:8]
                        st(a, OA, r, d)
                    add(j + PD, 0, s_res)
                else:
                    def s_res(i=i, r=r):
                        d = res(i)[16 * r:16 * r + 16] + val.pop(("o", i, r))
                        val["tok"] = d[:8]
                        val["of", i, r] = d
                    add(j + PD, 0, s_res)
                    def s_fin(i=i, a=a, r=r):
                        l = jnp.sum(val.pop(("lp", i, r)), axis=-1, keepdims=True)
                        r0 = pl.reciprocal(l, approx=True)
                        rl = r0 * (2.0 - l * r0)
                        ob = pltpu.bitcast((val.pop(("of", i, r)) * rl).astype(bf16), f32)
                        w_buf[pl.ds(z0 + qrow[a] + 8 * r, 8), :] = ob
                    add(max(j - la + LS + XD + FD, j + PD), 0, s_fin)
    items = [(rg, w) for rg in range(NGR) for w in range(D // 128)]
    gx = g0 * 16 if isinstance(g0, int) else pl.multiple_of(g0 * 16, 16)
    gw = g0 * 8 if isinstance(g0, int) else pl.multiple_of(g0 * 8, 8)
    for n_, (rg, w) in enumerate(items):
        def gate(rg=rg, w=w):
            xn = xn_buf[pl.ds(gx + 16 * rg, 16), pl.ds(w * 128, 128)].astype(f32)
            w_buf[pl.ds(z0 + gw + (P["GB"] + w * (S // 2) + 8 * rg), 8), :] = pltpu.bitcast((xn * sigmoid(xn)).astype(bf16), f32)
        add(P["GS"] + n_ * P["GD"], 0, gate)
    ev.sort(key=lambda e: e[:3])
    for e in ev: e[3]()


def make(flags=None, **kw):
    P = dict(BQ=128, NU=16, KC=512, DL=2, LA=4, LAL=4, LS=3, PD=8, LC=2, XD=9, FD=2, QA=2, BX=256, G=4, BO=256, HA=8, SKIP="",
             DS=('x0 wr q0 x1', 'x2', '', 'x3', '', 'q1', 'qr'), NSB=8, NAB=8, QT=8, GS=50, GD=2, UO=2, UJ=2, F0=19, FG=8, XB=1, DENSE=1, LN=64, XA=(0, 1, 2, 4, 8))
    P.update(kw)
    BQ, NU, KC, BX, G, BO, HA = (P[k] for k in "BQ NU KC BX G BO HA".split())
    P["QB"] = QB = 32
    P["GB"] = GB = QB + H * S // 2
    NB = S // BQ; NX = S // BX; NG = H // G; NO = S // BO
    L = SK // KC + P["DL"]

    def kernel(x_hbm, k_hbm, v_hbm, wq_hbm, wo_hbm, wr_hbm, wg_hbm, wu_hbm, wd_hbm, out_hbm,
               x_buf, xn_buf, w_buf, k_buf, v_buf, wq_buf, wo_buf, wg_buf, wu_buf, wd_buf, out_buf, z_ref,
               x_sem, wq_sem, kv_sem, misc_sem, out_sem, *bufs):
        s_bufs, a_bufs, wr_buf = bufs[:P['NSB']], bufs[P['NSB']:-1], bufs[-1]
        XA = P["XA"]; LN = P["LN"]
        xr = [(a_ * BX, (b_ - a_) * BX) for a_, b_ in zip(XA[:-1], XA[1:])]
        x_cp = lambda i: pltpu.make_async_copy(x_hbm.at[pl.ds(*xr[i])], x_buf.at[pl.ds(*xr[i])], x_sem.at[i])
        wq_cp = lambda j: pltpu.make_async_copy(wq_hbm.at[:, pl.ds(j * G * DH, G * DH)], wq_buf.at[j], wq_sem.at[j])
        hr = [(0, HA), (HA, H - HA)]
        k_cp = lambda j: pltpu.make_async_copy(k_hbm.at[pl.ds(*hr[j])], k_buf.at[pl.ds(*hr[j])], kv_sem.at[2 * j])
        v_cp = lambda j: pltpu.make_async_copy(v_hbm.at[pl.ds(*hr[j])], v_buf.at[pl.ds(*hr[j])], kv_sem.at[2 * j + 1])
        wr_cp = lambda: pltpu.make_async_copy(wr_hbm, wr_buf, misc_sem.at[0])
        wg_cp = lambda: pltpu.make_async_copy(wg_hbm, wg_buf, misc_sem.at[1])
        wu_cp = lambda: pltpu.make_async_copy(wu_hbm, wu_buf, misc_sem.at[2])
        wd_cp = lambda: pltpu.make_async_copy(wd_hbm, wd_buf, misc_sem.at[3])
        wo_cp = lambda: pltpu.make_async_copy(wo_hbm, wo_buf, misc_sem.at[4])

        cur = []
        def mark(name):
            if not P.get("PROF"): return
            if cur: cur.pop().__exit__(None, None, None)
            if name:
                cm = jax.named_scope(name); cm.__enter__(); cur.append(cm)
        mark("p0_wait_x0")
        cps = dict(x0=lambda: x_cp(0), x1=lambda: x_cp(1), x2=lambda: x_cp(2), x3=lambda: x_cp(3), wr=wr_cp,
                   q0=lambda: wq_cp(0), q1=lambda: wq_cp(1))
        def start(stage):
            for nm in P["DS"][stage].split():
                if nm == "qr":
                    for j in range(2, NG): wq_cp(j).start()
                else: cps[nm]().start()
        start(0)
        z_ref[0] = 0
        z_ref[1] = 0

        def store_q(j, g, i, q):
            q = (q * (DH ** -0.5 * LOG2E)).astype(bf16)
            r0 = pl.multiple_of(QB + (j * G + g) * (S // 2) + i * (BX // 2), 32)
            w_buf[pl.ds(r0, BX // 2), :] = pltpu.bitcast(q, f32)
            return q

        def qproj(j, i):
            q = jnp.dot(xn_buf[pl.ds(i * BX, BX), :], wq_buf[j], preferred_element_type=f32)
            return [store_q(j, g, i, q[:, g * DH:(g + 1) * DH]) for g in range(G)]

        lane = lax.broadcasted_iota(i32, (8, 128), 1)
        sub = lax.broadcasted_iota(i32, (8, 128), 0)

        def layernorm(r0, n):
            x = x_buf[pl.ds(r0, n), :].astype(f32)
            m = jnp.sum(x, axis=-1, keepdims=True)
            yield
            m = m * (1.0 / D)
            mb = rb(m)
            xc = x - mb
            dm = m - mb
            var = jnp.sum(xc * xc, axis=-1, keepdims=True)
            if P["XB"]: xb = xc.astype(bf16)
            yield
            var = jnp.broadcast_to(var * (1.0 / D) - dm * dm, (n, 128))
            if P["DENSE"]:
                dense = var[:8]
                for t in range(1, n // 8):
                    dense = jnp.where(lane == t, var[t * 8:(t + 1) * 8], dense)
                inv = 1.0 / rb(jnp.sqrt(rb(rb(jnp.maximum(dense, 0.0)) + EPS)))
                inv = jnp.concatenate([jnp.broadcast_to(inv[:, t:t + 1], (8, 128)) for t in range(n // 8)], axis=0)
                yield
            else:
                inv = 1.0 / rb(jnp.sqrt(rb(rb(jnp.maximum(var, 0.0)) + EPS)))
            xr_ = xb.astype(f32) if P["XB"] else rb(xc)
            xn = jnp.concatenate([xr_[:, w * 128:(w + 1) * 128] * inv for w in range(D // 128)], axis=1).astype(bf16)
            xn_buf[pl.ds(r0, n), :] = xn
            r = jnp.broadcast_to(jnp.sum(xn.astype(f32) * wr, axis=-1, keepdims=True), (n, 128))
            yield "stored"
            for t in range(n // 8):
                pos = r0 // 8 + t
                rd[pos // 128] = jnp.where(lane == pos % 128, r[t * 8:(t + 1) * 8], rd[pos // 128])

        ln = dict(next=0, done=0, live=[])
        def layernorm_upto(row, avail):
            while ln["done"] < row:
                for gen in list(ln["live"]):
                    st_ = next(gen, "end")
                    if st_ == "stored": ln["done"] += LN
                    if st_ == "end": ln["live"].remove(gen)
                if ln["next"] < avail:
                    gen = layernorm(ln["next"], LN); next(gen)
                    ln["live"].append(gen); ln["next"] += LN

        x_cp(0).wait()
        start(1)
        wr_cp().wait()
        mark('p1_ln0')
        wr = wr_buf[...].astype(f32).reshape(1, D)
        rd = [jnp.zeros((8, 128), f32) for _ in range(S // 1024)]
        layernorm_upto(BX, BX)
        mark('p2_wait_wq0')
        wq_cp(0).wait()
        start(2)
        starts = [r[0] // BX for r in xr]
        for i in range(NX):
            if i + 1 in starts:
                n_ = starts.index(i + 1)
                mark(f'p3_wait_x{n_}')
                start(2 + n_)
                x_cp(n_).wait()
                avail = xr[n_][0] + xr[n_][1]
            if i + 1 in starts: mark(f'p3_q{i}')
            qproj(0, i)
            if i + 1 < NX:
                layernorm_upto((i + 2) * BX, avail)
        for gen in ln["live"]:
            for _ in gen: pass
        start(6)
        mark('p35_wait_q1')
        wq_cp(1).wait()
        mark('p36_j1')
        for i in range(NX):
            qproj(1, i)

        mark('p4_wait_wq')
        for j in range(2, NG):
            if j == NG - 1:
                wg_cp().start(); wu_cp().start(); wd_cp().start(); k_cp(0).start(); v_cp(0).start()
            wq_cp(j).wait()
        mark('p5_1b')
        UJ = P["UJ"]
        if UJ:
            def p1_body(jj, _):
                for u in range(UJ):
                    for i in range(NX):
                        qproj(2 + jj * UJ + u, i)
            lax.fori_loop(0, (NG - 4) // UJ, p1_body, None)
        else:
            for j in range(2, NG - 2):
                for i in range(NX):
                    qproj(j, i)

        mark('p6_wait')
        wg_cp().wait(); wu_cp().wait(); wd_cp().wait()
        k_cp(1).start(); v_cp(1).start(); wo_cp().start()
        k_cp(0).wait(); v_cp(0).wait()
        mark('p7_1c')
        keys = []
        for t in range(len(rd)):
            r = rb(rd[t])
            r = jnp.where(r == 0.0, 0.0, r)
            b = lax.shift_right_logical(pltpu.bitcast(r, i32), 16)
            k16 = jnp.where(b >= 0x8000, 0xFFFF - b, b + 0x8000)
            k16 = jnp.where(r != r, 0, k16)
            tok = t * 1024 + lane * 8 + sub
            keys.append(pltpu.bitcast(0x20000000 + k16 * 2048 + (2047 - tok), f32))
        idxs = []
        ktop = jnp.zeros((8, 128), i32)
        for c in range(C):
            mx = functools.reduce(jnp.maximum, keys)
            mx = jnp.max(jnp.max(mx, axis=0, keepdims=True), axis=1, keepdims=True)
            mxb = jnp.broadcast_to(mx, (8, 128))
            keys = [jnp.where(kk == mxb, 0.0, kk) for kk in keys]
            mi = pltpu.bitcast(mxb, i32)
            ktop = jnp.where(sub == c, mi, ktop)
            idxs.append(2047 - (mi[0, 0] & 2047))
        k16 = lax.shift_right_logical(ktop - 0x20000000, 11)
        b = jnp.where(k16 >= 0x8000, k16 - 0x8000, 0xFFFF - k16)
        r_sel = pltpu.bitcast(lax.shift_left(b, 16), f32)[:, :1]
        row16 = lax.broadcasted_iota(i32, (16, D), 0)
        row8 = lax.broadcasted_iota(i32, (8, D), 0)
        x_sel = jnp.zeros((8, D), f32)
        bases = [pl.multiple_of(ix & -16, 16) for ix in idxs]
        for c in range(C):
            blk = xn_buf[pl.ds(bases[c], 16), :].astype(f32)
            rowv = jnp.sum(jnp.where(row16 == idxs[c] - bases[c], blk, 0.0), axis=0, keepdims=True)
            x_sel = jnp.where(row8 == c, rowv, x_sel)
        xs = x_sel.astype(bf16)
        KT = D // 128
        acc = {}
        def accum(key, d):
            acc[key] = acc[key] + d if key in acc else d
        def q_tile(j, i, g, k):
            accum((j, i, g), jnp.dot(xn_buf[pl.ds(i * BX, BX), pl.ds(k * 128, 128)], wq_buf[j, pl.ds(k * 128, 128), pl.ds(g * DH, DH)], preferred_element_type=f32))
            if k == KT - 1:
                store_q(j, g, i, acc.pop((j, i, g)))
        fr = [(f0, min(128, F - f0)) for f0 in range(0, F, 128)]
        def up_tile(name, w, f, k):
            accum((name, f), lax.dot_general(xs[:, k * 128:(k + 1) * 128], w[pl.ds(*fr[f]), pl.ds(k * 128, 128)], NT, preferred_element_type=f32))
        def down_tile(f, n):
            if n == 0:
                a = rb(acc.pop(("g", f)))
                acc["h"] = (rb(a * sigmoid(a)) * rb(acc.pop(("u", f)))).astype(bf16)
            accum(("y", n), jnp.dot(acc["h"], wd_buf[pl.ds(*fr[f]), pl.ds(n * 128, 128)], preferred_element_type=f32))
        part = functools.partial
        q_tiles = [part(q_tile, j, i, g, k) for j in (NG - 2, NG - 1) for i in range(NX) for g in range(G) for k in range(KT)]
        f_tiles = [part(up_tile, nm, w, f, k) for f in range(len(fr)) for nm, w in (("g", wg_buf), ("u", wu_buf)) for k in range(KT)]
        f_tiles += [None] * (4 * P["FG"])
        f_tiles += [part(down_tile, f, n) for f in range(len(fr)) for n in range(KT)]
        for rnd in range(len(q_tiles) // 4):
            for fn_ in q_tiles[4 * rnd:4 * rnd + 4]:
                fn_()
            if rnd >= P["F0"]:
                for fn_ in f_tiles[:4]:
                    if fn_ is not None: fn_()
                f_tiles = f_tiles[4:]
        assert not f_tiles
        y = rb(jnp.concatenate([acc.pop(("y", n)) for n in range(KT)], axis=1))
        z = rb(x_sel + rb(y * rb(sigmoid(r_sel))))
        for c in range(C):
            blk = xn_buf[pl.ds(bases[c], 16), :].astype(f32)
            xn_buf[pl.ds(bases[c], 16), :] = jnp.where(row16 == idxs[c] - bases[c], z[c:c + 1, :], blk).astype(bf16)

        mark('p8_att')
        NIT, N0 = divmod(H * NB, NU)
        GPI, G0 = divmod(S // 16, NIT)
        opaque = lambda i: pl.multiple_of(z_ref[i], 32)
        if N0 and "a" not in P["SKIP"]:
            attention_body(0, N0, 0, G0, opaque(0), opaque(1), w_buf, s_bufs, a_bufs, k_buf, v_buf, xn_buf, P)
        TA = (HA * NB - N0) // NU
        z0, z1 = opaque(0), opaque(1)
        def att_body(t, _):
            @pl.when(t == TA)
            def _():
                k_cp(1).wait(); v_cp(1).wait(); wo_cp().wait()
            if "a" not in P["SKIP"]:
                attention_body(N0 + t * NU, NU, G0 + t * GPI, GPI, z0, z1, w_buf, s_bufs, a_bufs, k_buf, v_buf, xn_buf, P)
        lax.fori_loop(0, NIT, att_body, None)

        out_cp = lambda i: pltpu.make_async_copy(out_buf.at[pl.ds(i * BO, BO)], out_hbm.at[pl.ds(i * BO, BO)], out_sem.at[i])
        mark('p9_out')
        UO = P["UO"]
        def p3_body(ii, _):
            for u in range(UO):
                i = ii * UO + u
                r0 = pl.multiple_of(i * BO, BO)
                packed = lambda base, n: jnp.concatenate([pltpu.bitcast(w_buf[pl.ds(pl.multiple_of(base + h * (S // 2) + i * (BO // 2), 32), BO // 2), :], bf16) for h in range(n)], axis=-1)
                s = jnp.dot(packed(QB, H), wo_buf[...], preferred_element_type=f32)
                out_buf[pl.ds(r0, BO), :] = (x_buf[pl.ds(r0, BO), :].astype(f32) + s * packed(GB, D // 128).astype(f32)).astype(bf16)
                out_cp(i).start()
        if UO == NO:
            p3_body(0, None)
        else:
            lax.fori_loop(0, NO // UO, p3_body, None)
        mark('pa_wait_out')
        for i in range(NO):
            out_cp(i).wait()
        mark(None)

    @jax.jit
    def fn(A_x, A_k_cache, A_v_cache, A_wq, A_wo, B_x, B_w_r, B_w_gate, B_w_up, B_w_down):
        any_spec = pl.BlockSpec(memory_space=pl.ANY)
        s_shape = pltpu.VMEM((L * BQ * (KC // 128) + 32, 128), f32)
        out = pl.pallas_call(
            kernel,
            in_specs=[any_spec] * 9,
            out_specs=any_spec,
            out_shape=jax.ShapeDtypeStruct((S, D), bf16),
            scratch_shapes=[
                pltpu.VMEM((S, D), bf16), pltpu.VMEM((S, D), bf16),
                pltpu.VMEM((GB + D // 128 * S // 2, DH), f32),
                pltpu.VMEM((H, SK, DH), bf16), pltpu.VMEM((H, SK, DH), bf16),
                pltpu.VMEM((NG, D, G * DH), bf16), pltpu.VMEM((H * DH, D), bf16),
                pltpu.VMEM((F, D), bf16), pltpu.VMEM((F, D), bf16), pltpu.VMEM((F, D), bf16),
                pltpu.VMEM((S, D), bf16), pltpu.SMEM((2,), i32),
                pltpu.SemaphoreType.DMA((len(P['XA']) - 1,)), pltpu.SemaphoreType.DMA((NG,)), pltpu.SemaphoreType.DMA((4,)),
                pltpu.SemaphoreType.DMA((5,)), pltpu.SemaphoreType.DMA((NO,)),
            ] + [s_shape] * P['NSB'] + [pltpu.VMEM((3 * BQ, 128), f32)] * P['NAB'] + [pltpu.VMEM((D,), bf16)],
            compiler_params=pltpu.CompilerParams(vmem_limit_bytes=120 * 1024 * 1024, flags=flags),
            name="fused_kernel",
        )(A_x.reshape(S, D), A_k_cache.reshape(H, SK, DH), A_v_cache.reshape(H, SK, DH), A_wq, A_wo,
          B_w_r, B_w_gate.T, B_w_up.T, B_w_down)
        return out.reshape(1, S, D)
    return fn


_impl = make(NU=32)


@jax.jit
def pallas_recurrent_scan__mha_block_cached__moe_arch_mod__prompt_kernel(
    A_x, A_k_cache, A_v_cache, A_wq, A_wo, B_x, B_w_r, B_w_gate, B_w_up, B_w_down
):
    return _impl(A_x, A_k_cache, A_v_cache, A_wq, A_wo, B_x, B_w_r, B_w_gate, B_w_up, B_w_down)
```

```python
import functools
import numpy as np
import jax
import jax.numpy as jnp
from jax import lax
import jax.experimental.pallas as pl
import jax.experimental.pallas.tpu as pltpu

S, D, H, DH, SK, F, C = 2048, 640, 32, 128, 2048, 1728, 8
LOG2E = 1.4426950408889634
EPS = float(np.asarray(1e-5, dtype=jnp.bfloat16))
f32, bf16, i32 = jnp.float32, jnp.bfloat16, jnp.int32
NT = (((1,), (1,)), ((), ()))


def rb(x):
    return x.astype(bf16).astype(f32)


def sigmoid(x):
    return 1.0 / (1.0 + jnp.exp2(x * (-LOG2E)))


def attention_body(n0, NU, g0, NGR, z0, z1, w_buf, s_bufs, a_bufs, k_buf, v_buf, xn_buf, P):
    BQ, KC, DL = P["BQ"], P["KC"], P["DL"]
    LA, LS, PD, LC, XD, FD, QA = (P[k] for k in "LA LS PD LC XD FD QA".split())
    NB = S // BQ; R = BQ // 16; NC = SK // KC; W = KC // 128; L = NC + DL
    def s_loc(g, w, r):
        return (g // L) % len(s_bufs), (((g % L) * R + r) * W + w) * 16
    def ld_s(g, w, r):
        par, o = s_loc(g, w, r)
        return s_bufs[par][pl.ds(z1 + o, 16), :]
    def st_s(g, w, r, v):
        par, o = s_loc(g, w, r)
        s_bufs[par][pl.ds(z0 + o, 16), :] = v
    def st_tok(g, v):
        s_bufs[s_loc(g, 0, 0)[0]][pl.ds(z0 + L * R * W * 16, 8), :] = v
    MX, LP, OA = 0, BQ, 2 * BQ
    def ld(a, off, r): return a_bufs[a % len(a_bufs)][pl.ds(z1 + (off + 16 * r), 16), :]
    def st(a, off, r, v): a_bufs[a % len(a_bufs)][pl.ds(z0 + (off + 16 * r), 16), :] = v
    heads = [(n0 + u) // NB if isinstance(n0, int) else lax.shift_right_logical(n0 + u, NB.bit_length() - 1) for u in range(NU)]
    qbase = P["QB"] + n0 * (BQ // 2)
    if not isinstance(n0, int): qbase = pl.multiple_of(qbase, 32)
    qrow = [qbase + u * (BQ // 2) for u in range(NU)]
    dots = []
    for g in range(NU * NC + L):
        if g < NU * NC: dots.append(("qk", g))
        if g - L >= 0: dots.append(("pv", g - L))
    ev = []; val = {}
    def add(slot, prio, fn): ev.append((slot, prio, len(ev), fn))
    def res(i):
        if ("res", i) not in val:
            kind, g = dots[i]; a, c = divmod(g, NC); h = heads[a]
            if kind == "qk":
                q = pltpu.bitcast(jnp.concatenate([val.pop(("q", i, r)) for r in range(R)], axis=0), bf16)
                val["res", i] = lax.dot_general(q, k_buf[h, pl.ds(c * KC, KC), :], NT, preferred_element_type=f32)
            else:
                p = jnp.concatenate([val.pop(("p", i, r)) for r in range(R)], axis=0).astype(bf16)
                val["res", i] = jnp.dot(p, v_buf[h, pl.ds(c * KC, KC), :], preferred_element_type=f32)
        return val["res", i]
    for i, (kind, g) in enumerate(dots):
        a, c = divmod(g, NC)
        la = P["LAL"] if i == len(dots) - 1 else LA
        for r in range(R):
            j = i * R + r
            if kind == "qk":
                def l_q(i=i, a=a, r=r):
                    if "tok" in val and r % P["QT"] == 0 and i >= 2: w_buf[pl.ds(z0, 8), :] = val["tok"]
                    val["q", i, r] = w_buf[pl.ds((0 if isinstance(n0, int) and i < 2 else z1) + qrow[a] + 8 * r, 8), :]
                add(min(j - QA, i * R + PD - 1), 1, l_q)
                if c > 0:
                    def l_acc(a=a, r=r): val["mx", a, r] = ld(a, MX, r)
                    add(j + PD - LC, 1, l_acc)
                def s_res(i=i, g=g, a=a, c=c, r=r):
                    s = res(i)[16 * r:16 * r + 16]
                    tiles = [s[:, w * 128:(w + 1) * 128] for w in range(W)]
                    for w in range(W): st_s(g, w, r, tiles[w])
                    val["tok"] = tiles[W - 1][:8]
                    mx = functools.reduce(jnp.maximum, tiles)
                    if c > 0: mx = jnp.maximum(mx, val.pop(("mx", a, r)))
                    if c == NC - 1:
                        val["m", a, r] = jnp.broadcast_to(jnp.max(mx, axis=-1, keepdims=True), (16, 128))
                    else: st(a, MX, r, mx)
                add(j + PD, 0, s_res)
                if c == NC - 1:
                    def s_m(a=a, r=r): st(a, MX, r, val.pop(("m", a, r)))
                    add(j + PD + XD, 0, s_m)
            else:
                def l_lhs(i=i, g=g, a=a, c=c, r=r):
                    m = ld(a, MX, r)
                    if "tok" in val: st_tok(g, val["tok"])
                    ps = [jnp.exp2(ld_s(g, w, r) - m) for w in range(W)]
                    lp = functools.reduce(lax.add, ps)
                    if c > 0: lp = lp + ld(a, LP, r)
                    val["lp", i, r] = lp
                    val["p", i, r] = jnp.concatenate(ps, axis=1)
                add(min(j - la, i * R + PD - 1), 1, l_lhs)
                if c < NC - 1:
                    def s_lp(i=i, a=a, r=r): st(a, LP, r, val.pop(("lp", i, r)))
                    add(j - la + LS, 0, s_lp)
                if c > 0:
                    def l_acc(i=i, a=a, r=r): val["o", i, r] = ld(a, OA, r)
                    add(j + PD - LC, 1, l_acc)
                if c < NC - 1:
                    def s_res(i=i, a=a, c=c, r=r):
                        d = res(i)[16 * r:16 * r + 16]
                        if c > 0: d = d + val.pop(("o", i, r))
                        val["tok"] = d[:8]
                        st(a, OA, r, d)
                    add(j + PD, 0, s_res)
                else:
                    def s_res(i=i, r=r):
                        d = res(i)[16 * r:16 * r + 16] + val.pop(("o", i, r))
                        val["tok"] = d[:8]
                        val["of", i, r] = d
                    add(j + PD, 0, s_res)
                    def s_fin(i=i, a=a, r=r):
                        l = jnp.sum(val.pop(("lp", i, r)), axis=-1, keepdims=True)
                        r0 = pl.reciprocal(l, approx=True)
                        rl = r0 * (2.0 - l * r0)
                        ob = pltpu.bitcast((val.pop(("of", i, r)) * rl).astype(bf16), f32)
                        w_buf[pl.ds(z0 + qrow[a] + 8 * r, 8), :] = ob
                    add(max(j - la + LS + XD + FD, j + PD), 0, s_fin)
    items = [(rg, w) for rg in range(NGR) for w in range(D // 128)]
    gx = g0 * 16 if isinstance(g0, int) else pl.multiple_of(g0 * 16, 16)
    gw = g0 * 8 if isinstance(g0, int) else pl.multiple_of(g0 * 8, 8)
    for n_, (rg, w) in enumerate(items):
        def gate(rg=rg, w=w):
            xn = xn_buf[pl.ds(gx + 16 * rg, 16), pl.ds(w * 128, 128)].astype(f32)
            w_buf[pl.ds(z0 + gw + (P["GB"] + w * (S // 2) + 8 * rg), 8), :] = pltpu.bitcast((xn * sigmoid(xn)).astype(bf16), f32)
        add(P["GS"] + n_ * P["GD"], 0, gate)
    ev.sort(key=lambda e: e[:3])
    for e in ev: e[3]()


def make(flags=None, **kw):
    P = dict(BQ=128, NU=39, KC=512, DL=2, LA=4, LAL=4, LS=3, PD=8, LC=2, XD=9, FD=2, QA=2, BX=256, G=4, BO=256, HA=10, SKIP="",
             DS=('x0 wr q0 x1', 'x2', '', 'x3', '', 'q1 qr', ''), BC=256, NJ=2, MB=20, TF=0, RP=128, R0=16, NSB=13, NAB=13, QT=8, GS=50, GD=2, UO=2, UJ=2, F0=0, FG=12, XB=1, DENSE=1, LN=64, XA=(0, 1, 2, 4, 8))
    P.update(kw)
    BQ, NU, KC, BX, G, BO, HA = (P[k] for k in "BQ NU KC BX G BO HA".split())
    P["QB"] = QB = 32
    P["GB"] = GB = QB + H * S // 2
    NB = S // BQ; NX = S // BX; NG = H // G; NO = S // BO
    L = SK // KC + P["DL"]

    def kernel(x_hbm, k_hbm, v_hbm, wq_hbm, wo_hbm, wr_hbm, wg_hbm, wu_hbm, wd_hbm, out_hbm,
               x_buf, xn_buf, w_buf, k_buf, v_buf, wq_buf, wo_buf, wg_buf, wu_buf, wd_buf, out_buf, z_ref,
               x_sem, wq_sem, kv_sem, misc_sem, out_sem, *bufs):
        s_bufs, a_bufs, wr_buf = bufs[:P['NSB']], bufs[P['NSB']:-1], bufs[-1]
        XA = P["XA"]; LN = P["LN"]
        xr = [(a_ * BX, (b_ - a_) * BX) for a_, b_ in zip(XA[:-1], XA[1:])]
        x_cp = lambda i: pltpu.make_async_copy(x_hbm.at[pl.ds(*xr[i])], x_buf.at[pl.ds(*xr[i])], x_sem.at[i])
        wq_cp = lambda j: pltpu.make_async_copy(wq_hbm.at[:, pl.ds(j * G * DH, G * DH)], wq_buf.at[j], wq_sem.at[j])
        hr = [(0, HA), (HA, H - HA)]
        k_cp = lambda j: pltpu.make_async_copy(k_hbm.at[pl.ds(*hr[j])], k_buf.at[pl.ds(*hr[j])], kv_sem.at[2 * j])
        v_cp = lambda j: pltpu.make_async_copy(v_hbm.at[pl.ds(*hr[j])], v_buf.at[pl.ds(*hr[j])], kv_sem.at[2 * j + 1])
        wr_cp = lambda: pltpu.make_async_copy(wr_hbm, wr_buf, misc_sem.at[0])
        wg_cp = lambda: pltpu.make_async_copy(wg_hbm, wg_buf, misc_sem.at[1])
        wu_cp = lambda: pltpu.make_async_copy(wu_hbm, wu_buf, misc_sem.at[2])
        wd_cp = lambda: pltpu.make_async_copy(wd_hbm, wd_buf, misc_sem.at[3])
        wo_cp = lambda: pltpu.make_async_copy(wo_hbm, wo_buf, misc_sem.at[4])

        cur = []
        def mark(name):
            if not P.get("PROF"): return
            if cur: cur.pop().__exit__(None, None, None)
            if name:
                cm = jax.named_scope(name); cm.__enter__(); cur.append(cm)
        mark("p0_wait_x0")
        cps = dict(x0=lambda: x_cp(0), x1=lambda: x_cp(1), x2=lambda: x_cp(2), x3=lambda: x_cp(3), wr=wr_cp,
                   q0=lambda: wq_cp(0), q1=lambda: wq_cp(1))
        def start(stage):
            for nm in P["DS"][stage].split():
                if nm == "qr":
                    for j in range(2, (NX + P['MB'] - 1) // NX + 1): wq_cp(j).start()
                else: cps[nm]().start()
        start(0)
        z_ref[0] = 0
        z_ref[1] = 0

        def store_q(j, g, i, q, BX=BX):
            q = (q * (DH ** -0.5 * LOG2E)).astype(bf16)
            r0 = pl.multiple_of(QB + (j * G + g) * (S // 2) + i * (BX // 2), 32)
            w_buf[pl.ds(r0, BX // 2), :] = pltpu.bitcast(q, f32)
            return q

        def qproj(j, i, after=None):
            xn = xn_buf[pl.ds(i * BX if isinstance(i, int) else pl.multiple_of(i * BX, BX), BX), :]
            if after is not None:
                head = jnp.where(lane > j + 1000, after, pltpu.bitcast(xn[:16, :128], f32))
                xn = jnp.concatenate([jnp.concatenate([pltpu.bitcast(head, bf16), xn[:16, 128:]], axis=1), xn[16:]], axis=0)
            q = jnp.dot(xn, wq_buf[j], preferred_element_type=f32)
            return [store_q(j, g, i, q[:, g * DH:(g + 1) * DH]) for g in range(G)]

        lane = lax.broadcasted_iota(i32, (8, 128), 1)
        sub = lax.broadcasted_iota(i32, (8, 128), 0)

        def layernorm(r0, n):
            x = x_buf[pl.ds(r0, n), :].astype(f32)
            m = jnp.sum(x, axis=-1, keepdims=True)
            yield
            m = m * (1.0 / D)
            mb = rb(m)
            xc = x - mb
            dm = m - mb
            var = jnp.sum(xc * xc, axis=-1, keepdims=True)
            if P["XB"]: xb = xc.astype(bf16)
            yield
            var = jnp.broadcast_to(var * (1.0 / D) - dm * dm, (n, 128))
            if P["DENSE"]:
                dense = var[:8]
                for t in range(1, n // 8):
                    dense = jnp.where(lane == t, var[t * 8:(t + 1) * 8], dense)
                inv = 1.0 / rb(jnp.sqrt(rb(rb(jnp.maximum(dense, 0.0)) + EPS)))
                inv = jnp.concatenate([jnp.broadcast_to(inv[:, t:t + 1], (8, 128)) for t in range(n // 8)], axis=0)
                yield
            else:
                inv = 1.0 / rb(jnp.sqrt(rb(rb(jnp.maximum(var, 0.0)) + EPS)))
            xr_ = xb.astype(f32) if P["XB"] else rb(xc)
            xn = jnp.concatenate([xr_[:, w * 128:(w + 1) * 128] * inv for w in range(D // 128)], axis=1).astype(bf16)
            xn_buf[pl.ds(r0, n), :] = xn
            out_buf[pl.ds(r0, n), :] = xn
            yield "stored"

        ln = dict(next=0, done=0, live=[])
        def layernorm_upto(row, avail):
            while ln["done"] < row:
                for gen in list(ln["live"]):
                    st_ = next(gen, "end")
                    if st_ == "stored": ln["done"] += LN
                    if st_ == "end": ln["live"].remove(gen)
                if ln["next"] < avail:
                    gen = layernorm(ln["next"], LN); next(gen)
                    ln["live"].append(gen); ln["next"] += LN

        x_cp(0).wait()
        start(1)
        wr_cp().wait()
        mark('p1_ln0')
        layernorm_upto(BX, BX)
        mark('p2_wait_wq0')
        wq_cp(0).wait()
        start(2)
        starts = [r[0] // BX for r in xr]
        for i in range(NX):
            if i + 1 in starts:
                n_ = starts.index(i + 1)
                mark(f'p3_wait_x{n_}')
                start(2 + n_)
                x_cp(n_).wait()
                avail = xr[n_][0] + xr[n_][1]
            if i + 1 in starts: mark(f'p3_q{i}')
            qproj(0, i)
            if i + 1 < NX:
                layernorm_upto((i + 2) * BX, avail)
        for gen in ln["live"]:
            for _ in gen: pass
        start(6)

        NJ, MB = P["NJ"], P["MB"]
        last = lambda jj: (NX + (jj + 1) * MB - 1) // NX
        RR = -(-S // (NJ * 256)) * 256
        row16 = lax.broadcasted_iota(i32, (16, D), 0)
        def top_k(rds):
            keys = []
            for t in range(NJ):
                r = rb(rds[t])
                r = jnp.where(r == 0.0, 0.0, r)
                b = lax.shift_right_logical(pltpu.bitcast(r, i32), 16)
                k16 = jnp.where(b >= 0x8000, 0xFFFF - b, b + 0x8000)
                k16 = jnp.where(r != r, 0, k16)
                tok = min(t * RR, S - RR) + lane * 8 + sub
                keys.append(pltpu.bitcast(jnp.where(lane < RR // 8, 0x20000000 + k16 * 2048 + (2047 - tok), 0), f32))
            ktop = jnp.zeros((8, 128), i32)
            x_sel = jnp.zeros((16, D), f32)
            for c in range(C):
                mx = functools.reduce(jnp.maximum, keys)
                mx = jnp.max(jnp.max(mx, axis=0, keepdims=True), axis=1, keepdims=True)
                mxb = jnp.broadcast_to(mx, (8, 128))
                keys = [jnp.where(kk == mxb, 0.0, kk) for kk in keys]
                mi = pltpu.bitcast(mxb, i32)
                ktop = jnp.where(sub == c, mi, ktop)
                idx = 2047 - (mi[0, 0] & 2047)
                base = pl.multiple_of(idx & -16, 16)
                blk = xn_buf[pl.ds(base, 16), :].astype(f32)
                rowv = jnp.sum(jnp.where(row16 == idx - base, blk, 0.0), axis=0, keepdims=True)
                x_sel = jnp.where(row16 == c, rowv, x_sel)
            return ktop, x_sel
        mark('p5_1b')
        def p1_body(jj, carry):
            for t in range(NJ):
                @pl.when(jj == t)
                def _():
                    js = list(range(last(t - 1) + 1, last(t) + 1))
                    for j in js[:-1]: wq_cp(j).wait()
                    if t == 0:
                        for j in range(last(0) + 1, NG): wq_cp(j).start()
                        wg_cp().start(); wu_cp().start(); wd_cp().start()
                    if t == 1:
                        k_cp(0).start(); v_cp(0).start()
                    wq_cp(js[-1]).wait()
            wr = wr_buf[...].astype(f32).reshape(1, D)
            r0 = pl.multiple_of(jnp.minimum(jj * RR, S - RR), 256)
            rd = jnp.zeros((8, 128), f32)
            RP = P["RP"]
            after = {}
            for p_ in range(RR // RP):
                r = jnp.sum(xn_buf[pl.ds(r0 + p_ * RP, RP), :].astype(f32) * wr, axis=-1, keepdims=True)
                r = jnp.broadcast_to(r, (RP, 128))
                for t in range(RP // 8):
                    rd = jnp.where(lane == p_ * (RP // 8) + t, r[t * 8:(t + 1) * 8], rd)
                after[1 + p_] = rd
            rds = [jnp.where(jnp.full((8, 128), jj) == t, rd, carry[0][t]) for t in range(NJ)]
            ktop, x_sel = top_k(rds)
            after[P['R0']] = functools.reduce(lax.add, [x_sel[:8, w * 128:(w + 1) * 128] for w in range(D // 128)])
            for n_ in range(MB):
                b_ = NX + jj * MB + n_
                qproj(lax.shift_right_logical(b_, NX.bit_length() - 1), b_ & (NX - 1), after.get(n_))
            return rds, ktop, x_sel
        zero = jnp.zeros((8, 128), f32)
        _, ktop, x_sel = lax.fori_loop(0, NJ, p1_body, ([zero] * NJ, jnp.zeros((8, 128), i32), jnp.zeros((16, D), f32)))
        x_sel = x_sel[:8]

        mark('p6_wait')
        for j in range(last(NJ - 1) + 1, NG): wq_cp(j).wait()
        wg_cp().wait(); wu_cp().wait(); wd_cp().wait()
        k_cp(0).wait(); v_cp(0).wait()
        mark('p7_1c')
        k16 = lax.shift_right_logical(ktop - 0x20000000, 11)
        b = jnp.where(k16 >= 0x8000, k16 - 0x8000, 0xFFFF - k16)
        r_sel = pltpu.bitcast(lax.shift_left(b, 16), f32)[:, :1]
        xs = x_sel.astype(bf16)
        KT = D // 128
        acc = {}
        def accum(key, d):
            acc[key] = acc[key] + d if key in acc else d
        BC = P["BC"]
        def q_tile(j, i, g, k):
            accum((j, i, g), jnp.dot(xn_buf[pl.ds(i * BC, BC), pl.ds(k * 128, 128)], wq_buf[j, pl.ds(k * 128, 128), pl.ds(g * DH, DH)], preferred_element_type=f32))
            if k == KT - 1:
                store_q(j, g, i, acc.pop((j, i, g)), BC)
        fr = [(f0, min(128, F - f0)) for f0 in range(0, F, 128)]
        def up_tile(name, w, f, k):
            accum((name, f), lax.dot_general(xs[:, k * 128:(k + 1) * 128], w[pl.ds(*fr[f]), pl.ds(k * 128, 128)], NT, preferred_element_type=f32))
        def down_tile(f, n):
            if n == 0:
                a = rb(acc.pop(("g", f)))
                acc["h"] = (rb(a * sigmoid(a)) * rb(acc.pop(("u", f)))).astype(bf16)
            accum(("y", n), jnp.dot(acc["h"], wd_buf[pl.ds(*fr[f]), pl.ds(n * 128, 128)], preferred_element_type=f32))
        part = functools.partial
        q_tiles = [part(q_tile, j, i, g, k) for j in range(NG) for i in range(S // BC) if j * S + i * BC >= (NX + NJ * MB) * BX for g in range(G) for k in range(KT)]
        f_tiles = [part(up_tile, nm, w, f, k) for f in range(len(fr)) for nm, w in (("g", wg_buf), ("u", wu_buf)) for k in range(KT)]
        f_tiles += [None] * (4 * P["FG"])
        f_tiles += [part(down_tile, f, n) for f in range(len(fr)) for n in range(KT)]
        for rnd in range(len(q_tiles) // 4):
            for fn_ in q_tiles[4 * rnd:4 * rnd + 4]:
                fn_()
            if rnd >= P["F0"]:
                for fn_ in f_tiles[:4]:
                    if fn_ is not None: fn_()
                f_tiles = f_tiles[4:]
        assert not f_tiles
        y = rb(jnp.concatenate([acc.pop(("y", n)) for n in range(KT)], axis=1))
        z = rb(x_sel + rb(y * rb(sigmoid(r_sel))))
        for c in range(C):
            idx = 2047 - (ktop[c, 0] & 2047)
            base = pl.multiple_of(idx & -16, 16)
            blk = out_buf[pl.ds(base, 16), :].astype(f32)
            out_buf[pl.ds(base, 16), :] = jnp.where(row16 == idx - base, z[c:c + 1, :], blk).astype(bf16)

        mark('p8_att')
        NIT, N0 = divmod(H * NB, NU)
        GPI, G0 = divmod(S // 16, NIT)
        opaque = lambda i: pl.multiple_of(z_ref[i], 32)
        if N0 and "a" not in P["SKIP"]:
            attention_body(0, N0, 0, G0, opaque(0), opaque(1), w_buf, s_bufs, a_bufs, k_buf, v_buf, out_buf, P)
        TA = (HA * NB - N0) // NU
        z0, z1 = opaque(0), opaque(1)
        def att_body(t, _):
            @pl.when(t == 0)
            def _():
                k_cp(1).start(); v_cp(1).start(); wo_cp().start()
            @pl.when(t == TA)
            def _():
                k_cp(1).wait(); v_cp(1).wait(); wo_cp().wait()
            if "a" not in P["SKIP"]:
                attention_body(N0 + t * NU, NU, G0 + t * GPI, GPI, z0, z1, w_buf, s_bufs, a_bufs, k_buf, v_buf, out_buf, P)
        lax.fori_loop(0, NIT, att_body, None)

        out_cp = lambda i: pltpu.make_async_copy(out_buf.at[pl.ds(i * BO, BO)], out_hbm.at[pl.ds(i * BO, BO)], out_sem.at[i])
        mark('p9_out')
        UO = P["UO"]
        def p3_body(ii, _):
            for u in range(UO):
                i = ii * UO + u
                r0 = pl.multiple_of(i * BO, BO)
                packed = lambda base, n: jnp.concatenate([pltpu.bitcast(w_buf[pl.ds(pl.multiple_of(base + h * (S // 2) + i * (BO // 2), 32), BO // 2), :], bf16) for h in range(n)], axis=-1)
                s = jnp.dot(packed(QB, H), wo_buf[...], preferred_element_type=f32)
                out_buf[pl.ds(r0, BO), :] = (x_buf[pl.ds(r0, BO), :].astype(f32) + s * packed(GB, D // 128).astype(f32)).astype(bf16)
                out_cp(i).start()
        if UO == NO:
            p3_body(0, None)
        else:
            lax.fori_loop(0, NO // UO, p3_body, None)
        mark('pa_wait_out')
        for i in range(NO):
            out_cp(i).wait()
        mark(None)

    @jax.jit
    def fn(A_x, A_k_cache, A_v_cache, A_wq, A_wo, B_x, B_w_r, B_w_gate, B_w_up, B_w_down):
        any_spec = pl.BlockSpec(memory_space=pl.ANY)
        s_shape = pltpu.VMEM((L * BQ * (KC // 128) + 32, 128), f32)
        out = pl.pallas_call(
            kernel,
            in_specs=[any_spec] * 9,
            out_specs=any_spec,
            out_shape=jax.ShapeDtypeStruct((S, D), bf16),
            scratch_shapes=[
                pltpu.VMEM((S, D), bf16), pltpu.VMEM((S, D), bf16),
                pltpu.VMEM((GB + D // 128 * S // 2, DH), f32),
                pltpu.VMEM((H, SK, DH), bf16), pltpu.VMEM((H, SK, DH), bf16),
                pltpu.VMEM((NG, D, G * DH), bf16), pltpu.VMEM((H * DH, D), bf16),
                pltpu.VMEM((F, D), bf16), pltpu.VMEM((F, D), bf16), pltpu.VMEM((F, D), bf16),
                pltpu.VMEM((S, D), bf16), pltpu.SMEM((2,), i32),
                pltpu.SemaphoreType.DMA((len(P['XA']) - 1,)), pltpu.SemaphoreType.DMA((NG,)), pltpu.SemaphoreType.DMA((4,)),
                pltpu.SemaphoreType.DMA((5,)), pltpu.SemaphoreType.DMA((NO,)),
            ] + [s_shape] * P['NSB'] + [pltpu.VMEM((3 * BQ, 128), f32)] * P['NAB'] + [pltpu.VMEM((D,), bf16)],
            compiler_params=pltpu.CompilerParams(vmem_limit_bytes=120 * 1024 * 1024, flags=flags),
            name="fused_kernel",
        )(A_x.reshape(S, D), A_k_cache.reshape(H, SK, DH), A_v_cache.reshape(H, SK, DH), A_wq, A_wo,
          B_w_r, B_w_gate.T, B_w_up.T, B_w_down)
        return out.reshape(1, S, D)
    return fn


_impl = make()


@jax.jit
def pallas_recurrent_scan__mha_block_cached__moe_arch_mod__prompt_kernel(
    A_x, A_k_cache, A_v_cache, A_wq, A_wo, B_x, B_w_r, B_w_gate, B_w_up, B_w_down
):
    return _impl(A_x, A_k_cache, A_v_cache, A_wq, A_wo, B_x, B_w_r, B_w_gate, B_w_up, B_w_down)
```

```python
import functools
import numpy as np
import jax
import jax.numpy as jnp
from jax import lax
import jax.experimental.pallas as pl
import jax.experimental.pallas.tpu as pltpu

S, D, H, DH, SK, F, C = 2048, 640, 32, 128, 2048, 1728, 8
LOG2E = 1.4426950408889634
EPS = float(np.asarray(1e-5, dtype=jnp.bfloat16))
f32, bf16, i32 = jnp.float32, jnp.bfloat16, jnp.int32
NT = (((1,), (1,)), ((), ()))


def rb(x):
    return x.astype(bf16).astype(f32)


def sigmoid(x):
    return 1.0 / (1.0 + jnp.exp2(x * (-LOG2E)))


def attention_body(grp, blk0, z0, z1, w_buf, s_bufs, a_bufs, k_buf, v_buf, wo_buf, x_buf, y_buf, out_buf, out_start, next_head, P):
    BQ, KC, DL = P["BQ"], P["KC"], P["DL"]
    LA, LS, PD, LC, XD, FD, QA = (P[k] for k in "LA LS PD LC XD FD QA".split())
    NB = S // BQ; R = BQ // 16; NC = SK // KC; W = KC // 128; L = NC + DL
    def s_loc(g, w, r):
        return (g // L) % len(s_bufs), (((g % L) * R + r) * W + w) * 16
    def ld_s(g, w, r):
        par, o = s_loc(g, w, r)
        return s_bufs[par][pl.ds(z1 + o, 16), :]
    def st_s(g, w, r, v):
        par, o = s_loc(g, w, r)
        s_bufs[par][pl.ds(z0 + o, 16), :] = v
    def st_tok(g, v):
        s_bufs[s_loc(g, 0, 0)[0]][pl.ds(z0 + L * R * W * 16, 8), :] = v
    MX, LP, OA = 0, BQ, 2 * BQ
    def ld(a, off, r): return a_bufs[a % len(a_bufs)][pl.ds(z1 + (off + 16 * r), 16), :]
    def st(a, off, r, v): a_bufs[a % len(a_bufs)][pl.ds(z0 + (off + 16 * r), 16), :] = v
    G, M = P["G"], P["M"]; NU = G * M; KT = D // 128
    heads = [grp * G + u % G for u in range(NU)]
    qbase = pl.multiple_of(P["QB"] + grp * (G * S // 2) + blk0 * (BQ // 2), 32)
    qrow = [qbase + (u % G) * (S // 2) + (u // G) * (BQ // 2) for u in range(NU)]
    row0 = pl.multiple_of(blk0 * BQ, BQ); row2 = pl.multiple_of(blk0 * (BQ // 2), BQ // 2)
    first = lax.broadcasted_iota(i32, (16, 128), 0) + grp * 16 < 16
    dots = []; pend = []
    for g in range(NU * NC + L):
        if g < NU * NC: dots.append(("qk", g))
        if g - L >= 0:
            dots.append(("pv", g - L))
            b_, rem = divmod(g - L - P["OL"] + 1, G * NC)
            if rem == 0 and 1 <= b_ <= M - 2: pend += [("op", (b_ - 1) * KT + n) for n in range(KT)]
            dots += pend[:P["OP"]]; pend = pend[P["OP"]:]
    dots += pend + [("op", n) for n in range((M - 2) * KT, M * KT)]
    ev = []; val = {}
    def add(slot, prio, fn): ev.append((slot, prio, len(ev), fn))
    def res(i):
        if ("res", i) not in val:
            kind, g = dots[i]; a, c = divmod(g, NC); h = heads[a]
            if kind == "op":
                o = jnp.concatenate([pltpu.bitcast(jnp.concatenate([val.pop(("ol", i, r, u)) for r in range(R)], axis=0), bf16) for u in range(G)], axis=1)
                val["res", i] = jnp.dot(o, wo_buf[grp, :, pl.ds(g % KT * 128, 128)], preferred_element_type=f32)
            elif kind == "qk":
                q = pltpu.bitcast(jnp.concatenate([val.pop(("q", i, r)) for r in range(R)], axis=0), bf16)
                if i == 0 and P["KT"]:
                    kt = jnp.concatenate([pltpu.bitcast(w_buf[pl.ds(32 + 64 * w, 64), :], bf16) for w in range(W)], axis=1)
                    val["res", i] = jnp.dot(q, kt, preferred_element_type=f32)
                else:
                    val["res", i] = lax.dot_general(q, k_buf[h, pl.ds(c * KC, KC), :], NT, preferred_element_type=f32)
            else:
                p = jnp.concatenate([val.pop(("p", i, r)) for r in range(R)], axis=0).astype(bf16)
                val["res", i] = jnp.dot(p, v_buf[h, pl.ds(c * KC, KC), :], preferred_element_type=f32)
        return val["res", i]
    for i, (kind, g) in enumerate(dots):
        a, c = divmod(g, NC)
        la = P["LAL"] if i == len(dots) - 1 else LA
        for r in range(R):
            j = i * R + r
            if kind == "op":
                b_, n = divmod(g, KT)
                def l_o(i=i, b_=b_, r=r):
                    if "tok" in val and r % P["QO"] == 0: w_buf[pl.ds(z0, 8), :] = val["tok"]
                    for u in range(G): val["ol", i, r, u] = w_buf[pl.ds(z1 + qrow[b_ * G + u] + 8 * r, 8), :]
                add(min(j - QA, i * R + PD - 1), 1, l_o)
                def l_y(i=i, b_=b_, n=n, r=r):
                    y = y_buf[pl.ds(z1 + row0 + (n * S + b_ * BQ + 16 * r), 16), :]
                    if r % P["XT"] == 0 and 'o' not in P['SKIP']: x_buf[pl.ds(z0 + 2 * S, 16), pl.ds(0, 128)] = pltpu.bitcast(val["tok"], bf16)
                    x, xn = (x_buf[pl.ds(z1 + row0 + (k * S + b_ * BQ + 16 * r), 16), pl.ds(n * 128, 128)].astype(f32) for k in range(2))
                    val["y", i, r] = (jnp.where(first, 0.0, y), x, xn * sigmoid(xn))
                add(j + PD - P["LY"], 1, l_y)
                def s_y(i=i, b_=b_, n=n, r=r):
                    y, x, gate = val.pop(("y", i, r))
                    y = y + res(i)[16 * r:16 * r + 16]
                    val["tok"] = y[:8]
                    y_buf[pl.ds(z0 + row0 + (n * S + b_ * BQ + 16 * r), 16), :] = y
                    out = x + y * gate
                    val['out', i, r] = out[:8] + out[8:]
                    if 'f' in P['SKIP']: y_buf[pl.ds(z0 + KT * S + 8, 8), :] = pltpu.bitcast(out.astype(bf16), f32)
                    elif 'o' not in P['SKIP']: out_buf[pl.ds(row0 + b_ * BQ + 16 * r, 16), pl.ds(n * 128, 128)] = out.astype(bf16)
                    if n == KT - 1 and r == R - 1 and b_ + 1 in P['OD']: out_start(blk0, P['OD'].index(b_ + 1))
                add(j + PD, 0, s_y)
                if P["OT"]:
                    def s_ot(i=i, r=r): y_buf[pl.ds(z0 + KT * S, 8), :] = val.pop(("out", i, r))
                    add(j + PD + P["OT"], 0, s_ot)
            elif kind == "qk":
                def l_q(i=i, a=a, r=r):
                    if "tok" in val and r % P["QT"] == 0: w_buf[pl.ds(z0, 8), :] = val["tok"]
                    val["q", i, r] = w_buf[pl.ds(z1 + qrow[a] + 8 * r, 8), :]
                add(min(j - QA, i * R + PD - 1), 1, l_q)
                if c > 0:
                    def l_acc(a=a, r=r): val["mx", a, r] = ld(a, MX, r)
                    add(j + PD - LC, 1, l_acc)
                def s_res(i=i, g=g, a=a, c=c, r=r):
                    s = res(i)[16 * r:16 * r + 16]
                    tiles = [s[:, w * 128:(w + 1) * 128] for w in range(W)]
                    for w in range(W): st_s(g, w, r, tiles[w])
                    val["tok"] = tiles[W - 1][:8]
                    mx = functools.reduce(jnp.maximum, tiles)
                    if c > 0: mx = jnp.maximum(mx, val.pop(("mx", a, r)))
                    if c == NC - 1:
                        val["m", a, r] = jnp.broadcast_to(jnp.max(mx, axis=-1, keepdims=True), (16, 128))
                    else: st(a, MX, r, mx)
                add(j + PD, 0, s_res)
                if c == NC - 1:
                    def s_m(a=a, r=r): st(a, MX, r, val.pop(("m", a, r)))
                    add(j + PD + XD, 0, s_m)
            else:
                def l_lhs(i=i, g=g, a=a, c=c, r=r):
                    m = ld(a, MX, r)
                    if "tok" in val: st_tok(g, val["tok"])
                    ps = [jnp.exp2(ld_s(g, w, r) - m) for w in range(W)]
                    lp = functools.reduce(lax.add, ps)
                    if c > 0: lp = lp + ld(a, LP, r)
                    val["lp", i, r] = lp
                    val["p", i, r] = jnp.concatenate(ps, axis=1)
                add(min(j - la, i * R + PD - 1), 1, l_lhs)
                if c < NC - 1:
                    def s_lp(i=i, a=a, r=r): st(a, LP, r, val.pop(("lp", i, r)))
                    add(j - la + LS, 0, s_lp)
                if c > 0:
                    def l_acc(i=i, a=a, r=r): val["o", i, r] = ld(a, OA, r)
                    add(j + PD - LC, 1, l_acc)
                if c < NC - 1:
                    def s_res(i=i, a=a, c=c, r=r):
                        d = res(i)[16 * r:16 * r + 16]
                        if c > 0: d = d + val.pop(("o", i, r))
                        val["tok"] = d[:8]
                        st(a, OA, r, d)
                    add(j + PD, 0, s_res)
                else:
                    def s_res(i=i, r=r):
                        d = res(i)[16 * r:16 * r + 16] + val.pop(("o", i, r))
                        val["tok"] = d[:8]
                        val["of", i, r] = d
                    add(j + PD, 0, s_res)
                    def s_fin(i=i, a=a, r=r):
                        l = jnp.sum(val.pop(("lp", i, r)), axis=-1, keepdims=True)
                        r0 = pl.reciprocal(l, approx=True)
                        rl = r0 * (2.0 - l * r0)
                        ob = pltpu.bitcast((val.pop(("of", i, r)) * rl).astype(bf16), f32)
                        w_buf[pl.ds(z0 + qrow[a] + 8 * r, 8), :] = ob
                    add(max(j - la + LS + XD + FD, j + PD), 0, s_fin)
    for w in range(W if P["KT"] else 0):
        def s_kt(w=w): w_buf[pl.ds(z0 + 32 + 64 * w, 64), :] = pltpu.bitcast(k_buf[next_head, pl.ds(w * 128, 128), :].T, f32)
        add(P["KT"] + 2 * w, 0, s_kt)
    ev.sort(key=lambda e: e[:3])
    for e in ev: e[3]()


def make(flags=None, **kw):
    P = dict(BQ=128, NU=39, KC=512, DL=2, LA=4, LAL=4, LS=3, PD=8, LC=2, XD=9, FD=2, QA=2, BX=256, G=4, BO=256, HA=8, TW=0, KT=0, SKIP="",
             DS=('x0 wr q0 x1', 'x2', 'x3', '', 'x4', '', 'q1 qr'), BC=256, M=8, OT=0, OD=(0, 1, 2, 3, 4, 5, 6, 7, 8), OL=2, OP=5, QO=1, LY=3, XT=2, NJ=2, RA=1, RS=1, MB=20, TF=0, RP=32, R0=16, NSB=11, NAB=11, QT=8, GS=50, GD=2, UO=2, UJ=2, F0=0, FG=8, FS=(5, 3), XB=1, DENSE=1, LN=64, XA=(0, 1, 2, 4, 6, 8))
    P.update(kw)
    BQ, NU, KC, BX, G, BO, HA = (P[k] for k in "BQ NU KC BX G BO HA".split())
    P["QB"] = QB = 32 + KC // 2
    P["GB"] = GB = QB + H * S // 2
    NB = S // BQ; NX = S // BX; NG = H // G; NO = S // BO
    L = SK // KC + P["DL"]

    def kernel(x_hbm, k_hbm, v_hbm, wq_hbm, wo_hbm, wr_hbm, wg_hbm, wu_hbm, wd_hbm, out_hbm,
               x_buf, xn_buf, w_buf, y_buf, k_buf, v_buf, wq_buf, wo_buf, wg_buf, wu_buf, wd_buf, out_buf, z_ref,
               x_sem, wq_sem, kv_sem, misc_sem, out_sem, *bufs):
        s_bufs, a_bufs, wr_buf = bufs[:P['NSB']], bufs[P['NSB']:-1], bufs[-1]
        KT = D // 128; XA = P["XA"]; LN = P["LN"]
        xr = [(a_ * BX, (b_ - a_) * BX) for a_, b_ in zip(XA[:-1], XA[1:])]
        x_cp = lambda i: pltpu.make_async_copy(x_hbm.at[pl.ds(*xr[i])], x_buf.at[pl.ds(*xr[i])], x_sem.at[i])
        wq_cp = lambda j: pltpu.make_async_copy(wq_hbm.at[:, pl.ds(j * G * DH, G * DH)], wq_buf.at[j], wq_sem.at[j])
        hr = [(0, HA), (HA, H - HA)]
        k_cp = lambda j: pltpu.make_async_copy(k_hbm.at[pl.ds(*hr[j])], k_buf.at[pl.ds(*hr[j])], kv_sem.at[2 * j])
        v_cp = lambda j: pltpu.make_async_copy(v_hbm.at[pl.ds(*hr[j])], v_buf.at[pl.ds(*hr[j])], kv_sem.at[2 * j + 1])
        wr_cp = lambda: pltpu.make_async_copy(wr_hbm, wr_buf, misc_sem.at[0])
        wg_cp = lambda: pltpu.make_async_copy(wg_hbm, wg_buf, misc_sem.at[1])
        wu_cp = lambda: pltpu.make_async_copy(wu_hbm, wu_buf, misc_sem.at[2])
        wd_cp = lambda: pltpu.make_async_copy(wd_hbm, wd_buf, misc_sem.at[3])
        wo_cp = lambda: pltpu.make_async_copy(wo_hbm, wo_buf, misc_sem.at[4])

        cur = []
        def mark(name):
            if not P.get("PROF"): return
            if cur: cur.pop().__exit__(None, None, None)
            if name:
                cm = jax.named_scope(name); cm.__enter__(); cur.append(cm)
        mark("p0_wait_x0")
        cps = dict(x0=lambda: x_cp(0), x1=lambda: x_cp(1), x2=lambda: x_cp(2), x3=lambda: x_cp(3), x4=lambda: x_cp(4), wr=wr_cp,
                   q0=lambda: wq_cp(0), q1=lambda: wq_cp(1))
        def start(stage):
            for nm in P["DS"][stage].split():
                if nm == "qr":
                    for j in range(2, (NX + P['MB'] - 1) // NX + 1): wq_cp(j).start()
                else: cps[nm]().start()
        start(0)
        z_ref[0] = 0
        z_ref[1] = 0

        def store_q(j, g, i, q, BX=BX):
            q = (q * (DH ** -0.5 * LOG2E)).astype(bf16)
            r0 = pl.multiple_of(QB + (j * G + g) * (S // 2) + i * (BX // 2), 32)
            w_buf[pl.ds(r0, BX // 2), :] = pltpu.bitcast(q, f32)
            return q

        def qproj(j, i, after=None):
            xn = xn_buf[pl.ds(i * BX if isinstance(i, int) else pl.multiple_of(i * BX, BX), BX), :]
            if after is not None:
                head = jnp.where(lane > j + 1000, after, pltpu.bitcast(xn[:16, :128], f32))
                xn = jnp.concatenate([jnp.concatenate([pltpu.bitcast(head, bf16), xn[:16, 128:]], axis=1), xn[16:]], axis=0)
            q = jnp.dot(xn, wq_buf[j], preferred_element_type=f32)
            return [store_q(j, g, i, q[:, g * DH:(g + 1) * DH]) for g in range(G)]

        lane = lax.broadcasted_iota(i32, (8, 128), 1)
        sub = lax.broadcasted_iota(i32, (8, 128), 0)

        def layernorm(r0, n):
            x = x_buf[pl.ds(r0, n), :].astype(f32)
            m = jnp.sum(x, axis=-1, keepdims=True)
            yield
            m = m * (1.0 / D)
            mb = rb(m)
            xc = x - mb
            dm = m - mb
            var = jnp.sum(xc * xc, axis=-1, keepdims=True)
            if P["XB"]: xb = xc.astype(bf16)
            yield
            var = jnp.broadcast_to(var * (1.0 / D) - dm * dm, (n, 128))
            if P["DENSE"]:
                dense = var[:8]
                for t in range(1, n // 8):
                    dense = jnp.where(lane == t, var[t * 8:(t + 1) * 8], dense)
                inv = 1.0 / rb(jnp.sqrt(rb(rb(jnp.maximum(dense, 0.0)) + EPS)))
                inv = jnp.concatenate([jnp.broadcast_to(inv[:, t:t + 1], (8, 128)) for t in range(n // 8)], axis=0)
                yield
            else:
                inv = 1.0 / rb(jnp.sqrt(rb(rb(jnp.maximum(var, 0.0)) + EPS)))
            xr_ = xb.astype(f32) if P["XB"] else rb(xc)
            xn = jnp.concatenate([xr_[:, w * 128:(w + 1) * 128] * inv for w in range(D // 128)], axis=1).astype(bf16)
            xn_buf[pl.ds(r0, n), :] = xn
            x_buf[pl.ds(S + r0, n), :] = xn
            yield "stored"

        ln = dict(next=0, done=0, live=[])
        def layernorm_upto(row, avail):
            while ln["done"] < row:
                for gen in list(ln["live"]):
                    st_ = next(gen, "end")
                    if st_ == "stored": ln["done"] += LN
                    if st_ == "end": ln["live"].remove(gen)
                if ln["next"] < avail:
                    gen = layernorm(ln["next"], LN); next(gen)
                    ln["live"].append(gen); ln["next"] += LN

        x_cp(0).wait()
        start(1)
        wr_cp().wait()
        mark('p1_ln0')
        layernorm_upto(BX, BX)
        mark('p2_wait_wq0')
        wq_cp(0).wait()
        start(2)
        starts = [r[0] // BX for r in xr]
        for i in range(NX):
            if i + 1 in starts:
                n_ = starts.index(i + 1)
                mark(f'p3_wait_x{n_}')
                start(2 + n_)
                x_cp(n_).wait()
                avail = xr[n_][0] + xr[n_][1]
            if i + 1 in starts: mark(f'p3_q{i}')
            qproj(0, i)
            if i + 1 < NX:
                layernorm_upto((i + 2) * BX, avail)
        for gen in ln["live"]:
            for _ in gen: pass

        NJ, MB = P["NJ"], P["MB"]
        last = lambda jj: (NX + (jj + 1) * MB - 1) // NX
        RR = -(-S // (NJ * 256)) * 256
        row16 = lax.broadcasted_iota(i32, (16, D), 0)
        def top_k(rds):
            keys = []
            for t in range(NJ):
                r = rb(rds[t])
                r = jnp.where(r == 0.0, 0.0, r)
                b = lax.shift_right_logical(pltpu.bitcast(r, i32), 16)
                k16 = jnp.where(b >= 0x8000, 0xFFFF - b, b + 0x8000)
                k16 = jnp.where(r != r, 0, k16)
                tok = min(t * RR, S - RR) + lane * 8 + sub
                keys.append(pltpu.bitcast(jnp.where(lane < RR // 8, 0x20000000 + k16 * 2048 + (2047 - tok), 0), f32))
            ktop = jnp.zeros((8, 128), i32)
            x_sel = jnp.zeros((16, D), f32)
            for c in range(C):
                mx = functools.reduce(jnp.maximum, keys)
                mx = jnp.max(jnp.max(mx, axis=0, keepdims=True), axis=1, keepdims=True)
                mxb = jnp.broadcast_to(mx, (8, 128))
                keys = [jnp.where(kk == mxb, 0.0, kk) for kk in keys]
                mi = pltpu.bitcast(mxb, i32)
                ktop = jnp.where(sub == c, mi, ktop)
                idx = 2047 - (mi[0, 0] & 2047)
                base = pl.multiple_of(idx & -16, 16)
                blk = xn_buf[pl.ds(base, 16), :].astype(f32)
                rowv = jnp.sum(jnp.where(row16 == idx - base, blk, 0.0), axis=0, keepdims=True)
                x_sel = jnp.where(row16 == c, rowv, x_sel)
            return ktop, x_sel
        mark('p5_1b')
        def p1_body(jj, carry):
            for t in range(NJ):
                @pl.when(jj == t)
                def _():
                    js = list(range(last(t - 1) + 1, last(t) + 1))
                    for j in js[:-1]: wq_cp(j).wait()
                    if t == 0:
                        for j in range(last(0) + 1, NG): wq_cp(j).start()
                        wg_cp().start(); wu_cp().start(); wd_cp().start()
                    if t == P['TW']: wo_cp().start()
                    if t == 1:
                        k_cp(0).start(); v_cp(0).start()
                    wq_cp(js[-1]).wait()
            wr = wr_buf[...].astype(f32).reshape(1, D)
            r0 = pl.multiple_of(jnp.minimum(jj * RR, S - RR), 256)
            rd = jnp.zeros((8, 128), f32)
            RP = P["RP"]
            never = lax.broadcasted_iota(i32, (8, 128), 1) > jj + 1000
            after = None
            for n_ in range(MB):
                b_ = NX + jj * MB + n_
                qs = qproj(lax.shift_right_logical(b_, NX.bit_length() - 1), b_ & (NX - 1), after if n_ == P["R0"] else None)
                for g in range(G if n_ * G * RP < RR else 0):
                    tok = pltpu.bitcast(qs[g][:16], f32)
                    for t in range((n_ * G + g) * RP // 16, (n_ * G + g + 1) * RP // 16):
                        r = 0.0
                        for w in range(KT):
                            xb = pltpu.bitcast(xn_buf[pl.ds(r0 + t * 16, 16), pl.ds(w * 128, 128)], f32)
                            d_ = pltpu.bitcast(jnp.where(never, tok, xb), bf16).astype(f32) * wr[:, w * 128:(w + 1) * 128]
                            r = d_ if w == 0 else r + d_
                        r = jnp.broadcast_to(jnp.sum(r, axis=-1, keepdims=True), (16, 128))
                        rd = jnp.where(lane == 2 * t, r[:8], jnp.where(lane == 2 * t + 1, r[8:], rd))
                if (n_ + 1) * G * RP == RR:
                    rds = [jnp.where(jnp.full((8, 128), jj) == t, rd, carry[0][t]) for t in range(NJ)]
                    ktop, x_sel = top_k(rds)
                    after = functools.reduce(lax.add, [x_sel[:8, w * 128:(w + 1) * 128] for w in range(KT)])
            return rds, ktop, x_sel
        zero = jnp.zeros((8, 128), f32)
        _, ktop, x_sel = lax.fori_loop(0, NJ, p1_body, ([zero] * NJ, jnp.zeros((8, 128), i32), jnp.zeros((16, D), f32)))
        x_sel = x_sel[:8]

        mark('p6_wait')
        for j in range(last(NJ - 1) + 1, NG): wq_cp(j).wait()
        wg_cp().wait(); wu_cp().wait(); wd_cp().wait()
        k_cp(0).wait(); v_cp(0).wait(); wo_cp().wait()
        mark('p7_1c')
        k16 = lax.shift_right_logical(ktop - 0x20000000, 11)
        b = jnp.where(k16 >= 0x8000, k16 - 0x8000, 0xFFFF - k16)
        r_sel = pltpu.bitcast(lax.shift_left(b, 16), f32)[:, :1]
        xs = x_sel.astype(bf16)
        acc = {}
        def accum(key, d):
            acc[key] = acc[key] + d if key in acc else d
        BC = P["BC"]
        def q_tile(j, i, g, k):
            accum((j, i, g), jnp.dot(xn_buf[pl.ds(i * BC, BC), pl.ds(k * 128, 128)], wq_buf[j, pl.ds(k * 128, 128), pl.ds(g * DH, DH)], preferred_element_type=f32))
            if k == KT - 1:
                store_q(j, g, i, acc.pop((j, i, g)), BC)
        fr = [(f0, min(128, F - f0)) for f0 in range(0, F, 128)]
        def up_tile(name, w, f, k):
            accum((name, f), lax.dot_general(xs[:, k * 128:(k + 1) * 128], w[pl.ds(*fr[f]), pl.ds(k * 128, 128)], NT, preferred_element_type=f32))
        def down_tile(f, n):
            if n == 0:
                a = rb(acc.pop(("g", f)))
                acc["h"] = (rb(a * sigmoid(a)) * rb(acc.pop(("u", f)))).astype(bf16)
            accum(("y", n), jnp.dot(acc["h"], wd_buf[pl.ds(*fr[f]), pl.ds(n * 128, 128)], preferred_element_type=f32))
        part = functools.partial
        q_tiles = [part(q_tile, j, i, g, k) for j in range(NG) for i in range(S // BC) if j * S + i * BC >= (NX + NJ * MB) * BX for g in range(G) for k in range(KT)]
        f_tiles = [part(up_tile, nm, w, f, k) for f in range(len(fr)) for nm, w in (("g", wg_buf), ("u", wu_buf)) for k in range(KT)]
        f_tiles += [None] * (4 * P["FG"])
        f_tiles += [part(down_tile, f, n) for f in range(len(fr)) for n in range(KT)]
        for rnd in range(len(q_tiles) // 4):
            for fn_ in q_tiles[4 * rnd:4 * rnd + 4]:
                fn_()
            if rnd >= P["F0"] and rnd % P['FS'][0] not in P['FS'][1:]:
                for fn_ in f_tiles[:4]:
                    if fn_ is not None: fn_()
                f_tiles = f_tiles[4:]
        assert not f_tiles
        y = rb(jnp.concatenate([acc.pop(("y", n)) for n in range(KT)], axis=1))
        z = rb(x_sel + rb(y * rb(sigmoid(r_sel))))
        for c in range(C):
            idx = 2047 - (ktop[c, 0] & 2047)
            at = pl.ds(S + pl.multiple_of(idx & -16, 16), 16)
            x_buf[at, :] = jnp.where(row16 == (idx & 15), z[c:c + 1, :], x_buf[at, :].astype(f32)).astype(bf16)

        k_cp(1).start(); v_cp(1).start()
        if P['KT']:
            for w in range(KC // 128):
                w_buf[pl.ds(32 + 64 * w, 64), :] = pltpu.bitcast(k_buf[0, pl.ds(w * 128, 128), :].T, f32)
        mark('p8_att')
        M = P["M"]; PG = NB // M
        OD = P["OD"]
        def out_cp(blk0, k):
            rows = pl.ds((blk0 + OD[k - 1]) * BQ, (OD[k] - OD[k - 1]) * BQ)
            return pltpu.make_async_copy(out_buf.at[rows], out_hbm.at[rows], out_sem.at[blk0 + k - 1])
        z0, z1 = (pl.multiple_of(z_ref[i], 32) for i in range(2))
        def att_body(t, _):
            @pl.when(t == HA // G * PG - 1)
            def _():
                if 'k' not in P['SKIP']: k_cp(1).wait(); v_cp(1).wait()
            grp = lax.shift_right_logical(t, PG.bit_length() - 1)
            def out_start(blk0, k):
                @pl.when(grp == NG - 1)
                def _():
                    out_cp(blk0, k).start()
            attention_body(grp, (t & (PG - 1)) * M, z0, z1, w_buf, s_bufs, a_bufs, k_buf, v_buf, wo_buf, x_buf, y_buf, out_buf, out_start, jnp.minimum(lax.shift_right_logical(t + 1, PG.bit_length() - 1), NG - 1) * G, P)
        lax.fori_loop(P.get('T0', 0), NG * PG, att_body, None)
        mark('pa_wait_out')
        for blk0 in range(0, NB, M):
            for k in range(1, len(OD)):
                out_cp(blk0, k).wait()
        mark(None)

    @jax.jit
    def fn(A_x, A_k_cache, A_v_cache, A_wq, A_wo, B_x, B_w_r, B_w_gate, B_w_up, B_w_down):
        any_spec = pl.BlockSpec(memory_space=pl.ANY)
        s_shape = pltpu.VMEM((L * BQ * (KC // 128) + 32, 128), f32)
        out = pl.pallas_call(
            kernel,
            in_specs=[any_spec] * 9,
            out_specs=any_spec,
            out_shape=jax.ShapeDtypeStruct((S, D), bf16),
            scratch_shapes=[
                pltpu.VMEM((2 * S + 64, D), bf16), pltpu.VMEM((S, D), bf16),
                pltpu.VMEM((GB, DH), f32), pltpu.VMEM((D // 128 * S + 32, DH), f32),
                pltpu.VMEM((H, SK, DH), bf16), pltpu.VMEM((H, SK, DH), bf16),
                pltpu.VMEM((NG, D, G * DH), bf16), pltpu.VMEM((NG, G * DH, D), bf16),
                pltpu.VMEM((F, D), bf16), pltpu.VMEM((F, D), bf16), pltpu.VMEM((F, D), bf16),
                pltpu.VMEM((S, D), bf16), pltpu.SMEM((2,), i32),
                pltpu.SemaphoreType.DMA((len(P['XA']) - 1,)), pltpu.SemaphoreType.DMA((NG,)), pltpu.SemaphoreType.DMA((4,)),
                pltpu.SemaphoreType.DMA((5,)), pltpu.SemaphoreType.DMA((NB,)),
            ] + [s_shape] * P['NSB'] + [pltpu.VMEM((3 * BQ, 128), f32)] * P['NAB'] + [pltpu.VMEM((D,), bf16)],
            compiler_params=pltpu.CompilerParams(vmem_limit_bytes=120 * 1024 * 1024, flags=flags),
            name="fused_kernel",
        )(A_x.reshape(S, D), A_k_cache.reshape(H, SK, DH), A_v_cache.reshape(H, SK, DH), A_wq, A_wo.reshape(NG, G * DH, D),
          B_w_r, B_w_gate.T, B_w_up.T, B_w_down)
        return out.reshape(1, S, D)
    return fn


_impl = make()


@jax.jit
def pallas_recurrent_scan__mha_block_cached__moe_arch_mod__prompt_kernel(
    A_x, A_k_cache, A_v_cache, A_wq, A_wo, B_x, B_w_r, B_w_gate, B_w_up, B_w_down
):
    return _impl(A_x, A_k_cache, A_v_cache, A_wq, A_wo, B_x, B_w_r, B_w_gate, B_w_up, B_w_down)
```

```python
import functools
import numpy as np
import jax
import jax.numpy as jnp
from jax import lax
import jax.experimental.pallas as pl
import jax.experimental.pallas.tpu as pltpu

S, D, H, DH, SK, F, C = 2048, 640, 32, 128, 2048, 1728, 8
LOG2E = 1.4426950408889634
EPS = float(np.asarray(1e-5, dtype=jnp.bfloat16))
f32, bf16, i32 = jnp.float32, jnp.bfloat16, jnp.int32
NT = (((1,), (1,)), ((), ()))


def rb(x):
    return x.astype(bf16).astype(f32)


def sigmoid(x):
    return 1.0 / (1.0 + jnp.exp2(x * (-LOG2E)))


def attention_body(grp, blk0, z0, z1, w_buf, s_bufs, a_bufs, k_buf, v_buf, wo_buf, x_buf, y_buf, out_buf, out_start, next_head, P):
    BQ, KC, DL = P["BQ"], P["KC"], P["DL"]
    LA, LS, PD, LC, XD, FD, QA = (P[k] for k in "LA LS PD LC XD FD QA".split())
    NB = S // BQ; R = BQ // 16; NC = SK // KC; W = KC // 128; L = NC + DL
    def s_loc(g, w, r):
        return (g // L) % len(s_bufs), (((g % L) * R + r) * W + w) * 16
    def ld_s(g, w, r):
        par, o = s_loc(g, w, r)
        return s_bufs[par][pl.ds(z1 + o, 16), :]
    def st_s(g, w, r, v):
        par, o = s_loc(g, w, r)
        s_bufs[par][pl.ds(z0 + o, 16), :] = v
    def st_tok(g, v):
        s_bufs[s_loc(g, 0, 0)[0]][pl.ds(z0 + L * R * W * 16, 8), :] = v
    MX, LP, OA = 0, BQ, 2 * BQ
    def ld(a, off, r): return a_bufs[a % len(a_bufs)][pl.ds(z1 + (off + 16 * r), 16), :]
    def st(a, off, r, v): a_bufs[a % len(a_bufs)][pl.ds(z0 + (off + 16 * r), 16), :] = v
    G, M = P["G"], P["M"]; NU = G * M; KT = D // 128
    heads = [grp * G + u % G for u in range(NU)]
    qbase = pl.multiple_of(P["QB"] + grp * (G * S // 2) + blk0 * (BQ // 2), 32)
    qrow = [qbase + (u % G) * (S // 2) + (u // G) * (BQ // 2) for u in range(NU)]
    row0 = pl.multiple_of(blk0 * BQ, BQ); row2 = pl.multiple_of(blk0 * (BQ // 2), BQ // 2)
    first = lax.broadcasted_iota(i32, (16, 128), 0) + grp * 16 < 16
    dots = []; pend = []
    for g in range(NU * NC + L):
        if g < NU * NC: dots.append(("qk", g))
        if g - L >= 0:
            dots.append(("pv", g - L))
            b_, rem = divmod(g - L - P["OL"] + 1, G * NC)
            if rem == 0 and 1 <= b_ <= M - 2: pend += [("op", (b_ - 1) * KT + n) for n in range(KT)]
            dots += pend[:P["OP"]]; pend = pend[P["OP"]:]
    dots += pend + [("op", n) for n in range((M - 2) * KT, M * KT)]
    ev = []; val = {}
    def add(slot, prio, fn): ev.append((slot, prio, len(ev), fn))
    def res(i):
        if ("res", i) not in val:
            kind, g = dots[i]; a, c = divmod(g, NC); h = heads[a]
            if kind == "op":
                o = jnp.concatenate([pltpu.bitcast(jnp.concatenate([val.pop(("ol", i, r, u)) for r in range(R)], axis=0), bf16) for u in range(G)], axis=1)
                val["res", i] = jnp.dot(o, wo_buf[grp, :, pl.ds(g % KT * 128, 128)], preferred_element_type=f32)
            elif kind == "qk":
                q = pltpu.bitcast(jnp.concatenate([val.pop(("q", i, r)) for r in range(R)], axis=0), bf16)
                if i == 0 and P["KT"]:
                    kt = jnp.concatenate([pltpu.bitcast(w_buf[pl.ds(32 + 64 * w, 64), :], bf16) for w in range(W)], axis=1)
                    val["res", i] = jnp.dot(q, kt, preferred_element_type=f32)
                else:
                    val["res", i] = lax.dot_general(q, k_buf[h, pl.ds(c * KC, KC), :], NT, preferred_element_type=f32)
            else:
                p = jnp.concatenate([val.pop(("p", i, r)) for r in range(R)], axis=0).astype(bf16)
                val["res", i] = jnp.dot(p, v_buf[h, pl.ds(c * KC, KC), :], preferred_element_type=f32)
        return val["res", i]
    for i, (kind, g) in enumerate(dots):
        a, c = divmod(g, NC)
        la = P["LAL"] if i == len(dots) - 1 else LA
        for r in range(R):
            j = i * R + r
            if kind == "op":
                b_, n = divmod(g, KT)
                def l_o(i=i, b_=b_, r=r):
                    if "tok" in val and r % P["QO"] == 0: w_buf[pl.ds(z0, 8), :] = val["tok"]
                    for u in range(G): val["ol", i, r, u] = w_buf[pl.ds(z1 + qrow[b_ * G + u] + 8 * r, 8), :]
                add(min(j - QA, i * R + PD - 1), 1, l_o)
                def l_y(i=i, b_=b_, n=n, r=r):
                    y = y_buf[pl.ds(z1 + row0 + (n * S + b_ * BQ + 16 * r), 16), :]
                    if r % P["XT"] == 0 and 'o' not in P['SKIP']: x_buf[pl.ds(z0 + 2 * S, 16), pl.ds(0, 128)] = pltpu.bitcast(val["tok"], bf16)
                    x, xn = (x_buf[pl.ds(z1 + row0 + (k * S + b_ * BQ + 16 * r), 16), pl.ds(n * 128, 128)].astype(f32) for k in range(2))
                    val["y", i, r] = (jnp.where(first, 0.0, y), x, xn * sigmoid(xn))
                add(j + PD - P["LY"], 1, l_y)
                def s_y(i=i, b_=b_, n=n, r=r):
                    y, x, gate = val.pop(("y", i, r))
                    y = y + res(i)[16 * r:16 * r + 16]
                    val["tok"] = y[:8]
                    y_buf[pl.ds(z0 + row0 + (n * S + b_ * BQ + 16 * r), 16), :] = y
                    out = x + y * gate
                    val['out', i, r] = out[:8] + out[8:]
                    if 'f' in P['SKIP']: y_buf[pl.ds(z0 + KT * S + 8, 8), :] = pltpu.bitcast(out.astype(bf16), f32)
                    elif 'o' not in P['SKIP']: out_buf[pl.ds(row0 + b_ * BQ + 16 * r, 16), pl.ds(n * 128, 128)] = out.astype(bf16)
                    if n == KT - 1 and r == R - 1 and b_ + 1 in P['OD']: out_start(blk0, P['OD'].index(b_ + 1))
                add(j + PD, 0, s_y)
                if P["OT"]:
                    def s_ot(i=i, r=r): y_buf[pl.ds(z0 + KT * S, 8), :] = val.pop(("out", i, r))
                    add(j + PD + P["OT"], 0, s_ot)
            elif kind == "qk":
                def l_q(i=i, a=a, r=r):
                    if "tok" in val and r % P["QT"] == 0: w_buf[pl.ds(z0, 8), :] = val["tok"]
                    val["q", i, r] = w_buf[pl.ds(z1 + qrow[a] + 8 * r, 8), :]
                add(min(j - QA, i * R + PD - 1), 1, l_q)
                if c > 0:
                    def l_acc(a=a, r=r): val["mx", a, r] = ld(a, MX, r)
                    add(j + PD - LC, 1, l_acc)
                def s_res(i=i, g=g, a=a, c=c, r=r):
                    s = res(i)[16 * r:16 * r + 16]
                    tiles = [s[:, w * 128:(w + 1) * 128] for w in range(W)]
                    for w in range(W): st_s(g, w, r, tiles[w])
                    val["tok"] = tiles[W - 1][:8]
                    mx = functools.reduce(jnp.maximum, tiles)
                    if c > 0: mx = jnp.maximum(mx, val.pop(("mx", a, r)))
                    if c == NC - 1:
                        val["m", a, r] = jnp.broadcast_to(jnp.max(mx, axis=-1, keepdims=True), (16, 128))
                    else: st(a, MX, r, mx)
                add(j + PD, 0, s_res)
                if c == NC - 1:
                    def s_m(a=a, r=r): st(a, MX, r, val.pop(("m", a, r)))
                    add(j + PD + XD, 0, s_m)
            else:
                def l_lhs(i=i, g=g, a=a, c=c, r=r):
                    m = ld(a, MX, r)
                    if "tok" in val: st_tok(g, val["tok"])
                    ps = [jnp.exp2(ld_s(g, w, r) - m) for w in range(W)]
                    lp = functools.reduce(lax.add, ps)
                    if c > 0: lp = lp + ld(a, LP, r)
                    val["lp", i, r] = lp
                    val["p", i, r] = jnp.concatenate(ps, axis=1)
                add(min(j - la, i * R + PD - 1), 1, l_lhs)
                if c < NC - 1:
                    def s_lp(i=i, a=a, r=r): st(a, LP, r, val.pop(("lp", i, r)))
                    add(j - la + LS, 0, s_lp)
                if c > 0:
                    def l_acc(i=i, a=a, r=r): val["o", i, r] = ld(a, OA, r)
                    add(j + PD - LC, 1, l_acc)
                if c < NC - 1:
                    def s_res(i=i, a=a, c=c, r=r):
                        d = res(i)[16 * r:16 * r + 16]
                        if c > 0: d = d + val.pop(("o", i, r))
                        val["tok"] = d[:8]
                        st(a, OA, r, d)
                    add(j + PD, 0, s_res)
                else:
                    def s_res(i=i, r=r):
                        d = res(i)[16 * r:16 * r + 16] + val.pop(("o", i, r))
                        val["tok"] = d[:8]
                        val["of", i, r] = d
                    add(j + PD, 0, s_res)
                    def s_fin(i=i, a=a, r=r):
                        l = jnp.sum(val.pop(("lp", i, r)), axis=-1, keepdims=True)
                        r0 = pl.reciprocal(l, approx=True)
                        rl = r0 * (2.0 - l * r0)
                        ob = pltpu.bitcast((val.pop(("of", i, r)) * rl).astype(bf16), f32)
                        w_buf[pl.ds(z0 + qrow[a] + 8 * r, 8), :] = ob
                    add(max(j - la + LS + XD + FD, j + PD), 0, s_fin)
    for w in range(W if P["KT"] else 0):
        def s_kt(w=w): w_buf[pl.ds(z0 + 32 + 64 * w, 64), :] = pltpu.bitcast(k_buf[next_head, pl.ds(w * 128, 128), :].T, f32)
        add(P["KT"] + 2 * w, 0, s_kt)
    ev.sort(key=lambda e: e[:3])
    for e in ev: e[3]()


def make(flags=None, **kw):
    P = dict(BQ=128, NU=39, KC=512, DL=2, LA=4, LAL=4, LS=3, PD=8, LC=2, XD=9, FD=2, QA=2, BX=256, G=4, BO=256, HA=8, TW=0, KT=0, SKIP="",
             DS=('x0 wr q0 x1', 'x2', 'x3', '', 'x4', '', 'q1 qr'), BC=256, M=8, OT=0, OD=(0, 1, 2, 3, 4, 5, 6, 7, 8), OL=2, OP=5, QO=1, LY=4, XT=2, NJ=2, HQ=0, RA=1, RS=1, MB=20, TF=0, RP=32, R0=16, NSB=11, NAB=11, QT=8, GS=50, GD=2, UO=2, UJ=2, F0=0, FG=8, FS=(5, 3), XB=1, DENSE=1, LN=64, XA=(0, 1, 2, 4, 6, 8))
    P.update(kw)
    BQ, NU, KC, BX, G, BO, HA = (P[k] for k in "BQ NU KC BX G BO HA".split())
    P["QB"] = QB = 32 + KC // 2
    P["GB"] = GB = QB + H * S // 2
    NB = S // BQ; NX = S // BX; NG = H // G; NO = S // BO
    L = SK // KC + P["DL"]

    def kernel(x_hbm, k_hbm, v_hbm, wq_hbm, wo_hbm, wr_hbm, wg_hbm, wu_hbm, wd_hbm, out_hbm,
               x_buf, xn_buf, w_buf, y_buf, k_buf, v_buf, wq_buf, wo_buf, wg_buf, wu_buf, wd_buf, out_buf, z_ref,
               x_sem, wq_sem, kv_sem, misc_sem, out_sem, *bufs):
        s_bufs, a_bufs, wr_buf = bufs[:P['NSB']], bufs[P['NSB']:-1], bufs[-1]
        KT = D // 128; XA = P["XA"]; LN = P["LN"]
        xr = [(a_ * BX, (b_ - a_) * BX) for a_, b_ in zip(XA[:-1], XA[1:])]
        x_cp = lambda i: pltpu.make_async_copy(x_hbm.at[pl.ds(*xr[i])], x_buf.at[pl.ds(*xr[i])], x_sem.at[i])
        wq_cp = lambda j: pltpu.make_async_copy(wq_hbm.at[:, pl.ds(j * G * DH, G * DH)], wq_buf.at[j], wq_sem.at[j])
        wq_half = lambda k: pltpu.make_async_copy(wq_hbm.at[:, pl.ds(k * 256, 256)], wq_buf.at[0, :, pl.ds(k * 256, 256)], misc_sem.at[5 + k])
        hr = [(0, HA), (HA, H - HA)]
        k_cp = lambda j: pltpu.make_async_copy(k_hbm.at[pl.ds(*hr[j])], k_buf.at[pl.ds(*hr[j])], kv_sem.at[2 * j])
        v_cp = lambda j: pltpu.make_async_copy(v_hbm.at[pl.ds(*hr[j])], v_buf.at[pl.ds(*hr[j])], kv_sem.at[2 * j + 1])
        wr_cp = lambda: pltpu.make_async_copy(wr_hbm, wr_buf, misc_sem.at[0])
        wg_cp = lambda: pltpu.make_async_copy(wg_hbm, wg_buf, misc_sem.at[1])
        wu_cp = lambda: pltpu.make_async_copy(wu_hbm, wu_buf, misc_sem.at[2])
        wd_cp = lambda: pltpu.make_async_copy(wd_hbm, wd_buf, misc_sem.at[3])
        wo_cp = lambda: pltpu.make_async_copy(wo_hbm, wo_buf, misc_sem.at[4])

        cur = []
        def mark(name):
            if not P.get("PROF"): return
            if cur: cur.pop().__exit__(None, None, None)
            if name:
                cm = jax.named_scope(name); cm.__enter__(); cur.append(cm)
        mark("p0_wait_x0")
        cps = dict(x0=lambda: x_cp(0), x1=lambda: x_cp(1), x2=lambda: x_cp(2), x3=lambda: x_cp(3), x4=lambda: x_cp(4), wr=wr_cp,
                   q0=lambda: wq_cp(0), qa=lambda: wq_half(0), qb=lambda: wq_half(1), q1=lambda: wq_cp(1))
        def start(stage):
            for nm in P["DS"][stage].split():
                if nm == "qr":
                    for j in range(2, (NX + P['MB'] - 1) // NX + 1): wq_cp(j).start()
                else: cps[nm]().start()
        start(0)
        z_ref[0] = 0
        z_ref[1] = 0

        def store_q(j, g, i, q, BX=BX):
            q = (q * (DH ** -0.5 * LOG2E)).astype(bf16)
            r0 = pl.multiple_of(QB + (j * G + g) * (S // 2) + i * (BX // 2), 32)
            w_buf[pl.ds(r0, BX // 2), :] = pltpu.bitcast(q, f32)
            return q

        def qproj(j, i, after=None):
            xn = xn_buf[pl.ds(i * BX if isinstance(i, int) else pl.multiple_of(i * BX, BX), BX), :]
            if after is not None:
                head = jnp.where(lane > j + 1000, after, pltpu.bitcast(xn[:16, :128], f32))
                xn = jnp.concatenate([jnp.concatenate([pltpu.bitcast(head, bf16), xn[:16, 128:]], axis=1), xn[16:]], axis=0)
            q = jnp.dot(xn, wq_buf[j], preferred_element_type=f32)
            return [store_q(j, g, i, q[:, g * DH:(g + 1) * DH]) for g in range(G)]

        lane = lax.broadcasted_iota(i32, (8, 128), 1)
        sub = lax.broadcasted_iota(i32, (8, 128), 0)

        def layernorm(r0, n):
            x = x_buf[pl.ds(r0, n), :].astype(f32)
            m = jnp.sum(x, axis=-1, keepdims=True)
            yield
            m = m * (1.0 / D)
            mb = rb(m)
            xc = x - mb
            dm = m - mb
            var = jnp.sum(xc * xc, axis=-1, keepdims=True)
            if P["XB"]: xb = xc.astype(bf16)
            yield
            var = jnp.broadcast_to(var * (1.0 / D) - dm * dm, (n, 128))
            if P["DENSE"]:
                dense = var[:8]
                for t in range(1, n // 8):
                    dense = jnp.where(lane == t, var[t * 8:(t + 1) * 8], dense)
                inv = 1.0 / rb(jnp.sqrt(rb(rb(jnp.maximum(dense, 0.0)) + EPS)))
                inv = jnp.concatenate([jnp.broadcast_to(inv[:, t:t + 1], (8, 128)) for t in range(n // 8)], axis=0)
                yield
            else:
                inv = 1.0 / rb(jnp.sqrt(rb(rb(jnp.maximum(var, 0.0)) + EPS)))
            xr_ = xb.astype(f32) if P["XB"] else rb(xc)
            xn = jnp.concatenate([xr_[:, w * 128:(w + 1) * 128] * inv for w in range(D // 128)], axis=1).astype(bf16)
            xn_buf[pl.ds(r0, n), :] = xn
            x_buf[pl.ds(S + r0, n), :] = xn
            yield "stored"

        ln = dict(next=0, done=0, live=[])
        def layernorm_upto(row, avail):
            while ln["done"] < row:
                for gen in list(ln["live"]):
                    st_ = next(gen, "end")
                    if st_ == "stored": ln["done"] += LN
                    if st_ == "end": ln["live"].remove(gen)
                if ln["next"] < avail:
                    gen = layernorm(ln["next"], LN); next(gen)
                    ln["live"].append(gen); ln["next"] += LN

        x_cp(0).wait()
        start(1)
        wr_cp().wait()
        mark('p1_ln0')
        layernorm_upto(BX, BX)
        mark('p2_wait_wq0')
        (wq_half(0) if P['HQ'] else wq_cp(0)).wait()
        start(2)
        starts = [r[0] // BX for r in xr]
        for i in range(NX):
            if i + 1 in starts:
                n_ = starts.index(i + 1)
                mark(f'p3_wait_x{n_}')
                start(2 + n_)
                x_cp(n_).wait()
                avail = xr[n_][0] + xr[n_][1]
            if i + 1 in starts: mark(f'p3_q{i}')
            def half(i, k):
                q = jnp.dot(xn_buf[pl.ds(i * BX, BX), :], wq_buf[0, :, pl.ds(k * 256, 256)], preferred_element_type=f32)
                for g in range(2): store_q(0, 2 * k + g, i, q[:, g * DH:(g + 1) * DH])
            if P["HQ"] and i == 0:
                half(0, 0); layernorm_upto(2 * BX, avail); half(1, 0)
                continue
            if P["HQ"] and i == 1:
                wq_half(1).wait(); half(0, 1); half(1, 1)
            else:
                qproj(0, i)
            if i + 1 < NX:
                layernorm_upto((i + 2) * BX, avail)
        for gen in ln["live"]:
            for _ in gen: pass

        NJ, MB = P["NJ"], P["MB"]
        last = lambda jj: (NX + (jj + 1) * MB - 1) // NX
        RR = -(-S // (NJ * 256)) * 256
        row16 = lax.broadcasted_iota(i32, (16, D), 0)
        def top_k(rds):
            keys = []
            for t in range(NJ):
                r = rb(rds[t])
                r = jnp.where(r == 0.0, 0.0, r)
                b = lax.shift_right_logical(pltpu.bitcast(r, i32), 16)
                k16 = jnp.where(b >= 0x8000, 0xFFFF - b, b + 0x8000)
                k16 = jnp.where(r != r, 0, k16)
                tok = min(t * RR, S - RR) + lane * 8 + sub
                keys.append(pltpu.bitcast(jnp.where(lane < RR // 8, 0x20000000 + k16 * 2048 + (2047 - tok), 0), f32))
            ktop = jnp.zeros((8, 128), i32)
            x_sel = jnp.zeros((16, D), f32)
            for c in range(C):
                mx = functools.reduce(jnp.maximum, keys)
                mx = jnp.max(jnp.max(mx, axis=0, keepdims=True), axis=1, keepdims=True)
                mxb = jnp.broadcast_to(mx, (8, 128))
                keys = [jnp.where(kk == mxb, 0.0, kk) for kk in keys]
                mi = pltpu.bitcast(mxb, i32)
                ktop = jnp.where(sub == c, mi, ktop)
                idx = 2047 - (mi[0, 0] & 2047)
                base = pl.multiple_of(idx & -16, 16)
                blk = xn_buf[pl.ds(base, 16), :].astype(f32)
                rowv = jnp.sum(jnp.where(row16 == idx - base, blk, 0.0), axis=0, keepdims=True)
                x_sel = jnp.where(row16 == c, rowv, x_sel)
            return ktop, x_sel
        mark('p5_1b')
        def p1_body(jj, carry):
            for t in range(NJ):
                @pl.when(jj == t)
                def _():
                    js = list(range(last(t - 1) + 1, last(t) + 1))
                    for j in js[:-1]: wq_cp(j).wait()
                    if t == 0:
                        for j in range(last(0) + 1, NG): wq_cp(j).start()
                        wg_cp().start(); wu_cp().start(); wd_cp().start()
                    if t == P['TW']: wo_cp().start()
                    if t == 1:
                        k_cp(0).start(); v_cp(0).start()
                    wq_cp(js[-1]).wait()
            wr = wr_buf[...].astype(f32).reshape(1, D)
            r0 = pl.multiple_of(jnp.minimum(jj * RR, S - RR), 256)
            rd = jnp.zeros((8, 128), f32)
            RP = P["RP"]
            never = lax.broadcasted_iota(i32, (8, 128), 1) > jj + 1000
            after = None
            for n_ in range(MB):
                b_ = NX + jj * MB + n_
                qs = qproj(lax.shift_right_logical(b_, NX.bit_length() - 1), b_ & (NX - 1), after if n_ == P["R0"] else None)
                for g in range(G if n_ * G * RP < RR else 0):
                    tok = pltpu.bitcast(qs[g][:16], f32)
                    for t in range((n_ * G + g) * RP // 16, (n_ * G + g + 1) * RP // 16):
                        r = 0.0
                        for w in range(KT):
                            xb = pltpu.bitcast(xn_buf[pl.ds(r0 + t * 16, 16), pl.ds(w * 128, 128)], f32)
                            d_ = pltpu.bitcast(jnp.where(never, tok, xb), bf16).astype(f32) * wr[:, w * 128:(w + 1) * 128]
                            r = d_ if w == 0 else r + d_
                        r = jnp.broadcast_to(jnp.sum(r, axis=-1, keepdims=True), (16, 128))
                        rd = jnp.where(lane == 2 * t, r[:8], jnp.where(lane == 2 * t + 1, r[8:], rd))
                if (n_ + 1) * G * RP == RR:
                    rds = [jnp.where(jnp.full((8, 128), jj) == t, rd, carry[0][t]) for t in range(NJ)]
                    ktop, x_sel = top_k(rds)
                    after = functools.reduce(lax.add, [x_sel[:8, w * 128:(w + 1) * 128] for w in range(KT)])
            return rds, ktop, x_sel
        zero = jnp.zeros((8, 128), f32)
        _, ktop, x_sel = lax.fori_loop(0, NJ, p1_body, ([zero] * NJ, jnp.zeros((8, 128), i32), jnp.zeros((16, D), f32)))
        x_sel = x_sel[:8]

        mark('p6_wait')
        for j in range(last(NJ - 1) + 1, NG): wq_cp(j).wait()
        wg_cp().wait(); wu_cp().wait(); wd_cp().wait()
        k_cp(0).wait(); v_cp(0).wait(); wo_cp().wait()
        mark('p7_1c')
        k16 = lax.shift_right_logical(ktop - 0x20000000, 11)
        b = jnp.where(k16 >= 0x8000, k16 - 0x8000, 0xFFFF - k16)
        r_sel = pltpu.bitcast(lax.shift_left(b, 16), f32)[:, :1]
        xs = x_sel.astype(bf16)
        acc = {}
        def accum(key, d):
            acc[key] = acc[key] + d if key in acc else d
        BC = P["BC"]
        def q_tile(j, i, g, k):
            accum((j, i, g), jnp.dot(xn_buf[pl.ds(i * BC, BC), pl.ds(k * 128, 128)], wq_buf[j, pl.ds(k * 128, 128), pl.ds(g * DH, DH)], preferred_element_type=f32))
            if k == KT - 1:
                store_q(j, g, i, acc.pop((j, i, g)), BC)
        fr = [(f0, min(128, F - f0)) for f0 in range(0, F, 128)]
        def up_tile(name, w, f, k):
            accum((name, f), lax.dot_general(xs[:, k * 128:(k + 1) * 128], w[pl.ds(*fr[f]), pl.ds(k * 128, 128)], NT, preferred_element_type=f32))
        def down_tile(f, n):
            if n == 0:
                a = rb(acc.pop(("g", f)))
                acc["h"] = (rb(a * sigmoid(a)) * rb(acc.pop(("u", f)))).astype(bf16)
            accum(("y", n), jnp.dot(acc["h"], wd_buf[pl.ds(*fr[f]), pl.ds(n * 128, 128)], preferred_element_type=f32))
        part = functools.partial
        q_tiles = [part(q_tile, j, i, g, k) for j in range(NG) for i in range(S // BC) if j * S + i * BC >= (NX + NJ * MB) * BX for g in range(G) for k in range(KT)]
        f_tiles = [part(up_tile, nm, w, f, k) for f in range(len(fr)) for nm, w in (("g", wg_buf), ("u", wu_buf)) for k in range(KT)]
        f_tiles += [None] * (4 * P["FG"])
        f_tiles += [part(down_tile, f, n) for f in range(len(fr)) for n in range(KT)]
        for rnd in range(len(q_tiles) // 4):
            for fn_ in q_tiles[4 * rnd:4 * rnd + 4]:
                fn_()
            if rnd >= P["F0"] and rnd % P['FS'][0] not in P['FS'][1:]:
                for fn_ in f_tiles[:4]:
                    if fn_ is not None: fn_()
                f_tiles = f_tiles[4:]
        assert not f_tiles
        y = rb(jnp.concatenate([acc.pop(("y", n)) for n in range(KT)], axis=1))
        z = rb(x_sel + rb(y * rb(sigmoid(r_sel))))
        for c in range(C):
            idx = 2047 - (ktop[c, 0] & 2047)
            at = pl.ds(S + pl.multiple_of(idx & -16, 16), 16)
            x_buf[at, :] = jnp.where(row16 == (idx & 15), z[c:c + 1, :], x_buf[at, :].astype(f32)).astype(bf16)

        k_cp(1).start(); v_cp(1).start()
        if P['KT']:
            for w in range(KC // 128):
                w_buf[pl.ds(32 + 64 * w, 64), :] = pltpu.bitcast(k_buf[0, pl.ds(w * 128, 128), :].T, f32)
        mark('p8_att')
        M = P["M"]; PG = NB // M
        OD = P["OD"]
        def out_cp(blk0, k):
            rows = pl.ds((blk0 + OD[k - 1]) * BQ, (OD[k] - OD[k - 1]) * BQ)
            return pltpu.make_async_copy(out_buf.at[rows], out_hbm.at[rows], out_sem.at[blk0 + k - 1])
        z0, z1 = (pl.multiple_of(z_ref[i], 32) for i in range(2))
        def att_body(t, _):
            @pl.when(t == HA // G * PG - 1)
            def _():
                if 'k' not in P['SKIP']: k_cp(1).wait(); v_cp(1).wait()
            grp = lax.shift_right_logical(t, PG.bit_length() - 1)
            def out_start(blk0, k):
                @pl.when(grp == NG - 1)
                def _():
                    out_cp(blk0, k).start()
            attention_body(grp, (t & (PG - 1)) * M, z0, z1, w_buf, s_bufs, a_bufs, k_buf, v_buf, wo_buf, x_buf, y_buf, out_buf, out_start, jnp.minimum(lax.shift_right_logical(t + 1, PG.bit_length() - 1), NG - 1) * G, P)
        lax.fori_loop(P.get('T0', 0), NG * PG, att_body, None)
        mark('pa_wait_out')
        for blk0 in range(0, NB, M):
            for k in range(1, len(OD)):
                out_cp(blk0, k).wait()
        mark(None)

    @jax.jit
    def fn(A_x, A_k_cache, A_v_cache, A_wq, A_wo, B_x, B_w_r, B_w_gate, B_w_up, B_w_down):
        any_spec = pl.BlockSpec(memory_space=pl.ANY)
        s_shape = pltpu.VMEM((L * BQ * (KC // 128) + 32, 128), f32)
        out = pl.pallas_call(
            kernel,
            in_specs=[any_spec] * 9,
            out_specs=any_spec,
            out_shape=jax.ShapeDtypeStruct((S, D), bf16),
            scratch_shapes=[
                pltpu.VMEM((2 * S + 64, D), bf16), pltpu.VMEM((S, D), bf16),
                pltpu.VMEM((GB, DH), f32), pltpu.VMEM((D // 128 * S + 32, DH), f32),
                pltpu.VMEM((H, SK, DH), bf16), pltpu.VMEM((H, SK, DH), bf16),
                pltpu.VMEM((NG, D, G * DH), bf16), pltpu.VMEM((NG, G * DH, D), bf16),
                pltpu.VMEM((F, D), bf16), pltpu.VMEM((F, D), bf16), pltpu.VMEM((F, D), bf16),
                pltpu.VMEM((S, D), bf16), pltpu.SMEM((2,), i32),
                pltpu.SemaphoreType.DMA((len(P['XA']) - 1,)), pltpu.SemaphoreType.DMA((NG,)), pltpu.SemaphoreType.DMA((4,)),
                pltpu.SemaphoreType.DMA((7,)), pltpu.SemaphoreType.DMA((NB,)),
            ] + [s_shape] * P['NSB'] + [pltpu.VMEM((3 * BQ, 128), f32)] * P['NAB'] + [pltpu.VMEM((D,), bf16)],
            compiler_params=pltpu.CompilerParams(vmem_limit_bytes=120 * 1024 * 1024, flags=flags),
            name="fused_kernel",
        )(A_x.reshape(S, D), A_k_cache.reshape(H, SK, DH), A_v_cache.reshape(H, SK, DH), A_wq, A_wo.reshape(NG, G * DH, D),
          B_w_r, B_w_gate.T, B_w_up.T, B_w_down)
        return out.reshape(1, S, D)
    return fn


_impl = make()


@jax.jit
def pallas_recurrent_scan__mha_block_cached__moe_arch_mod__prompt_kernel(
    A_x, A_k_cache, A_v_cache, A_wq, A_wo, B_x, B_w_r, B_w_gate, B_w_up, B_w_down
):
    return _impl(A_x, A_k_cache, A_v_cache, A_wq, A_wo, B_x, B_w_r, B_w_gate, B_w_up, B_w_down)
```

```python
import functools
import numpy as np
import jax
import jax.numpy as jnp
from jax import lax
import jax.experimental.pallas as pl
import jax.experimental.pallas.tpu as pltpu

S, D, H, DH, SK, F, C = 2048, 640, 32, 128, 2048, 1728, 8
LOG2E = 1.4426950408889634
EPS = float(np.asarray(1e-5, dtype=jnp.bfloat16))
f32, bf16, i32 = jnp.float32, jnp.bfloat16, jnp.int32
NT = (((1,), (1,)), ((), ()))


def rb(x):
    return x.astype(bf16).astype(f32)


def sigmoid(x):
    return 1.0 / (1.0 + jnp.exp2(x * (-LOG2E)))


def attention_body(grp, blk0, z0, z1, w_buf, s_bufs, a_bufs, k_buf, v_buf, wo_buf, x_buf, y_buf, out_buf, u_buf, out_start, next_head, gate_row, P):
    BQ, KC, DL = P["BQ"], P["KC"], P["DL"]
    LA, LS, PD, LC, XD, FD, QA = (P[k] for k in "LA LS PD LC XD FD QA".split())
    NB = S // BQ; R = BQ // 16; NC = SK // KC; W = KC // 128; L = NC + DL
    def s_loc(g, w, r):
        return (g // L) % len(s_bufs), (((g % L) * R + r) * W + w) * 16
    def ld_s(g, w, r):
        par, o = s_loc(g, w, r)
        return s_bufs[par][pl.ds(z1 + o, 16), :]
    def st_s(g, w, r, v):
        par, o = s_loc(g, w, r)
        s_bufs[par][pl.ds(z0 + o, 16), :] = v
    def st_tok(g, v):
        s_bufs[s_loc(g, 0, 0)[0]][pl.ds(z0 + L * R * W * 16, 8), :] = v
    MX, LP, OA = 0, BQ, 2 * BQ
    def ld(a, off, r): return a_bufs[a % len(a_bufs)][pl.ds(z1 + (off + 16 * r), 16), :]
    def st(a, off, r, v): a_bufs[a % len(a_bufs)][pl.ds(z0 + (off + 16 * r), 16), :] = v
    G, M = P["G"], P["M"]; NU = G * M; KT = D // 128
    heads = [grp * G + u % G for u in range(NU)]
    qbase = pl.multiple_of(P["QB"] + grp * (G * S // 2) + blk0 * (BQ // 2), 32)
    qrow = [qbase + (u % G) * (S // 2) + (u // G) * (BQ // 2) for u in range(NU)]
    row0 = pl.multiple_of(blk0 * BQ, BQ); row2 = pl.multiple_of(blk0 * (BQ // 2), BQ // 2)
    first = lax.broadcasted_iota(i32, (16, 128), 0) + grp * 16 < 16
    STEPS = [
        ("e", 0, [(0, 4, 1)]),
        (((0, 0, 1), (0, 1, 1)), (1, 1), [(0, 0, -1), (0, 2, 1)]),
        (((1, 0, 1), (1, 1, 1)), (0, 0), [(1, 0, 1), (1, 2, -1)]),
        (((0, 0, 1),), 0, [(0, 2, 1), (1, 2, 1)]),
        (((1, 1, 1),), 1, [(0, 0, 1), (1, 0, 1)]),
        (((0, 1, 1), (1, 1, -1)), 2, [(0, 0, 1)]),
        (((0, 0, 1), (1, 1, 1)), 3, [(0, 0, 1), (1, 2, 1)]),
        (((1, 0, 1), (0, 0, -1)), 4, [(1, 2, 1)]),
        ("e", 1, [(1, 4, 1)]),
    ]
    U_SUMS = [((0, 1), (1, 1), -1), ((1, 0), (0, 0), -1), ((1, 0), (1, 1), 1), ((0, 0), (1, 1), 1), ((0, 0), (0, 1), 1)]
    NS_ = len(STEPS)
    dots = []; pend = []
    for g in range(NU * NC + L):
        if g < NU * NC: dots.append(("qk", g))
        if g - L >= 0:
            dots.append(("pv", g - L))
            b_, rem = divmod(g - L - P["OL"] + 1, 2 * G * NC)
            if rem == 0 and 1 <= b_ <= M // 2 - 1: pend += [("op", (b_ - 1) * NS_ + n) for n in range(NS_)]
            if len(pend) > (P['HB'] if g - L >= (M - 2) * G * NC else 0):
                n_ = min(P['OP'], len(pend) - (P['HB'] if g - L >= (M - 2) * G * NC else 0))
                dots += pend[:n_]; pend = pend[n_:]
    dots += pend + [("op", n) for n in range((M // 2 - 1) * NS_, M // 2 * NS_)]
    ev = []; val = {}
    def add(slot, prio, fn): ev.append((slot, prio, len(ev), fn))
    def res(i):
        if ("res", i) not in val:
            kind, g = dots[i]; a, c = divmod(g, NC); h = heads[a]
            if kind == "op":
                lhs, rhs, _ = STEPS[g % NS_]
                o = jnp.concatenate([val.pop(("ol", i, r)) for r in range(R)], axis=0)
                if lhs == "e": w_ = wo_buf[grp, :, pl.ds(512, 128)]
                elif isinstance(rhs, tuple): w_ = wo_buf[grp, pl.ds(rhs[0] * 256, 256), pl.ds(rhs[1] * 256, 256)]
                else: w_ = pltpu.bitcast(u_buf[pl.ds(z1 + rhs * 128, 128), :], bf16)
                val["res", i] = jnp.dot(o, w_, preferred_element_type=f32)
            elif kind == "qk":
                q = pltpu.bitcast(jnp.concatenate([val.pop(("q", i, r)) for r in range(R)], axis=0), bf16)
                if i == 0 and P["KT"]:
                    kt = jnp.concatenate([pltpu.bitcast(w_buf[pl.ds(32 + 64 * w, 64), :], bf16) for w in range(W)], axis=1)
                    val["res", i] = jnp.dot(q, kt, preferred_element_type=f32)
                else:
                    val["res", i] = lax.dot_general(q, k_buf[h, pl.ds(c * KC, KC), :], NT, preferred_element_type=f32)
            else:
                p = jnp.concatenate([val.pop(("p", i, r)) for r in range(R)], axis=0).astype(bf16)
                val["res", i] = jnp.dot(p, v_buf[h, pl.ds(c * KC, KC), :], preferred_element_type=f32)
        return val["res", i]
    for i, (kind, g) in enumerate(dots):
        a, c = divmod(g, NC)
        la = P["LAL"] if i == len(dots) - 1 else LA
        for r in range(R):
            j = i * R + r
            if kind == "op":
                bp, n = divmod(g, NS_)
                lhs, rhs, outs = STEPS[n]
                def l_o(i=i, bp=bp, lhs=lhs, rhs=rhs, r=r):
                    if "tok" in val and r % P["QO"] == 0: w_buf[pl.ds(z0, 8), :] = val["tok"]
                    get = lambda b_, u: pltpu.bitcast(w_buf[pl.ds(z1 + qrow[(2 * bp + b_) * G + u] + 8 * r, 8), :], bf16)
                    if lhs == "e": tiles = [get(rhs, u) for u in range(G)]
                    elif len(lhs) == 1: tiles = [get(lhs[0][0], 2 * lhs[0][1] + u) for u in range(2)]
                    else:
                        tiles = []
                        for u in range(2):
                            t0, t1 = (get(b_, 2 * k + u).astype(f32) for b_, k, _ in lhs)
                            tiles.append((t0 + t1 if lhs[1][2] > 0 else t0 - t1).astype(bf16))
                    val["ol", i, r] = jnp.concatenate(tiles, axis=1)
                add(min(j - P["QP"], i * R + PD - 1), 1, l_o)
                todo = []
                for b_, n0_, sign in outs:
                    users = [k for k, st_ in enumerate(STEPS) if any(o_[:2] == (b_, n0_) for o_ in st_[2])]
                    todo += [(2 * bp + b_, n0_ + u, u, sign, n == users[0], n == users[-1]) for u in range(1 if lhs == "e" else 2)]
                def l_y(i=i, todo=todo, r=r):
                    if r % P["XT"] == 0 and any(t_[5] for t_ in todo): x_buf[pl.ds(z0 + 2 * S, 16), pl.ds(0, 128)] = pltpu.bitcast(val["tok"], bf16)
                    for b_, n_, u, sign, is_first, is_last in todo:
                        y = y_buf[pl.ds(z1 + row0 + (n_ * S + b_ * BQ + 16 * r), 16), :]
                        val["y", i, r, b_, n_] = jnp.where(first, 0.0, y) if is_first else y
                        if is_last:
                            x, xn = (x_buf[pl.ds(z1 + row0 + (k * S + b_ * BQ + 16 * r), 16), pl.ds(n_ * 128, 128)].astype(f32) for k in range(2))
                            val["xg", i, r, b_, n_] = (x, xn)
                add(j + PD - P["LY"], 1, l_y)
                def s_y(i=i, todo=todo, n=n, bp=bp, r=r):
                    for b_, n_, u, sign, is_first, is_last in todo:
                        d = res(i)[16 * r:16 * r + 16, u * 128:(u + 1) * 128]
                        y = val.pop(("y", i, r, b_, n_))
                        y = y + d if sign > 0 else y - d
                        y_buf[pl.ds(z0 + row0 + (n_ * S + b_ * BQ + 16 * r), 16), :] = y
                        if is_last:
                            x, gate = val.pop(("xg", i, r, b_, n_))
                            out_buf[pl.ds(row0 + b_ * BQ + 16 * r, 16), pl.ds(n_ * 128, 128)] = (x + y * gate).astype(bf16)
                    val["tok"] = y[:8]
                    if r == R - 1 and n in (NS_ - 3, NS_ - 1): out_start(blk0, 2 * bp + 1 + (n == NS_ - 1))
                add(j + PD, 0, s_y)
            elif kind == "qk":
                def l_q(i=i, a=a, r=r):
                    if "tok" in val and r % P["QT"] == 0: w_buf[pl.ds(z0, 8), :] = val["tok"]
                    val["q", i, r] = w_buf[pl.ds(z1 + qrow[a] + 8 * r, 8), :]
                add(min(j - QA, i * R + PD - 1), 1, l_q)
                if c > 0:
                    def l_acc(a=a, r=r): val["mx", a, r] = ld(a, MX, r)
                    add(j + PD - LC, 1, l_acc)
                def s_res(i=i, g=g, a=a, c=c, r=r):
                    s = res(i)[16 * r:16 * r + 16]
                    tiles = [s[:, w * 128:(w + 1) * 128] for w in range(W)]
                    for w in range(W): st_s(g, w, r, tiles[w])
                    val["tok"] = tiles[W - 1][:8]
                    mx = functools.reduce(jnp.maximum, tiles)
                    if c > 0: mx = jnp.maximum(mx, val.pop(("mx", a, r)))
                    if c == NC - 1:
                        val["m", a, r] = jnp.broadcast_to(jnp.max(mx, axis=-1, keepdims=True), (16, 128))
                    else: st(a, MX, r, mx)
                add(j + PD, 0, s_res)
                if c == NC - 1:
                    def s_m(a=a, r=r): st(a, MX, r, val.pop(("m", a, r)))
                    add(j + PD + XD, 0, s_m)
            else:
                def l_lhs(i=i, g=g, a=a, c=c, r=r):
                    m = ld(a, MX, r)
                    if "tok" in val: st_tok(g, val["tok"])
                    ps = [jnp.exp2(ld_s(g, w, r) - m) for w in range(W)]
                    lp = functools.reduce(lax.add, ps)
                    if c > 0: lp = lp + ld(a, LP, r)
                    val["lp", i, r] = lp
                    val["p", i, r] = jnp.concatenate(ps, axis=1)
                add(min(j - la, i * R + PD - 1), 1, l_lhs)
                if c < NC - 1:
                    def s_lp(i=i, a=a, r=r): st(a, LP, r, val.pop(("lp", i, r)))
                    add(j - la + LS, 0, s_lp)
                if c > 0:
                    def l_acc(i=i, a=a, r=r): val["o", i, r] = ld(a, OA, r)
                    add(j + PD - LC, 1, l_acc)
                if c < NC - 1:
                    def s_res(i=i, a=a, c=c, r=r):
                        d = res(i)[16 * r:16 * r + 16]
                        if c > 0: d = d + val.pop(("o", i, r))
                        val["tok"] = d[:8]
                        st(a, OA, r, d)
                    add(j + PD, 0, s_res)
                else:
                    def s_res(i=i, r=r):
                        d = res(i)[16 * r:16 * r + 16] + val.pop(("o", i, r))
                        val["tok"] = d[:8]
                        val["of", i, r] = d
                    add(j + PD, 0, s_res)
                    def s_fin(i=i, a=a, r=r):
                        l = jnp.sum(val.pop(("lp", i, r)), axis=-1, keepdims=True)
                        r0 = pl.reciprocal(l, approx=True)
                        rl = r0 * (2.0 - l * r0)
                        ob = pltpu.bitcast((val.pop(("of", i, r)) * rl).astype(bf16), f32)
                        w_buf[pl.ds(z0 + qrow[a] + 8 * r, 8), :] = ob
                    add(max(j - la + LS + XD + FD, j + PD), 0, s_fin)
    for w in range(W if P["KT"] else 0):
        def s_kt(w=w): w_buf[pl.ds(z0 + 32 + 64 * w, 64), :] = pltpu.bitcast(k_buf[next_head, pl.ds(w * 128, 128), :].T, f32)
        add(P["KT"] + 2 * w, 0, s_kt)
    for k, (p0, p1, sign) in enumerate(U_SUMS):
        for r in range(16):
            def s_u(k=k, p0=p0, p1=p1, sign=sign, r=r):
                never = lax.broadcasted_iota(i32, (8, 256), 1) > grp + 1000
                tok = jnp.concatenate([val["tok"]] * 2, axis=1)
                t0, t1 = (pltpu.bitcast(jnp.where(never, tok, pltpu.bitcast(wo_buf[grp, pl.ds(p_[0] * 256 + 16 * r, 16), pl.ds(p_[1] * 256, 256)], f32)), bf16).astype(f32) for p_ in (p0, p1))
                u_ = pltpu.bitcast((t0 + t1 if sign > 0 else t0 - t1).astype(bf16), f32)
                u_buf[pl.ds(z0 + k * 128 + 8 * r, 8), :] = u_
                val["utok", k, r] = u_[:, :128]
            add(P["US"] + (k * 16 + r) * P["UD"], 2, s_u)
            def s_ut(k=k, r=r): w_buf[pl.ds(z0 + 8, 8), :] = val.pop(("utok", k, r))
            add(P["US"] + (k * 16 + r) * P["UD"] + 3, 0, s_ut)
    for r in range(S * M // (H // G * NB) // 16):
        for w in range(KT):
            def l_g(r=r, w=w):
                x_buf[pl.ds(z0 + 2 * S, 16), pl.ds(0, 128)] = pltpu.bitcast(val["tok"], bf16)
                xn = x_buf[pl.ds(z1 + gate_row + (S + 16 * r), 16), pl.ds(w * 128, 128)].astype(f32)
                val["g", r, w] = (xn * sigmoid(xn)).astype(bf16)
            add(P["GS"] + (r * KT + w) * 5, 2, l_g)
            def s_g(r=r, w=w):
                g_ = val.pop(("g", r, w))
                x_buf[pl.ds(z0 + gate_row + (S + 16 * r), 16), pl.ds(w * 128, 128)] = g_
                w_buf[pl.ds(z0 + 16, 8), :] = pltpu.bitcast(g_, f32)
            add(P["GS"] + (r * KT + w) * 5 + 4, 0, s_g)
    ev.sort(key=lambda e: e[:3])
    for e in ev: e[3]()


def make(flags=None, **kw):
    P = dict(BQ=128, NU=39, KC=512, DL=2, LA=4, LAL=4, LS=3, PD=8, LC=2, XD=9, FD=2, QA=2, BX=256, G=4, BO=256, HA=8, TW=0, KT=0, SKIP="",
             DS=('x0 wr q0 x1', 'x2', 'x3', '', 'x4', '', 'q1 qr'), BC=256, M=8, OT=0, OD=(0, 1, 2, 3, 4, 5, 6, 7, 8), OL=2, OP=1, QO=1, LY=3, XT=2, NJ=2, HB=5, QP=3, US=40, UD=4, AT=0, HQ=0, RA=1, RS=1, MB=20, TF=0, RP=32, R0=9, NSB=11, NAB=11, QT=8, GS=370, GD=2, UO=2, UJ=2, F0=0, FG=8, FS=(9, 7), XB=1, DENSE=1, LN=64, XA=(0, 1, 2, 4, 6, 8))
    P.update(kw)
    BQ, NU, KC, BX, G, BO, HA = (P[k] for k in "BQ NU KC BX G BO HA".split())
    P["QB"] = QB = 32 + KC // 2
    P["GB"] = GB = QB + H * S // 2
    NB = S // BQ; NX = S // BX; NG = H // G; NO = S // BO
    L = SK // KC + P["DL"]

    def kernel(x_hbm, k_hbm, v_hbm, wq_hbm, wo_hbm, wr_hbm, wg_hbm, wu_hbm, wd_hbm, out_hbm,
               x_buf, xn_buf, w_buf, y_buf, u_buf, k_buf, v_buf, wq_buf, wo_buf, wg_buf, wu_buf, wd_buf, out_buf, z_ref,
               x_sem, wq_sem, kv_sem, misc_sem, out_sem, *bufs):
        s_bufs, a_bufs, wr_buf = bufs[:P['NSB']], bufs[P['NSB']:-1], bufs[-1]
        KT = D // 128; XA = P["XA"]; LN = P["LN"]
        xr = [(a_ * BX, (b_ - a_) * BX) for a_, b_ in zip(XA[:-1], XA[1:])]
        x_cp = lambda i: pltpu.make_async_copy(x_hbm.at[pl.ds(*xr[i])], x_buf.at[pl.ds(*xr[i])], x_sem.at[i])
        wq_cp = lambda j: pltpu.make_async_copy(wq_hbm.at[:, pl.ds(j * G * DH, G * DH)], wq_buf.at[j], wq_sem.at[j])
        wq_half = lambda k: pltpu.make_async_copy(wq_hbm.at[:, pl.ds(k * 256, 256)], wq_buf.at[0, :, pl.ds(k * 256, 256)], misc_sem.at[5 + k])
        hr = [(0, HA), (HA, H - HA)]
        k_cp = lambda j: pltpu.make_async_copy(k_hbm.at[pl.ds(*hr[j])], k_buf.at[pl.ds(*hr[j])], kv_sem.at[2 * j])
        v_cp = lambda j: pltpu.make_async_copy(v_hbm.at[pl.ds(*hr[j])], v_buf.at[pl.ds(*hr[j])], kv_sem.at[2 * j + 1])
        wr_cp = lambda: pltpu.make_async_copy(wr_hbm, wr_buf, misc_sem.at[0])
        wg_cp = lambda: pltpu.make_async_copy(wg_hbm, wg_buf, misc_sem.at[1])
        wu_cp = lambda: pltpu.make_async_copy(wu_hbm, wu_buf, misc_sem.at[2])
        wd_cp = lambda: pltpu.make_async_copy(wd_hbm, wd_buf, misc_sem.at[3])
        wo_cp = lambda: pltpu.make_async_copy(wo_hbm, wo_buf, misc_sem.at[4])

        cur = []
        def mark(name):
            if not P.get("PROF"): return
            if cur: cur.pop().__exit__(None, None, None)
            if name:
                cm = jax.named_scope(name); cm.__enter__(); cur.append(cm)
        mark("p0_wait_x0")
        cps = dict(x0=lambda: x_cp(0), x1=lambda: x_cp(1), x2=lambda: x_cp(2), x3=lambda: x_cp(3), x4=lambda: x_cp(4), wr=wr_cp,
                   q0=lambda: wq_cp(0), qa=lambda: wq_half(0), qb=lambda: wq_half(1), q1=lambda: wq_cp(1))
        def start(stage):
            for nm in P["DS"][stage].split():
                if nm == "qr":
                    for j in range(2, P['NJ'] * P['MB'] // NX + 1): wq_cp(j).start()
                else: cps[nm]().start()
        start(0)
        z_ref[0] = 0
        z_ref[1] = 0

        def store_q(j, g, i, q, BX=BX):
            q = (q * (DH ** -0.5 * LOG2E)).astype(bf16)
            r0 = pl.multiple_of(QB + (j * G + g) * (S // 2) + i * (BX // 2), 32)
            w_buf[pl.ds(r0, BX // 2), :] = pltpu.bitcast(q, f32)
            return q

        def qproj(j, i, after=None):
            xn = xn_buf[pl.ds(i * BX if isinstance(i, int) else pl.multiple_of(i * BX, BX), BX), :]
            if after is not None:
                head = jnp.where(lane > j + 1000, after, pltpu.bitcast(xn[:16, :128], f32))
                xn = jnp.concatenate([jnp.concatenate([pltpu.bitcast(head, bf16), xn[:16, 128:]], axis=1), xn[16:]], axis=0)
            q = jnp.dot(xn, wq_buf[j], preferred_element_type=f32)
            return [store_q(j, g, i, q[:, g * DH:(g + 1) * DH]) for g in range(G)]

        HK = 256
        A_SUMS = {1: (0, 0, 1, 1, 1), 2: (1, 0, 1, 1, 1), 5: (0, 0, 0, 1, 1), 6: (1, 0, 0, 0, -1), 7: (0, 1, 1, 1, -1)}
        B_SUMS = {1: (0, 0, 1, 1, 1), 3: (0, 1, 1, 1, -1), 4: (1, 0, 0, 0, -1), 6: (0, 0, 0, 1, 1), 7: (1, 0, 1, 1, 1)}
        def combine(get, spec):
            a, b = get(*spec[:2]).astype(f32), get(*spec[2:4]).astype(f32)
            return (a + b if spec[4] > 0 else a - b).astype(bf16)
        def strassen(j, p, sums, after=None):
            st_ = isinstance(p, int)
            xa = lambda r, k, w=HK: xn_buf[pl.ds((2 * p + r) * BX if st_ else pl.multiple_of((2 * p + r) * BX, BX), BX), pl.ds(k * HK, w)]
            wb = lambda k, c: wq_buf[j, pl.ds(k * HK, HK), pl.ds(c * HK, HK)]
            def m(i):
                if i in A_SUMS:
                    if i not in sums: sums[i] = combine(xa, A_SUMS[i])
                    a = sums[i]
                else:
                    a = xa(0, 0) if i == 3 else xa(1, 1)
                b = combine(wb, B_SUMS[i]) if i in B_SUMS else (wb(0, 0) if i == 2 else wb(1, 1))
                return jnp.dot(a, b, preferred_element_type=f32)
            def rest(r, after=None):
                a = xa(r, 2, 128)
                if after is not None:
                    head = jnp.where(lane > p + 1000, after, pltpu.bitcast(a[:16], f32))
                    a = jnp.concatenate([pltpu.bitcast(head, bf16), a[16:]], axis=0)
                e = jnp.dot(a, wq_buf[j, pl.ds(2 * HK, 128), :], preferred_element_type=f32)
                return e[:, :HK], e[:, HK:]
            def put(r, c, q):
                return [store_q(j, 2 * c + g, 2 * p + r, q[:, g * DH:(g + 1) * DH]) for g in range(2)]
            c11, c12 = rest(0, after); yield
            d = m(5); c11 = c11 - d; c12 = c12 + d; yield
            d = m(3); yield put(0, 1, c12 + d)
            c21, c22 = rest(1); c22 = c22 + d; yield
            d = m(2); c21 = c21 + d; c22 = c22 - d; yield
            d = m(4); c11 = c11 + d; yield put(1, 0, c21 + d)
            c11 = c11 + m(7); yield
            d = m(1); c22 = c22 + d; yield put(0, 0, c11 + d)
            yield put(1, 1, c22 + m(6))

        lane = lax.broadcasted_iota(i32, (8, 128), 1)
        sub = lax.broadcasted_iota(i32, (8, 128), 0)

        def layernorm(r0, n):
            x = x_buf[pl.ds(r0, n), :].astype(f32)
            m = jnp.sum(x, axis=-1, keepdims=True)
            yield
            m = m * (1.0 / D)
            mb = rb(m)
            xc = x - mb
            dm = m - mb
            var = jnp.sum(xc * xc, axis=-1, keepdims=True)
            if P["XB"]: xb = xc.astype(bf16)
            yield
            var = jnp.broadcast_to(var * (1.0 / D) - dm * dm, (n, 128))
            if P["DENSE"]:
                dense = var[:8]
                for t in range(1, n // 8):
                    dense = jnp.where(lane == t, var[t * 8:(t + 1) * 8], dense)
                inv = 1.0 / rb(jnp.sqrt(rb(rb(jnp.maximum(dense, 0.0)) + EPS)))
                inv = jnp.concatenate([jnp.broadcast_to(inv[:, t:t + 1], (8, 128)) for t in range(n // 8)], axis=0)
                yield
            else:
                inv = 1.0 / rb(jnp.sqrt(rb(rb(jnp.maximum(var, 0.0)) + EPS)))
            xr_ = xb.astype(f32) if P["XB"] else rb(xc)
            xn = jnp.concatenate([xr_[:, w * 128:(w + 1) * 128] * inv for w in range(D // 128)], axis=1).astype(bf16)
            xn_buf[pl.ds(r0, n), :] = xn
            x_buf[pl.ds(S + r0, n), :] = xn
            yield "stored"

        ln = dict(next=0, done=0, live=[])
        def layernorm_upto(row, avail):
            while ln["done"] < row:
                for gen in list(ln["live"]):
                    st_ = next(gen, "end")
                    if st_ == "stored": ln["done"] += LN
                    if st_ == "end": ln["live"].remove(gen)
                if ln["next"] < avail:
                    gen = layernorm(ln["next"], LN); next(gen)
                    ln["live"].append(gen); ln["next"] += LN

        x_cp(0).wait()
        start(1)
        wr_cp().wait()
        mark('p1_ln0')
        layernorm_upto(BX, BX)
        mark('p2_wait_wq0')
        (wq_half(0) if P['HQ'] else wq_cp(0)).wait()
        start(2)
        starts = [r[0] // BX for r in xr]
        for i in range(NX):
            if i + 1 in starts:
                n_ = starts.index(i + 1)
                mark(f'p3_wait_x{n_}')
                start(2 + n_)
                x_cp(n_).wait()
                avail = xr[n_][0] + xr[n_][1]
            if i + 1 in starts: mark(f'p3_q{i}')
            def half(i, k):
                q = jnp.dot(xn_buf[pl.ds(i * BX, BX), :], wq_buf[0, :, pl.ds(k * 256, 256)], preferred_element_type=f32)
                for g in range(2): store_q(0, 2 * k + g, i, q[:, g * DH:(g + 1) * DH])
            if P["HQ"] and i == 0:
                half(0, 0); layernorm_upto(2 * BX, avail); half(1, 0)
                continue
            if P["HQ"] and i == 1:
                wq_half(1).wait(); half(0, 1); half(1, 1)
            else:
                qs = qproj(0, i)
            if i + 1 < NX:
                layernorm_upto((i + 2) * BX, avail)
        for gen in ln["live"]:
            for _ in gen: pass

        NJ, MB = P["NJ"], P["MB"]
        JL = NJ * MB // NX
        RR = -(-S // (NJ * 256)) * 256
        row16 = lax.broadcasted_iota(i32, (16, D), 0)
        def top_k(rds):
            keys = []
            for t in range(NJ):
                r = rb(rds[t])
                r = jnp.where(r == 0.0, 0.0, r)
                b = lax.shift_right_logical(pltpu.bitcast(r, i32), 16)
                k16 = jnp.where(b >= 0x8000, 0xFFFF - b, b + 0x8000)
                k16 = jnp.where(r != r, 0, k16)
                tok = min(t * RR, S - RR) + lane * 8 + sub
                keys.append(pltpu.bitcast(jnp.where(lane < RR // 8, 0x20000000 + k16 * 2048 + (2047 - tok), 0), f32))
            ktop = jnp.zeros((8, 128), i32)
            x_sel = jnp.zeros((16, D), f32)
            for c in range(C):
                mx = functools.reduce(jnp.maximum, keys)
                mx = jnp.max(jnp.max(mx, axis=0, keepdims=True), axis=1, keepdims=True)
                mxb = jnp.broadcast_to(mx, (8, 128))
                keys = [jnp.where(kk == mxb, 0.0, kk) for kk in keys]
                mi = pltpu.bitcast(mxb, i32)
                ktop = jnp.where(sub == c, mi, ktop)
                idx = 2047 - (mi[0, 0] & 2047)
                base = pl.multiple_of(idx & -16, 16)
                blk = xn_buf[pl.ds(base, 16), :].astype(f32)
                rowv = jnp.sum(jnp.where(row16 == idx - base, blk, 0.0), axis=0, keepdims=True)
                x_sel = jnp.where(row16 == c, rowv, x_sel)
            return ktop, x_sel
        mark('p5_1b')
        def p1_body(jj, carry):
            @pl.when(jj == 1)
            def _():
                k_cp(0).start(); v_cp(0).start()
            @pl.when(jj == 0)
            def _():
                for j in range(1, JL): wq_cp(j).wait()
                for j in range(JL + 1, NG): wq_cp(j).start()
                wg_cp().start(); wu_cp().start(); wd_cp().start(); wo_cp().start()
                wq_cp(JL).wait()
            wr = wr_buf[...].astype(f32).reshape(1, D)
            r0 = pl.multiple_of(jnp.minimum(jj * RR, S - RR), 256)
            rd = jnp.zeros((8, 128), f32)
            RP = P["RP"]
            never = lax.broadcasted_iota(i32, (8, 128), 1) > jj + 1000
            after = None
            piece = 0
            for n_ in range(MB // 2):
                if n_ % JL == 0: sums = {}
                for qs in strassen(1 + n_ % JL, jj * (MB // 2 // JL) + n_ // JL, sums, after if n_ == P["R0"] else None):
                    if qs is None or piece * RP == RR: continue
                    tok = pltpu.bitcast(qs[0][:16], f32)
                    for t in range(piece * RP // 16, (piece + 1) * RP // 16):
                        r = 0.0
                        for w in range(KT):
                            xb = pltpu.bitcast(xn_buf[pl.ds(r0 + t * 16, 16), pl.ds(w * 128, 128)], f32)
                            d_ = pltpu.bitcast(jnp.where(never, tok, xb), bf16).astype(f32) * wr[:, w * 128:(w + 1) * 128]
                            r = d_ if w == 0 else r + d_
                        r = jnp.broadcast_to(jnp.sum(r, axis=-1, keepdims=True), (16, 128))
                        rd = jnp.where(lane == 2 * t, r[:8], jnp.where(lane == 2 * t + 1, r[8:], rd))
                    piece += 1
                    if piece * RP == RR:
                        rds = [jnp.where(jnp.full((8, 128), jj) == t, rd, carry[0][t]) for t in range(NJ)]
                        ktop, x_sel = top_k(rds)
                        after = functools.reduce(lax.add, [x_sel[:8, w * 128:(w + 1) * 128] for w in range(KT)])
            return rds, ktop, x_sel
        zero = jnp.zeros((8, 128), f32)
        _, ktop, x_sel = lax.fori_loop(0, NJ, p1_body, ([zero] * NJ, jnp.zeros((8, 128), i32), jnp.zeros((16, D), f32)))
        x_sel = x_sel[:8]

        mark('p6_wait')
        for j in range(JL + 1, NG): wq_cp(j).wait()
        wg_cp().wait(); wu_cp().wait(); wd_cp().wait()
        k_cp(0).wait(); v_cp(0).wait(); wo_cp().wait()
        mark('p7_1c')
        k16 = lax.shift_right_logical(ktop - 0x20000000, 11)
        b = jnp.where(k16 >= 0x8000, k16 - 0x8000, 0xFFFF - k16)
        r_sel = pltpu.bitcast(lax.shift_left(b, 16), f32)[:, :1]
        xs = x_sel.astype(bf16)
        acc = {}
        def accum(key, d):
            acc[key] = acc[key] + d if key in acc else d
        BC = P["BC"]
        def q_tile(j, i, g, k):
            accum((j, i, g), jnp.dot(xn_buf[pl.ds(i * BC, BC), pl.ds(k * 128, 128)], wq_buf[j, pl.ds(k * 128, 128), pl.ds(g * DH, DH)], preferred_element_type=f32))
            if k == KT - 1:
                store_q(j, g, i, acc.pop((j, i, g)), BC)
        fr = [(f0, min(128, F - f0)) for f0 in range(0, F, 128)]
        def up_tile(name, w, f, k):
            accum((name, f), lax.dot_general(xs[:, k * 128:(k + 1) * 128], w[pl.ds(*fr[f]), pl.ds(k * 128, 128)], NT, preferred_element_type=f32))
        def down_tile(f, n):
            if n == 0:
                a = rb(acc.pop(("g", f)))
                acc["h"] = (rb(a * sigmoid(a)) * rb(acc.pop(("u", f)))).astype(bf16)
            accum(("y", n), jnp.dot(acc["h"], wd_buf[pl.ds(*fr[f]), pl.ds(n * 128, 128)], preferred_element_type=f32))
        part = functools.partial
        f_tiles = [part(up_tile, nm, w, f, k) for f in range(len(fr)) for nm, w in (("g", wg_buf), ("u", wu_buf)) for k in range(KT)]
        f_tiles += [None] * (4 * P["FG"])
        f_tiles += [part(down_tile, f, n) for f in range(len(fr)) for n in range(KT)]
        sums = [{} for p in range(NX // 2)]
        rounds = (_ for p in range(NX // 2) for j in range(JL + 1, NG) for _ in strassen(j, p, sums[p]))
        for rnd, _ in enumerate(rounds):
            if rnd >= P["F0"] and rnd % P['FS'][0] not in P['FS'][1:]:
                for fn_ in f_tiles[:4]:
                    if fn_ is not None: fn_()
                f_tiles = f_tiles[4:]
        assert not f_tiles
        y = rb(jnp.concatenate([acc.pop(("y", n)) for n in range(KT)], axis=1))
        z = rb(x_sel + rb(y * rb(sigmoid(r_sel))))
        for c in range(C):
            idx = 2047 - (ktop[c, 0] & 2047)
            at = pl.ds(S + pl.multiple_of(idx & -16, 16), 16)
            x_buf[at, :] = jnp.where(row16 == (idx & 15), z[c:c + 1, :], x_buf[at, :].astype(f32)).astype(bf16)

        k_cp(1).start(); v_cp(1).start()
        if P['KT']:
            for w in range(KC // 128):
                w_buf[pl.ds(32 + 64 * w, 64), :] = pltpu.bitcast(k_buf[0, pl.ds(w * 128, 128), :].T, f32)
        mark('p8_att')
        M = P["M"]; PG = NB // M
        OD = P["OD"]
        def out_cp(blk0, k):
            rows = pl.ds((blk0 + OD[k - 1]) * BQ, (OD[k] - OD[k - 1]) * BQ)
            return pltpu.make_async_copy(out_buf.at[rows], out_hbm.at[rows], out_sem.at[blk0 + k - 1])
        z0, z1 = (pl.multiple_of(z_ref[i], 32) for i in range(2))
        def att_body(t, _):
            @pl.when(t == HA // G * PG - 1)
            def _():
                if 'k' not in P['SKIP']: k_cp(1).wait(); v_cp(1).wait()
            grp = lax.shift_right_logical(t, PG.bit_length() - 1)
            def out_start(blk0, k):
                @pl.when(grp == NG - 1)
                def _():
                    out_cp(blk0, k).start()
            attention_body(grp, (t & (PG - 1)) * M, z0, z1, w_buf, s_bufs, a_bufs, k_buf, v_buf, wo_buf, x_buf, y_buf, out_buf, u_buf, out_start, jnp.minimum(lax.shift_right_logical(t + 1, PG.bit_length() - 1), NG - 1) * G, pl.multiple_of(t * (S // (NG * PG)), 16), P)
        lax.fori_loop(P.get('T0', 0), NG * PG, att_body, None)
        mark('pa_wait_out')
        for blk0 in range(0, NB, M):
            for k in range(1, len(OD)):
                out_cp(blk0, k).wait()
        mark(None)

    @jax.jit
    def fn(A_x, A_k_cache, A_v_cache, A_wq, A_wo, B_x, B_w_r, B_w_gate, B_w_up, B_w_down):
        any_spec = pl.BlockSpec(memory_space=pl.ANY)
        s_shape = pltpu.VMEM((L * BQ * (KC // 128) + 32, 128), f32)
        out = pl.pallas_call(
            kernel,
            in_specs=[any_spec] * 9,
            out_specs=any_spec,
            out_shape=jax.ShapeDtypeStruct((S, D), bf16),
            scratch_shapes=[
                pltpu.VMEM((2 * S + 64, D), bf16), pltpu.VMEM((S, D), bf16),
                pltpu.VMEM((GB, DH), f32), pltpu.VMEM((D // 128 * S + 32, DH), f32), pltpu.VMEM((640, 256), f32),
                pltpu.VMEM((H, SK, DH), bf16), pltpu.VMEM((H, SK, DH), bf16),
                pltpu.VMEM((NG, D, G * DH), bf16), pltpu.VMEM((NG, G * DH, D), bf16),
                pltpu.VMEM((F, D), bf16), pltpu.VMEM((F, D), bf16), pltpu.VMEM((F, D), bf16),
                pltpu.VMEM((S, D), bf16), pltpu.SMEM((2,), i32),
                pltpu.SemaphoreType.DMA((len(P['XA']) - 1,)), pltpu.SemaphoreType.DMA((NG,)), pltpu.SemaphoreType.DMA((4,)),
                pltpu.SemaphoreType.DMA((7,)), pltpu.SemaphoreType.DMA((NB,)),
            ] + [s_shape] * P['NSB'] + [pltpu.VMEM((3 * BQ, 128), f32)] * P['NAB'] + [pltpu.VMEM((D,), bf16)],
            compiler_params=pltpu.CompilerParams(vmem_limit_bytes=120 * 1024 * 1024, flags=flags),
            name="fused_kernel",
        )(A_x.reshape(S, D), A_k_cache.reshape(H, SK, DH), A_v_cache.reshape(H, SK, DH), A_wq, A_wo.reshape(NG, G * DH, D),
          B_w_r, B_w_gate.T, B_w_up.T, B_w_down)
        return out.reshape(1, S, D)
    return fn


_impl = make()


@jax.jit
def pallas_recurrent_scan__mha_block_cached__moe_arch_mod__prompt_kernel(
    A_x, A_k_cache, A_v_cache, A_wq, A_wo, B_x, B_w_r, B_w_gate, B_w_up, B_w_down
):
    return _impl(A_x, A_k_cache, A_v_cache, A_wq, A_wo, B_x, B_w_r, B_w_gate, B_w_up, B_w_down)
```

```python
import functools
import numpy as np
import jax
import jax.numpy as jnp
from jax import lax
import jax.experimental.pallas as pl
import jax.experimental.pallas.tpu as pltpu

S, D, H, DH, SK, F, C = 2048, 640, 32, 128, 2048, 1728, 8
LOG2E = 1.4426950408889634
EPS = float(np.asarray(1e-5, dtype=jnp.bfloat16))
f32, bf16, i32 = jnp.float32, jnp.bfloat16, jnp.int32
NT = (((1,), (1,)), ((), ()))


def rb(x):
    return x.astype(bf16).astype(f32)


def sigmoid(x):
    return 1.0 / (1.0 + jnp.exp2(x * (-LOG2E)))


PRODS = [
    (((1, 1, 1),), ((0, 0, 1), (1, 0, 1)), ((0, 0, -1), (1, 0, 1))),
    (((0, 0, 1),), ((0, 1, 1), (1, 1, 1)), ((0, 1, 1), (1, 1, -1))),
    (((1, 0, 1), (1, 1, -1)), ((0, 0, 1),), ((1, 0, 1), (1, 1, 1))),
    (((0, 1, 1), (0, 0, -1)), ((1, 1, 1),), ((0, 0, 1), (0, 1, 1))),
    (((0, 1, 1), (1, 1, 1)), ((1, 0, 1), (1, 1, -1)), ((0, 0, 1),)),
    (((0, 0, 1), (1, 1, 1)), ((0, 0, 1), (1, 1, 1)), ((0, 0, 1), (1, 1, 1))),
    (((0, 0, 1), (1, 0, 1)), ((0, 1, 1), (0, 0, -1)), ((1, 1, 1),)),
]
VROW = {(0, 0): 1, (1, 1): 0, (0, 1): 7, (1, 0): 8}
def signed_sum(get, terms):
    v = get(*terms[0][:2])
    for t in terms[1:]: v = v + get(*t[:2]) if t[2] > 0 else v - get(*t[:2])
    return v

STEPS = [
    ("e", 0, [(0, 4, 1)]),
    (((0, 0, 1), (0, 1, 1)), (1, 1), [(0, 0, -1), (0, 2, 1)]),
    (((1, 0, 1), (1, 1, 1)), (0, 0), [(1, 0, 1), (1, 2, -1)]),
    (((0, 0, 1),), 0, [(0, 2, 1), (1, 2, 1)]),
    (((1, 1, 1),), 1, [(0, 0, 1), (1, 0, 1)]),
    (((0, 1, 1), (1, 1, -1)), 2, [(0, 0, 1)]),
    (((0, 0, 1), (1, 1, 1)), 3, [(0, 0, 1), (1, 2, 1)]),
    (((1, 0, 1), (0, 0, -1)), 4, [(1, 2, 1)]),
    ("e", 1, [(1, 4, 1)]),
]
U_SUMS = [((0, 1, 1), (1, 1, -1)), ((1, 0, 1), (0, 0, -1)), ((1, 0, 1), (1, 1, 1)), ((0, 0, 1), (1, 1, 1)), ((0, 0, 1), (0, 1, 1))]

def attention_body(grp, qh, gate_row, z0, z1, w_buf, s_bufs, u_bufs, c_bufs, t_bufs, k_buf, v_buf, wo_buf, x_buf, y_buf, out_buf, ws_buf, out_start, P):
    KM = P['KM']; n = 8; PD = P["PD"]; KT = D // 128; R = 8
    heads = [grp * 4 + a % 4 for a in range(n)]
    qrows = [1 + grp * 16 + qh * 2 + a % 4 * 4 + a // 4 for a in range(n)]
    row0 = pl.multiple_of(qh * 1024, 1024)
    first_grp = lax.broadcasted_iota(i32, (16, 128), 0) + grp * 16 < 16
    dots = []; pend = [("op", bp, k) for bp in range(2) for k in range(9)]; np_ = 0
    for hp in range(2 * n + P['LAG']):
        for c in range(8):
            if hp < 2 * n and c % KM == 0: dots += [("qk", hp // 2, 8 * (hp % 2) + c + e) for e in range(KM)]
            if hp >= P['LAG'] and c < 7: dots.append(("pv", (hp - P['LAG']) // 2, 7 * ((hp - P['LAG']) % 2) + c))
            if hp >= 9 + P['LAG'] and c < 7:
                np_ += 1
                while pend and 18 - len(pend) < np_ * P["OR"]: dots.append(pend.pop(0))
    dots += pend + [("op", bp, k) for bp in range(2, 4) for k in range(9)]
    start = {d: 8 * i for i, d in enumerate(dots)}
    ev = []; val = {}
    def add(slot, prio, fn): ev.append((slot, prio, len(ev), fn))
    sb = lambda a, p: s_bufs[(2 * a + p) % len(s_bufs)]
    ub = lambda a, p: u_bufs[(2 * a + p) % len(u_bufs)]
    cb = lambda a, p: c_bufs[(2 * a + p) % len(c_bufs)]
    tb = lambda a: t_bufs[a % 4]
    tokb = lambda: pltpu.bitcast(val['tok'], bf16)
    y0, y1 = lax.shift_right_logical(z0, 6), lax.shift_right_logical(z1, 6)
    def ldb(ref, r0, n_, blk=0): return pltpu.bitcast(ref.bitcast(f32)[y1 + blk, pl.ds(r0 // 2, n_ // 2), :], bf16)
    def stb(ref, r0, v, blk=0): ref[y0 + blk, pl.ds(r0, v.shape[0]), :] = v
    def tok(ref, r0, v=None): ref.bitcast(f32)[y0, pl.ds(r0 // 2, 8), :] = val['tok'] if v is None else v
    never8 = lax.broadcasted_iota(i32, (8, 128), 1) > z0 + 1000
    def res(d):
        if ("res", d) not in val:
            kind, a, c = d
            if kind == "qk" and c % KM:
                val["res", d] = res((kind, a, c - c % KM))[c % KM * 128:(c % KM + 1) * 128]
            elif kind == "qk":
                q = jnp.concatenate([val.pop(("q", d, j, r)) for j in range(4) for r in range(4)], axis=0)
                val["res", d] = lax.dot_general(jnp.concatenate([val.pop(("k", a, c * 8 + r)) for r in range(8 * KM)], axis=0), q, NT, preferred_element_type=f32)
            elif kind == "op":
                lhs, rhs, _ = STEPS[c]
                o = jnp.concatenate([val.pop(("ol", d, r)) for r in range(R)], axis=0)
                if lhs == "e": w_ = wo_buf[grp, :, pl.ds(512, 128)]
                elif isinstance(rhs, tuple): w_ = wo_buf[grp, pl.ds(rhs[0] * 256, 256), pl.ds(rhs[1] * 256, 256)]
                else: w_ = jnp.concatenate([ldb(ws_buf, (2 * rhs + u) * 256, 256) for u in range(2)], axis=1)
                val["res", d] = jnp.dot(o, w_, preferred_element_type=f32)
            else:
                lhs = jnp.concatenate([jnp.concatenate([val.pop(("t", d, w * 4 + r)) for r in range(4)], axis=0) for w in range(2)], axis=1)
                rhs = jnp.concatenate([val.pop(("u", d, k, r)) for k in range(8) for r in range(4)], axis=0)
                val["res", d] = jnp.dot(lhs, rhs, preferred_element_type=f32)
        return val["res", d]
    for d in dots:
        kind, a, c = d; j0 = start[d]
        if kind == "qk":
            for r in range(4 if c % KM == 0 else 0):
                def l_q(d=d, a=a, r=r):
                    if "tok" in val: tok(w_buf, 0)
                    for j in range(4): val["q", d, j, 3 - r] = ldb(w_buf, 128 * j + 32 * (3 - r), 32, qrows[a])
                add(j0 + r - P["QA"], 1, l_q)
            for r in range(8):
                def l_k(a=a, c=c, r=r):
                    if "tok" in val and r % P["KT"] == 0: k_buf.bitcast(f32)[y0 + H, pl.ds(0, 8), :] = val["tok"]
                    val["k", a, c * 8 + r] = ldb(k_buf, c * 128 + 16 * r, 16, heads[a])
                add(min(j0 + r - P["KA"], j0 - c % KM * 8 + PD - 1), 1, l_k)
                def s_res(d=d, a=a, c=c, r=r):
                    s = res(d)[16 * r:16 * r + 16]
                    for j in range(4):
                        t = s[:, j * 128:(j + 1) * 128]
                        sb(a, j // 2)[pl.ds(z0 + ((c * 8 + r) * 2 + j % 2) * 16, 16), :] = t
                        x = jnp.maximum(t[:8], t[8:])
                        if ("pend", j) in val: x = jnp.maximum(x, val.pop(("pend", j)))
                        if r % P["ON"] == P["ON"] - 1:
                            oldm = val.get(("m", a, j))
                            if oldm is None: m = x; l = jnp.ones_like(x)
                            else:
                                m = jnp.maximum(oldm, x)
                                l = jnp.exp2(x - m) + val["l", a, j] * jnp.exp2(oldm - m)
                            val["m", a, j] = m; val["l", a, j] = l
                            val["ltok", d, r] = l
                        else: val["pend", j] = x
                    val["tok"] = s[:8, 384:]
                add(j0 + r + PD, 0, s_res)
                if r % (P["ON"] * P["LT"]) == P["ON"] * P["LT"] - 1:
                    def s_lt(d=d, r=r): tok(w_buf, 16, val.pop(("ltok", d, r)))
                    add(j0 + r + PD + P["LS"], 0, s_lt)
            if c == 15:
              for j5 in range(4):
                def s_m(a=a, j=j5):
                    if True:
                        m, l = val.pop(("m", a, j)), val.pop(("l", a, j))
                        mm = jnp.max(m, axis=0, keepdims=True)
                        ll = jnp.broadcast_to(jnp.sum(l * jnp.exp2(m - mm), axis=0, keepdims=True), (8, 128))
                        sb(a, j // 2)[pl.ds(z0 + 4096 + 8 * (j % 2), 8), :] = mm + (0.5 * np.log2(SK) / np.log2(SK / (2 * P['ON']))) * jnp.log2(ll)
                add(j0 + 8 + PD + P["MD"] + P['MS'] * j5, 0, s_m)
        elif kind == "op":
            lhs, rhs, outs = STEPS[c]
            todo = []
            for b_, n0_, sign in outs:
                users = [k for k, st_ in enumerate(STEPS) if any(o_[:2] == (b_, n0_) for o_ in st_[2])]
                todo += [(2 * a + b_, n0_ + u, u, sign, c == users[0], c == users[-1]) for u in range(1 if lhs == "e" else 2)]
            assert j0 - P["QP"] > start["pv", a // 2 * 4 + 3, a % 2 * 7 + 6] + 8 + PD + 5 + P["FD"]
            for r in range(R):
                j = j0 + r
                def l_o(d=d, bp=a, lhs=lhs, rhs=rhs, r=r):
                    if r % P["QO"] == 0: tok(w_buf, 0)
                    get = lambda b_, u: ldb(w_buf, (bp % 2 * 2 + b_) * 128 + 16 * r, 16, qrows[bp // 2 * 4 + u])
                    if lhs == "e": tiles = [get(rhs, u) for u in range(4)]
                    elif len(lhs) == 1: tiles = [get(lhs[0][0], 2 * lhs[0][1] + u) for u in range(2)]
                    else: tiles = [signed_sum(lambda b_, k: get(b_, 2 * k + u).astype(f32), lhs).astype(bf16) for u in range(2)]
                    val["ol", d, r] = jnp.concatenate(tiles, axis=1)
                add(j - P["QP"], 1, l_o)
                def l_y(d=d, todo=todo, r=r):
                    if r % P["XT"] == 0 and any(t_[5] for t_ in todo): x_buf[pl.ds(z0 + 2 * S, 16), pl.ds(0, 128)] = tokb()
                    for b_, n_, u, sign, is_first, is_last in todo:
                        y = y_buf[pl.ds(z1 + row0 + (n_ * S + b_ * 128 + 16 * r), 16), :]
                        val["y", d, r, b_, n_] = jnp.where(first_grp, 0.0, y) if is_first else y
                        if is_last:
                            val["xg", d, r, b_, n_] = [x_buf[pl.ds(z1 + row0 + (k * S + b_ * 128 + 16 * r), 16), pl.ds(n_ * 128, 128)].astype(f32) for k in range(2)]
                add(j + PD - P["LY"], 1, l_y)
                def s_y(d=d, todo=todo, c=c, bp=a, r=r):
                    for b_, n_, u, sign, is_first, is_last in todo:
                        e = res(d)[16 * r:16 * r + 16, u * 128:(u + 1) * 128]
                        y = val.pop(("y", d, r, b_, n_))
                        y = y + e if sign > 0 else y - e
                        y_buf[pl.ds(z0 + row0 + (n_ * S + b_ * 128 + 16 * r), 16), :] = y
                        if is_last:
                            x, gate = val.pop(("xg", d, r, b_, n_))
                            out_buf[pl.ds(row0 + b_ * 128 + 16 * r, 16), pl.ds(n_ * 128, 128)] = (x + y * gate).astype(bf16)
                    val["tok"] = y[:8]
                    if r == R - 1 and c in (6, 8): out_start(2 * bp + (c == 8))
                add(j + PD - P["PO"], 0, s_y)
        else:
            p, i = divmod(c, 7)
            for r in range(8):
                def l_u(d=d, a=a, p=p, i=i, r=r):
                    if r % P["UT"] == 0: tok(ub(a, p), 7 * 1024)
                    w, rr = r // 4, 3 - r % 4
                    for k in range(4): val["u", d, 4 * w + k, rr] = ldb(ub(a, p), (i * 8 + 4 * w + k) * 128 + 32 * rr, 32)
                add(j0 + r - P["UA"], 1, l_u)
                def l_t(d=d, a=a, i=i, r=r):
                    w, rr = divmod(r, 4)
                    if r % P['TT'] == 0: t_bufs[1].bitcast(f32)[y0 + 8, pl.ds(0, 8), :] = val['tok']
                    val["t", d, r] = jnp.concatenate([ldb(t_bufs[1], (i * 8 + 4 * w + k) * 64 + rr * 16, 16, (grp & 1) * 4 + a % 4) for k in range(4)], axis=1)
                add(j0 + r - P["TA"], 1, l_t)
            for r in range(4):
                todo = []
                for dh, qt, sign in PRODS[i][2]:
                    users = [k for k, pr in enumerate(PRODS) if any(o[:2] == (dh, qt) for o in pr[2])]
                    todo.append((dh, qt, sign, i == users[0], i == users[-1]))
                at = lambda z, dh, qt, r: pl.ds(z + qt * 128 + dh * 64 + 16 * r, 16)
                def l_c(d=d, a=a, p=p, todo=todo, r=r):
                    for dh, qt, sign, first, last in todo:
                        if not first: val["c", d, r, dh, qt] = cb(a, p)[at(z1, dh, qt, r), :]
                        if last: val["rl", d, r, dh, qt] = cb(a, p)[pl.ds(z1 + 256 + qt * 8, 8), :]
                add(j0 + 4 + r + PD - P["LC"], 1, l_c)
                def s_c(d=d, a=a, p=p, todo=todo, r=r):
                    x = res(d)[16 * r:16 * r + 16]
                    for dh, qt, sign, first, last in todo:
                        if first: y = x if sign > 0 else -x
                        else:
                            y = val.pop(("c", d, r, dh, qt)); y = y + x if sign > 0 else y - x
                        if last: stb(ub(a, p), 7 * 1024 + 64 + qt * 128 + dh * 64 + 16 * r, (y * jnp.tile(val.pop(("rl", d, r, dh, qt)), (2, 1))).astype(bf16))
                        else: cb(a, p)[at(z0, dh, qt, r), :] = y
                    val["tok"] = x[:8]
                add(j0 + 4 + r + PD, 0, s_c)
            if i == 6:
                for qt in range(2):
                    def l_f(a=a, p=p, qt=qt):
                        val["o", a, p, qt] = ldb(ub(a, p), 7 * 1024 + 64 + qt * 128, 128).T
                    add(j0 + 8 + PD + 1 + 4 * qt, 1, l_f)
                    def s_f(a=a, p=p, qt=qt): stb(w_buf, (2 * p + qt) * 128, val.pop(("o", a, p, qt)), qrows[a])
                    add(j0 + 8 + PD + 1 + 4 * qt + P["FD"], 0, s_f)
    prev_end = 0
    heavy = {start[d] + PD + r: P['WH'] if d[0] == 'qk' else P['WP'] for d in dots if d[0] != "pv" for r in range(8)}
    wt = lambda j: P['W0'] if j < start['pv', 0, 0] else heavy.get(j - P["WO"], 1.0)
    cum = np.concatenate([[0], np.cumsum([wt(j) for j in range(8 * len(dots))])])
    NU_ = len(u_bufs)
    lo = [max(start["qk", g // 2, 15] + 8 + PD + P["MD"] + 1 + P['MS'] * (g % 2 * 2 + 1), start["pv", (g - NU_) // 2, (g - NU_) % 2 * 7 + 6] + 8 if g >= NU_ else 0) for g in range(2 * n)]
    hi = [start["pv", g // 2, g % 2 * 7] - P["UA"] - P["PS"] - 1 for g in range(2 * n)]
    b = [cum[lo[0]]] + [cum[h] for h in hi]
    for _ in range(200):
        for g in range(1, 2 * n): b[g] = min(max((b[g - 1] + b[g + 1]) / 2, cum[lo[g]]), cum[hi[g - 1]])
    for a in range(n):
        for p in range(2):
            for e in range(64):
                k, rr = divmod(e, 8); g = 2 * a + p
                slot = int(np.searchsorted(cum, b[g] + (b[g + 1] - b[g]) * (e + 0.5) / 64)) - 1
                def l_p(a=a, p=p, k=k, rr=rr):
                    sb(a, p)[pl.ds(z0 + 4096 + 16, 8), :] = jnp.where(never8, val.pop("utok"), val["tok"]) if "utok" in val else val["tok"]
                    pt = {}
                    for qt in range(2):
                        mb = sb(a, p)[pl.ds(z1 + 4096 + 8 * qt, 8), :]
                        mb = jnp.concatenate([mb, mb], axis=0)
                        for kh in range(2):
                            pt[kh, qt] = jnp.exp2(sb(a, p)[pl.ds(z1 + (((kh * 8 + k) * 8 + rr) * 2 + qt) * 16, 16), :] - mb)
                    us = [signed_sum(lambda *ix: pt[ix], pr[1]) for pr in PRODS]
                    val["up", a, p, k, rr] = [u.astype(bf16) for u in us]
                    for qt in range(2):
                        x = us[qt][:8] + us[qt][8:]
                        val["ls", a, p, qt] = val["ls", a, p, qt] + x if ("ls", a, p, qt) in val else x
                    val['ut', a, p, k, rr] = val["ls", a, p, 1]
                add(slot, 1, l_p)
                def s_p(a=a, p=p, k=k, rr=rr):
                    u = val.pop(("up", a, p, k, rr))
                    for i in range(7): stb(ub(a, p), (i * 8 + k) * 128 + rr * 16, u[i])
                    val['utok'] = val.pop(('ut', a, p, k, rr))
                add(slot + P["PS"], 0, s_p)
            def s_l(a=a, p=p):
                for qt in range(2):
                    l = jnp.broadcast_to(jnp.sum(val.pop(("ls", a, p, qt)), axis=0, keepdims=True), (8, 128))
                    r0 = pl.reciprocal(l, approx=True)
                    cb(a, p)[pl.ds(z0 + 256 + qt * 8, 8), :] = r0 * (2.0 - l * r0)
            add(slot + P["PS"] + 2, 0, s_l)
    nxt = jnp.minimum(grp + 1, H // 4 - 1)
    for hh in range(2):
        head = nxt * 4 + 2 * qh + hh; tn = t_bufs[2]; blk = ((grp + 1) & 1) * 4 + 2 * qh + hh
        for k in range(8):
            sp = (P['VW'][1] - P['VW'][0]) / 16; j = P['VW'][0] + sp * (hh * 8 + k)
            for kh in range(2):
                def l_v(head=head, hh=hh, k=k, kh=kh):
                    v_buf.bitcast(f32)[y0 + H, pl.ds(0, 8), :] = val["tok"]
                    val["vt", hh, k, kh] = ldb(v_buf, (kh * 8 + k) * 128, 128, head).T
                add(j + sp / 2 * kh, 2, l_v)
                def s_v(hh=hh, k=k, kh=kh):
                    stb(tn, kh * 128, val.pop(("vt", hh, k, kh)))
                add(j + sp / 2 * kh + P["FD"], 0, s_v)
            for rr in range(4):
                def l_s(hh=hh, k=k, rr=rr):
                    tok(tn, 256)
                    vt = {(dh, kh): ldb(tn, kh * 128 + dh * 64 + 16 * rr, 16).astype(f32) for dh in range(2) for kh in range(2)}
                    val["ts", hh, k, rr] = [signed_sum(lambda *ix: vt[ix], pr[0]) for pr in PRODS]
                add(j + sp / 2 + 1 + P["FD"] + sp / 9 * rr, 2, l_s)
                def s_s(hh=hh, k=k, rr=rr, blk=blk):
                    for i, x in enumerate(val.pop(("ts", hh, k, rr))): stb(t_bufs[1], (i * 8 + k) * 64 + 16 * rr, x.astype(bf16), blk)
                    tok(w_buf, 32, x[:8])
                add(j + sp / 2 + 3 + P["FD"] + sp / 9 * rr, 0, s_s)
    j0 = P['WS']
    for k, terms in enumerate(U_SUMS):
        for r in range(16):
            def s_u(k=k, terms=terms, r=r):
                for u in range(2):
                    get = lambda kh, nh: pltpu.bitcast(jnp.where(never8, val["tok"], pltpu.bitcast(wo_buf[grp, pl.ds(kh * 256 + 16 * r, 16), pl.ds(nh * 256 + u * 128, 128)], f32)), bf16).astype(f32)
                    x = signed_sum(get, terms)
                    stb(ws_buf, (2 * k + u) * 256 + 16 * r, x.astype(bf16))
                val["wtok", k, r] = x[:8]
            add(j0 + (k * 16 + r) * P["UD"], 2, s_u)
            def s_ut(k=k, r=r): tok(w_buf, 48, val.pop(("wtok", k, r)))
            add(j0 + (k * 16 + r) * P["UD"] + 3, 0, s_ut)
    j0 = P['GS']
    for r in range(8):
        for w in range(KT):
            def l_g(r=r, w=w):
                x_buf[pl.ds(z0 + 2 * S, 16), pl.ds(0, 128)] = tokb()
                xn = x_buf[pl.ds(z1 + gate_row + (S + 16 * r), 16), pl.ds(w * 128, 128)].astype(f32)
                val["g", r, w] = xn * sigmoid(xn)
            add(j0 + (r * KT + w) * P['GD'], 2, l_g)
            def s_g(r=r, w=w):
                g_ = val.pop(("g", r, w))
                x_buf[pl.ds(z0 + gate_row + (S + 16 * r), 16), pl.ds(w * 128, 128)] = g_.astype(bf16)
                tok(w_buf, 64, g_[8:])
            add(j0 + (r * KT + w) * P['GD'] + 4, 0, s_g)
    ev.sort(key=lambda e: e[:3])
    for e in ev: e[3]()

def make(flags=None, **kw):
    P = dict(KM=2, KA=3, KT=8, MS=8, W0=0.4, LAG=5, WH=0.8, WP=0.5, WO=-2, VW=(330, 1300), WS=14, GD=8, GS=1300, PD=10, QA=8, ON=8, LT=1, LS=4, MD=6, UA=8, UT=4, TT=8, TA=2, LC=3, FD=15, PS=3, NS=7, NUB=4, NC=8,
             OR=0.55, QP=3, QO=1, XT=2, LY=4, PO=1, UD=1.6,
             BQ=128, BX=256, G=4, BO=256, HA=4, SKIP="", DS=('x0 wr q0 x1', 'x2', 'x3', 'x4', '', 'q1 qr', ''), NJ=2, HQ=0, MB=20, RP=32, R0=9,
             F0=0, FG=8, FS=(9, 7), XB=1, DENSE=1, LN=64, XA=(0, 1, 2, 4, 6, 8), BC=256)
    P.update(kw)
    BQ, BX, G, BO, HA = (P[k] for k in "BQ BX G BO HA".split())
    NB = S // BQ; NX = S // BX; NG = H // G; NO = S // BO

    def kernel(x_hbm, k_hbm, v_hbm, wq_hbm, wo_hbm, wr_hbm, wg_hbm, wu_hbm, wd_hbm, out_hbm,
               x_buf, xn_buf, w_buf, y_buf, u_buf, k_buf, v_buf, wq_buf, wo_buf, wg_buf, wu_buf, wd_buf, out_buf, z_ref,
               x_sem, wq_sem, kv_sem, misc_sem, out_sem, *bufs):
        o1 = P['NS']; o2 = o1 + P['NUB']; o3 = o2 + P['NC']
        s_bufs, u_bufs, c_bufs, t_bufs, wr_buf = bufs[:o1], bufs[o1:o2], bufs[o2:o3], bufs[o3:-1], bufs[-1]
        KT = D // 128; XA = P["XA"]; LN = P["LN"]
        xr = [(a_ * BX, (b_ - a_) * BX) for a_, b_ in zip(XA[:-1], XA[1:])]
        x_cp = lambda i: pltpu.make_async_copy(x_hbm.at[pl.ds(*xr[i])], x_buf.at[pl.ds(*xr[i])], x_sem.at[i])
        wq_cp = lambda j: pltpu.make_async_copy(wq_hbm.at[:, pl.ds(j * G * DH, G * DH)], wq_buf.at[j], wq_sem.at[j])
        wq_half = lambda k: pltpu.make_async_copy(wq_hbm.at[:, pl.ds(k * 256, 256)], wq_buf.at[0, :, pl.ds(k * 256, 256)], misc_sem.at[5 + k])
        hr = [(0, HA), (HA, H - HA)]; vr = [(0, HA + 4), (HA + 4, H - HA - 4)]
        k_cp = lambda j: pltpu.make_async_copy(k_hbm.at[pl.ds(*hr[j])], k_buf.at[pl.ds(*hr[j])], kv_sem.at[2 * j])
        v_cp = lambda j: pltpu.make_async_copy(v_hbm.at[pl.ds(*vr[j])], v_buf.at[pl.ds(*vr[j])], kv_sem.at[2 * j + 1])
        wr_cp = lambda: pltpu.make_async_copy(wr_hbm, wr_buf, misc_sem.at[0])
        wg_cp = lambda: pltpu.make_async_copy(wg_hbm, wg_buf, misc_sem.at[1])
        wu_cp = lambda: pltpu.make_async_copy(wu_hbm, wu_buf, misc_sem.at[2])
        wd_cp = lambda: pltpu.make_async_copy(wd_hbm, wd_buf, misc_sem.at[3])
        wo_cp = lambda: pltpu.make_async_copy(wo_hbm, wo_buf, misc_sem.at[4])

        cur = []
        def mark(name):
            if not P.get("PROF"): return
            if cur: cur.pop().__exit__(None, None, None)
            if name:
                cm = jax.named_scope(name); cm.__enter__(); cur.append(cm)
        mark("p0_wait_x0")
        cps = dict(x0=lambda: x_cp(0), x1=lambda: x_cp(1), x2=lambda: x_cp(2), x3=lambda: x_cp(3), x4=lambda: x_cp(4), wr=wr_cp,
                   q0=lambda: wq_cp(0), qa=lambda: wq_half(0), qb=lambda: wq_half(1), q1=lambda: wq_cp(1))
        def start(stage):
            for nm in P["DS"][stage].split():
                if nm == "qr":
                    for j in range(2, P['NJ'] * P['MB'] // NX + 1): wq_cp(j).start()
                else: cps[nm]().start()
        start(0)
        z_ref[0] = 0
        z_ref[1] = 0

        def store_q(j, g, i, q, BX=BX):
            q32 = q * (DH ** -0.5 * LOG2E); q = q32.astype(bf16)
            if isinstance(i, int): w_buf[1 + (j * G + g) * 4 + i // 2, pl.ds(i % 2 * BX, BX), :] = q
            else: w_buf[1 + (j * G + g) * 4 + i[0], pl.ds(i[1] * BX, BX), :] = q
            return q32

        def qproj(j, i, after=None):
            xn = xn_buf[pl.ds(i * BX if isinstance(i, int) else pl.multiple_of(i * BX, BX), BX), :]
            if after is not None:
                head = jnp.where(lane > j + 1000, after, pltpu.bitcast(xn[:16, :128], f32))
                xn = jnp.concatenate([jnp.concatenate([pltpu.bitcast(head, bf16), xn[:16, 128:]], axis=1), xn[16:]], axis=0)
            q = jnp.dot(xn, wq_buf[j], preferred_element_type=f32)
            return [store_q(j, g, i, q[:, g * DH:(g + 1) * DH]) for g in range(G)]

        HK = 256
        A_SUMS = {1: (0, 0, 1, 1, 1), 2: (1, 0, 1, 1, 1), 5: (0, 0, 0, 1, 1), 6: (1, 0, 0, 0, -1), 7: (0, 1, 1, 1, -1)}
        B_SUMS = {1: (0, 0, 1, 1, 1), 3: (0, 1, 1, 1, -1), 4: (1, 0, 0, 0, -1), 6: (0, 0, 0, 1, 1), 7: (1, 0, 1, 1, 1)}
        def combine(get, spec):
            a, b = get(*spec[:2]).astype(f32), get(*spec[2:4]).astype(f32)
            return (a + b if spec[4] > 0 else a - b).astype(bf16)
        def strassen(j, p, sums, after=None):
            st_ = isinstance(p, int)
            xa = lambda r, k, w=HK: xn_buf[pl.ds((2 * p + r) * BX if st_ else pl.multiple_of((2 * p + r) * BX, BX), BX), pl.ds(k * HK, w)]
            wb = lambda k, c: wq_buf[j, pl.ds(k * HK, HK), pl.ds(c * HK, HK)]
            def m(i):
                if i in A_SUMS:
                    if i not in sums: sums[i] = combine(xa, A_SUMS[i])
                    a = sums[i]
                else:
                    a = xa(0, 0) if i == 3 else xa(1, 1)
                b = combine(wb, B_SUMS[i]) if i in B_SUMS else (wb(0, 0) if i == 2 else wb(1, 1))
                return jnp.dot(a, b, preferred_element_type=f32)
            def rest(r, after=None):
                a = xa(r, 2, 128)
                if after is not None:
                    head = jnp.where(lane > p + 1000, after, pltpu.bitcast(a[:16], f32))
                    a = jnp.concatenate([pltpu.bitcast(head, bf16), a[16:]], axis=0)
                e = jnp.dot(a, wq_buf[j, pl.ds(2 * HK, 128), :], preferred_element_type=f32)
                return e[:, :HK], e[:, HK:]
            def put(r, c, q):
                return [store_q(j, 2 * c + g, (p, r), q[:, g * DH:(g + 1) * DH]) for g in range(2)]
            c11, c12 = rest(0, after); yield
            d = m(5); c11 = c11 - d; c12 = c12 + d; yield
            d = m(3); yield put(0, 1, c12 + d)
            c21, c22 = rest(1); c22 = c22 + d; yield
            d = m(2); c21 = c21 + d; c22 = c22 - d; yield
            d = m(4); c11 = c11 + d; yield put(1, 0, c21 + d)
            c11 = c11 + m(7); yield
            d = m(1); c22 = c22 + d; yield put(0, 0, c11 + d)
            yield put(1, 1, c22 + m(6))

        lane = lax.broadcasted_iota(i32, (8, 128), 1)
        sub = lax.broadcasted_iota(i32, (8, 128), 0)

        def layernorm(r0, n):
            x = x_buf[pl.ds(r0, n), :].astype(f32)
            m = jnp.sum(x, axis=-1, keepdims=True)
            yield
            m = m * (1.0 / D)
            mb = rb(m)
            xc = x - mb
            dm = m - mb
            var = jnp.sum(xc * xc, axis=-1, keepdims=True)
            if P["XB"]: xb = xc.astype(bf16)
            yield
            var = jnp.broadcast_to(var * (1.0 / D) - dm * dm, (n, 128))
            if P["DENSE"]:
                dense = var[:8]
                for t in range(1, n // 8):
                    dense = jnp.where(lane == t, var[t * 8:(t + 1) * 8], dense)
                inv = 1.0 / rb(jnp.sqrt(rb(rb(jnp.maximum(dense, 0.0)) + EPS)))
                inv = jnp.concatenate([jnp.broadcast_to(inv[:, t:t + 1], (8, 128)) for t in range(n // 8)], axis=0)
                yield
            else:
                inv = 1.0 / rb(jnp.sqrt(rb(rb(jnp.maximum(var, 0.0)) + EPS)))
            xr_ = xb.astype(f32) if P["XB"] else rb(xc)
            xn = jnp.concatenate([xr_[:, w * 128:(w + 1) * 128] * inv for w in range(D // 128)], axis=1).astype(bf16)
            xn_buf[pl.ds(r0, n), :] = xn
            x_buf[pl.ds(S + r0, n), :] = xn
            yield "stored"

        ln = dict(next=0, done=0, live=[])
        def layernorm_upto(row, avail):
            while ln["done"] < row:
                for gen in list(ln["live"]):
                    st_ = next(gen, "end")
                    if st_ == "stored": ln["done"] += LN
                    if st_ == "end": ln["live"].remove(gen)
                if ln["next"] < avail:
                    gen = layernorm(ln["next"], LN); next(gen)
                    ln["live"].append(gen); ln["next"] += LN

        x_cp(0).wait()
        start(1)
        wr_cp().wait()
        mark('p1_ln0')
        if 'p' in P['SKIP']: ln['done'] = S
        layernorm_upto(BX, BX)
        mark('p2_wait_wq0')
        (wq_half(0) if P['HQ'] else wq_cp(0)).wait()
        start(2)
        starts = [r[0] // BX for r in xr]
        for i in range(NX):
            if i + 1 in starts:
                n_ = starts.index(i + 1)
                mark(f'p3_wait_x{n_}')
                start(2 + n_)
                x_cp(n_).wait()
                avail = xr[n_][0] + xr[n_][1]
            if i + 1 in starts: mark(f'p3_q{i}')
            def half(i, k):
                q = jnp.dot(xn_buf[pl.ds(i * BX, BX), :], wq_buf[0, :, pl.ds(k * 256, 256)], preferred_element_type=f32)
                for g in range(2): store_q(0, 2 * k + g, i, q[:, g * DH:(g + 1) * DH])
            if P["HQ"] and i == 0:
                half(0, 0); layernorm_upto(2 * BX, avail); half(1, 0)
                continue
            if P["HQ"] and i == 1:
                wq_half(1).wait(); half(0, 1); half(1, 1)
            else:
                qs = qproj(0, i)
            if i + 1 < NX:
                layernorm_upto((i + 2) * BX, avail)
        for gen in ln["live"]:
            for _ in gen: pass

        NJ, MB = P["NJ"], P["MB"]
        JL = NJ * MB // NX
        RR = -(-S // (NJ * 256)) * 256
        row16 = lax.broadcasted_iota(i32, (16, D), 0)
        def top_k(rds):
            keys = []
            for t in range(NJ):
                r = rb(rds[t])
                r = jnp.where(r == 0.0, 0.0, r)
                b = lax.shift_right_logical(pltpu.bitcast(r, i32), 16)
                k16 = jnp.where(b >= 0x8000, 0xFFFF - b, b + 0x8000)
                k16 = jnp.where(r != r, 0, k16)
                tok = min(t * RR, S - RR) + lane * 8 + sub
                keys.append(pltpu.bitcast(jnp.where(lane < RR // 8, 0x20000000 + k16 * 2048 + (2047 - tok), 0), f32))
            ktop = jnp.zeros((8, 128), i32)
            x_sel = jnp.zeros((16, D), f32)
            for c in range(C):
                mx = functools.reduce(jnp.maximum, keys)
                mx = jnp.max(jnp.max(mx, axis=0, keepdims=True), axis=1, keepdims=True)
                mxb = jnp.broadcast_to(mx, (8, 128))
                keys = [jnp.where(kk == mxb, 0.0, kk) for kk in keys]
                mi = pltpu.bitcast(mxb, i32)
                ktop = jnp.where(sub == c, mi, ktop)
                idx = 2047 - (mi[0, 0] & 2047)
                base = pl.multiple_of(idx & -16, 16)
                blk = xn_buf[pl.ds(base, 16), :].astype(f32)
                rowv = jnp.sum(jnp.where(row16 == idx - base, blk, 0.0), axis=0, keepdims=True)
                x_sel = jnp.where(row16 == c, rowv, x_sel)
            return ktop, x_sel
        mark('p5_1b')
        def p1_body(jj, carry):
            @pl.when(jj == 1)
            def _():
                k_cp(0).start(); v_cp(0).start()
            @pl.when(jj == 0)
            def _():
                for j in range(1, JL): wq_cp(j).wait()
                for j in range(JL + 1, NG): wq_cp(j).start()
                wg_cp().start(); wu_cp().start(); wd_cp().start(); wo_cp().start()
                wq_cp(JL).wait()
            wr = wr_buf[...].astype(f32).reshape(1, D)
            r0 = pl.multiple_of(jnp.minimum(jj * RR, S - RR), 256)
            rd = jnp.zeros((8, 128), f32)
            RP = P["RP"]
            never = lax.broadcasted_iota(i32, (8, 128), 1) > jj + 1000
            after = None
            piece = 0
            for n_ in range(MB // 2 if 'p' not in P['SKIP'] else 0):
                if n_ % JL == 0: sums = {}
                for qs in strassen(1 + n_ % JL, jj * (MB // 2 // JL) + n_ // JL, sums, after if n_ == P["R0"] else None):
                    if qs is None or piece * RP == RR: continue
                    tok = qs[0][:8]
                    for t in range(piece * RP // 16, (piece + 1) * RP // 16):
                        r = 0.0
                        for w in range(KT):
                            xb = pltpu.bitcast(xn_buf[pl.ds(r0 + t * 16, 16), pl.ds(w * 128, 128)], f32)
                            d_ = pltpu.bitcast(jnp.where(never, tok, xb), bf16).astype(f32) * wr[:, w * 128:(w + 1) * 128]
                            r = d_ if w == 0 else r + d_
                        r = jnp.broadcast_to(jnp.sum(r, axis=-1, keepdims=True), (16, 128))
                        rd = jnp.where(lane == 2 * t, r[:8], jnp.where(lane == 2 * t + 1, r[8:], rd))
                    piece += 1
                    if piece * RP == RR:
                        rds = [jnp.where(jnp.full((8, 128), jj) == t, rd, carry[0][t]) for t in range(NJ)]
                        ktop, x_sel = top_k(rds)
                        after = functools.reduce(lax.add, [x_sel[:8, w * 128:(w + 1) * 128] for w in range(KT)])
            if 'p' in P['SKIP']: return carry
            return rds, ktop, x_sel
        zero = jnp.zeros((8, 128), f32)
        _, ktop, x_sel = lax.fori_loop(0, NJ, p1_body, ([zero] * NJ, jnp.zeros((8, 128), i32), jnp.zeros((16, D), f32)))
        x_sel = x_sel[:8]

        mark('p6_wait')
        for j in range(JL + 1, NG): wq_cp(j).wait()
        wg_cp().wait(); wu_cp().wait(); wd_cp().wait()
        k_cp(0).wait(); v_cp(0).wait(); wo_cp().wait()
        mark('p7_1c')
        k16 = lax.shift_right_logical(ktop - 0x20000000, 11)
        b = jnp.where(k16 >= 0x8000, k16 - 0x8000, 0xFFFF - k16)
        r_sel = pltpu.bitcast(lax.shift_left(b, 16), f32)[:, :1]
        xs = x_sel.astype(bf16)
        acc = {}
        def accum(key, d):
            acc[key] = acc[key] + d if key in acc else d
        BC = P["BC"]
        def q_tile(j, i, g, k):
            accum((j, i, g), jnp.dot(xn_buf[pl.ds(i * BC, BC), pl.ds(k * 128, 128)], wq_buf[j, pl.ds(k * 128, 128), pl.ds(g * DH, DH)], preferred_element_type=f32))
            if k == KT - 1:
                store_q(j, g, i, acc.pop((j, i, g)), BC)
        fr = [(f0, min(128, F - f0)) for f0 in range(0, F, 128)]
        def up_tile(name, w, f, k):
            accum((name, f), lax.dot_general(xs[:, k * 128:(k + 1) * 128], w[pl.ds(*fr[f]), pl.ds(k * 128, 128)], NT, preferred_element_type=f32))
        def down_tile(f, n):
            if n == 0:
                a = rb(acc.pop(("g", f)))
                acc["h"] = (rb(a * sigmoid(a)) * rb(acc.pop(("u", f)))).astype(bf16)
            accum(("y", n), jnp.dot(acc["h"], wd_buf[pl.ds(*fr[f]), pl.ds(n * 128, 128)], preferred_element_type=f32))
        part = functools.partial
        f_tiles = [part(up_tile, nm, w, f, k) for f in range(len(fr)) for nm, w in (("g", wg_buf), ("u", wu_buf)) for k in range(KT)]
        f_tiles += [None] * (4 * P["FG"])
        f_tiles += [part(down_tile, f, n) for f in range(len(fr)) for n in range(KT)]
        sums = [{} for p in range(NX // 2)]
        rounds = (_ for p in range(NX // 2) for j in range(JL + 1, NG) for _ in strassen(j, p, sums[p]))
        for rnd, _ in enumerate(rounds if 'p' not in P['SKIP'] else range(72)):
            if rnd >= P["F0"] and rnd % P['FS'][0] not in P['FS'][1:]:
                for fn_ in f_tiles[:4]:
                    if fn_ is not None: fn_()
                f_tiles = f_tiles[4:]
        assert not f_tiles
        y = rb(jnp.concatenate([acc.pop(("y", n)) for n in range(KT)], axis=1))
        z = rb(x_sel + rb(y * rb(sigmoid(r_sel))))
        for c in range(C):
            idx = 2047 - (ktop[c, 0] & 2047)
            at = pl.ds(S + pl.multiple_of(idx & -16, 16), 16)
            x_buf[at, :] = jnp.where(row16 == (idx & 15), z[c:c + 1, :], x_buf[at, :].astype(f32)).astype(bf16)

        k_cp(1).start(); v_cp(1).start()
        for hh in range(4):
            for k in range(8):
                vt = [v_buf[hh, pl.ds((kh * 8 + k) * 128, 128), :].T for kh in range(2)]
                for i, pr in enumerate(PRODS):
                    t_bufs[1][hh, pl.ds((i * 8 + k) * 64, 64), :] = signed_sum(lambda dh, kh: vt[kh][dh * 64:(dh + 1) * 64].astype(f32), pr[0]).astype(bf16)
        mark('p8_att')
        def out_cp(i):
            return pltpu.make_async_copy(out_buf.at[pl.ds(i * BQ, BQ)], out_hbm.at[pl.ds(i * BQ, BQ)], out_sem.at[i])
        z0, z1 = (pl.multiple_of(z_ref[i], 64) for i in range(2))
        def att_body(t, _):
            @pl.when(t == HA // G * 2)
            def _():
                k_cp(1).wait(); v_cp(1).wait()
            grp = lax.shift_right_logical(t, 1); qh = t & 1
            def out_start(b_):
                @pl.when(grp == NG - 1)
                def _():
                    out_cp(qh * 8 + b_).start()
            attention_body(grp, qh, pl.multiple_of(t * 128, 128), z0, z1, w_buf, s_bufs, u_bufs, c_bufs, t_bufs, k_buf, v_buf, wo_buf, x_buf, y_buf, out_buf, u_buf, out_start, P)
        lax.fori_loop(P.get('T0', 0), NG * 2, att_body, None)
        mark('pa_wait_out')
        for i in range(NB):
            out_cp(i).wait()
        mark(None)

    @jax.jit
    def fn(A_x, A_k_cache, A_v_cache, A_wq, A_wo, B_x, B_w_r, B_w_gate, B_w_up, B_w_down):
        any_spec = pl.BlockSpec(memory_space=pl.ANY)
        V = pltpu.VMEM
        out = pl.pallas_call(
            kernel,
            in_specs=[any_spec] * 9,
            out_specs=any_spec,
            out_shape=jax.ShapeDtypeStruct((S, D), bf16),
            scratch_shapes=[
                pltpu.VMEM((2 * S + 64, D), bf16), pltpu.VMEM((S, D), bf16),
                V((1 + H * 4, 512, DH), bf16), pltpu.VMEM((D // 128 * S + 32, DH), f32), V((1, 2560, 128), bf16),
                pltpu.VMEM((H + 1, SK, DH), bf16), pltpu.VMEM((H + 1, SK, DH), bf16),
                pltpu.VMEM((NG, D, G * DH), bf16), pltpu.VMEM((NG, G * DH, D), bf16),
                pltpu.VMEM((F, D), bf16), pltpu.VMEM((F, D), bf16), pltpu.VMEM((F, D), bf16),
                pltpu.VMEM((S, D), bf16), pltpu.SMEM((2,), i32),
                pltpu.SemaphoreType.DMA((len(P['XA']) - 1,)), pltpu.SemaphoreType.DMA((NG,)), pltpu.SemaphoreType.DMA((4,)),
                pltpu.SemaphoreType.DMA((7,)), pltpu.SemaphoreType.DMA((NB,)),
            ] + [V((4096 + 32, 128), f32)] * P['NS'] + [V((1, 7 * 1024 + 320, 128), bf16)] * P['NUB'] + [V((288, 128), f32)] * P['NC'] + [V((1, 64, 128), bf16), V((9, 56 * 64, 128), bf16), V((1, 320, 128), bf16)] + [pltpu.VMEM((D,), bf16)],
            compiler_params=pltpu.CompilerParams(vmem_limit_bytes=126 * 1024 * 1024, flags=flags),
            name="fused_kernel",
        )(A_x.reshape(S, D), A_k_cache.reshape(H, SK, DH), A_v_cache.reshape(H, SK, DH), A_wq, A_wo.reshape(NG, G * DH, D),
          B_w_r, B_w_gate.T, B_w_up.T, B_w_down)
        return out.reshape(1, S, D)
    return fn


_impl = make()


@jax.jit
def pallas_recurrent_scan__mha_block_cached__moe_arch_mod__prompt_kernel(
    A_x, A_k_cache, A_v_cache, A_wq, A_wo, B_x, B_w_r, B_w_gate, B_w_up, B_w_down
):
    return _impl(A_x, A_k_cache, A_v_cache, A_wq, A_wo, B_x, B_w_r, B_w_gate, B_w_up, B_w_down)
```

```python
import functools

import jax
import jax.experimental.pallas as pl
import jax.experimental.pallas.tpu as pltpu
import jax.numpy as jnp
import numpy as np
from jax import lax

S, D, H, DH, SK, F, C = 2048, 640, 32, 128, 2048, 1728, 8
KT = D // 128
G = 4
NG = H // G
BX = 256
NX = S // BX
LOG2E = 1.4426950408889634
EPS = float(np.asarray(1e-5, dtype=jnp.bfloat16))
f32, bf16, i32 = jnp.float32, jnp.bfloat16, jnp.int32
NT = (((1,), (1,)), ((), ()))

PV = [
    (((1, 1, 1),), ((0, 0, 1), (1, 0, 1)), ((0, 0, -1), (1, 0, 1))),
    (((0, 0, 1),), ((0, 1, 1), (1, 1, 1)), ((0, 1, 1), (1, 1, -1))),
    (((1, 0, 1), (1, 1, -1)), ((0, 0, 1),), ((1, 0, 1), (1, 1, 1))),
    (((0, 1, 1), (0, 0, -1)), ((1, 1, 1),), ((0, 0, 1), (0, 1, 1))),
    (((0, 1, 1), (1, 1, 1)), ((1, 0, 1), (1, 1, -1)), ((0, 0, 1),)),
    (((0, 0, 1), (1, 1, 1)), ((0, 0, 1), (1, 1, 1)), ((0, 0, 1), (1, 1, 1))),
    (((0, 0, 1), (1, 0, 1)), ((0, 1, 1), (0, 0, -1)), ((1, 1, 1),)),
]
OP = [
    0,
    (((0, 0, 1), (0, 1, 1)), ((1, 1, 1),), ((0, 0, -1), (0, 1, 1))),
    (((1, 0, 1), (1, 1, 1)), ((0, 0, 1),), ((1, 0, 1), (1, 1, -1))),
    (((0, 0, 1),), ((0, 1, 1), (1, 1, -1)), ((0, 1, 1), (1, 1, 1))),
    (((1, 1, 1),), ((1, 0, 1), (0, 0, -1)), ((0, 0, 1), (1, 0, 1))),
    (((0, 1, 1), (1, 1, -1)), ((1, 0, 1), (1, 1, 1)), ((0, 0, 1),)),
    (((0, 0, 1), (1, 1, 1)), ((0, 0, 1), (1, 1, 1)), ((0, 0, 1), (1, 1, 1))),
    (((1, 0, 1), (0, 0, -1)), ((0, 0, 1), (0, 1, 1)), ((1, 1, 1),)),
    1,
]
OP_SUMS = [c for c, step in enumerate(OP) if not isinstance(step, int) and len(step[1]) > 1]

TIMING = dict(
    POP=10,
    K=3, Q=8, U=8, T=2, O=3,
    ACC=3,
    PREP=3,
    STAT=6, STAT_STEP=8, STAT_TOK=4,
    XPOSE=15,
    LAG=5,
    W_START=0.4, W_QK=0.7, W_OP=0.5, W_SHIFT=-1,
    OP_RATE=0.55,
    V_PREP=(330, 1300), WO_PREP=(14, 1.6), GATE=(1300, 8),
)
N_S, N_U, N_C = 7, 4, 8


def rb(x):
    return x.astype(bf16).astype(f32)


def sigmoid(x):
    return 1.0 / (1.0 + jnp.exp2(x * (-LOG2E)))


def signed_sum(get, terms):
    v = get(*terms[0][:2])
    for i, j, sign in terms[1:]:
        v = v + get(i, j) if sign > 0 else v - get(i, j)
    return v


def updates(outputs):
    result = []
    for c, outs in enumerate(outputs):
        users = lambda i, j: [k for k, other in enumerate(outputs) if any(o[:2] == (i, j) for o in other)]
        result.append([(i, j, sign, c == users(i, j)[0], c == users(i, j)[-1]) for i, j, sign in outs])
    return result


def attention_step(t, z_st, z_ld, q_buf, k_buf, v_buf, wo_buf, x_buf, out_buf, vt_buf, t_buf, ws_buf,
                   y_bufs, s_bufs, u_bufs, c_bufs, out_start):
    T = TIMING
    POP = T["POP"]
    n = 2 * G
    grp, half = lax.shift_right_logical(t, 1), t & 1
    heads = [grp * G + a % G for a in range(n)]
    q_blocks = [1 + heads[a] * 4 + half * 2 + a // G for a in range(n)]
    row0 = pl.multiple_of(half * (S // 2), S // 2)
    r_st, r_ld = pl.multiple_of(z_st * 64, 64), pl.multiple_of(z_ld * 64, 64)
    never = lax.broadcasted_iota(i32, (8, 128), 1) > z_st + 1000

    dots, pending, seen = [], [("op", b, c) for b in range(2) for c in range(len(OP))], 0
    for hp in range(2 * n + T["LAG"]):
        for c in range(8):
            if hp < 2 * n and c % 2 == 0:
                dots += [("qk", hp // 2, 8 * (hp % 2) + c + e) for e in range(2)]
            if hp >= T["LAG"] and c < 7:
                dots.append(("pv", (hp - T["LAG"]) // 2, 7 * ((hp - T["LAG"]) % 2) + c))
            if hp > n + T["LAG"] and c < 7:
                seen += 1
                while pending and 2 * len(OP) - len(pending) < seen * T["OP_RATE"] and (c in (1, 3, 5, 6) or hp >= 2 * n):
                    dots.append(pending.pop(0))
    dots += pending + [("op", b, c) for b in range(2, 4) for c in range(len(OP))]
    start = {d: 8 * i for i, d in enumerate(dots)}

    events, val = [], {}

    def at(slot, order):
        return lambda fn: events.append((slot, order, len(events), fn))

    def load(ref, r, rows, block=0):
        return pltpu.bitcast(ref.bitcast(f32)[z_ld + block, pl.ds(r // 2, rows // 2), :], bf16)

    def store(ref, r, v, block=0):
        ref[z_st + block, pl.ds(r, v.shape[0]), :] = v

    def token(ref, r, v=None, block=0):
        v = val.get("token") if v is None else v
        if v is not None:
            ref.bitcast(f32)[z_st + block, pl.ds(r // 2, 8), :] = v

    def x_token():
        x_buf.bitcast(f32)[pl.ds(r_st + S, 4), pl.ds(0, 128)] = val["token"][:4]

    ring = lambda bufs, a, p: bufs[(2 * a + p) % len(bufs)]

    def result(d):
        if d not in val:
            kind, a, c = d
            if kind == "qk" and c % 2:
                val[d] = result((kind, a, c - 1))[128:]
            elif kind == "qk":
                k = jnp.concatenate([val.pop(("k", a, 8 * c + r)) for r in range(16)], axis=0)
                q = jnp.concatenate([val.pop(("q", d, j, r)) for j in range(4) for r in range(4)], axis=0)
                val[d] = lax.dot_general(k, q, NT, preferred_element_type=f32)
            elif kind == "pv":
                vt = jnp.concatenate([jnp.concatenate([val.pop(("t", d, 4 * w + r)) for r in range(4)], axis=0)
                                      for w in range(2)], axis=1)
                pt = jnp.concatenate([val.pop(("u", d, k, r)) for k in range(8) for r in range(4)], axis=0)
                val[d] = jnp.dot(vt, pt, preferred_element_type=f32)
            else:
                o = jnp.concatenate([val.pop(("o", d, r)) for r in range(8)], axis=0)
                if isinstance(OP[c], int):
                    w = wo_buf[grp, :, pl.ds(512, 128)]
                elif c in OP_SUMS:
                    w = jnp.concatenate([load(ws_buf, (2 * OP_SUMS.index(c) + u) * 256, 256) for u in range(2)], axis=1)
                else:
                    w = wo_buf[grp, pl.ds(OP[c][1][0][0] * 256, 256), pl.ds(OP[c][1][0][1] * 256, 256)]
                val[d] = jnp.dot(o, w, preferred_element_type=f32)
        return val[d]

    def scores(d):
        _, a, c = d
        j0 = start[d]
        for r in range(4 if c % 2 == 0 else 0):
            @at(j0 + r - T["Q"], 1)
            def _(r=3 - r):
                token(q_buf, 0)
                for j in range(4):
                    val["q", d, j, r] = load(q_buf, 128 * j + 32 * r, 32, q_blocks[a])
        for r in range(8):
            @at(min(j0 + r - T["K"], j0 - c % 2 * 8 + POP - 1), 1)
            def _(r=r):
                if r == 0:
                    token(k_buf, 0, block=H)
                val["k", a, 8 * c + r] = load(k_buf, 128 * c + 16 * r, 16, heads[a])

            @at(j0 + r + POP, 0)
            def _(r=r):
                s = result(d)[16 * r:16 * r + 16]
                for j in range(4):
                    tile = s[:, 128 * j:128 * (j + 1)]
                    ring(s_bufs, a, j // 2)[pl.ds(r_st + ((8 * c + r) * 2 + j % 2) * 16, 16), :] = tile
                    x = jnp.maximum(tile[:8], tile[8:])
                    val["max", j] = x if r == 0 else jnp.maximum(x, val["max", j])
                    if r == 7:
                        x = val["max", j]
                        if c == 0:
                            m, e = x, jnp.ones_like(x)
                        else:
                            m0, e0 = val["stat", a, j]
                            m = jnp.maximum(m0, x)
                            e = jnp.exp2(x - m) + e0 * jnp.exp2(m0 - m)
                        val["stat", a, j] = (m, e)
                        val["stat token", d] = e
                val["token"] = s[:8, 384:]

        @at(j0 + 7 + POP + T["STAT_TOK"], 0)
        def _():
            token(q_buf, 16, val.pop(("stat token", d)))

        for j in range(4 if c == 15 else 0):
            @at(j0 + 8 + POP + T["STAT"] + T["STAT_STEP"] * j, 0)
            def _(j=j):
                m, e = val.pop(("stat", a, j))
                top = jnp.max(m, axis=0, keepdims=True)
                e = jnp.broadcast_to(jnp.sum(e * jnp.exp2(m - top), axis=0, keepdims=True), (8, 128))
                shift = (0.5 * np.log2(SK) / np.log2(SK / 16)) * jnp.log2(e)
                ring(s_bufs, a, j // 2)[pl.ds(r_st + 2 * SK + 8 * (j % 2), 8), :] = top + shift

    def probabilities(a, p, slot_of):
        s_buf, u_buf = ring(s_bufs, a, p), ring(u_bufs, a, p)
        for e in range(64):
            @at(slot_of(e), 1)
            def _(e=e):
                pace = jnp.where(never, val.pop("prep"), val["token"]) if "prep" in val else val["token"]
                s_buf[pl.ds(r_st + 2 * SK + 16, 8), :] = pace
                pt = {}
                for j in range(2):
                    m = s_buf[pl.ds(r_ld + 2 * SK + 8 * j, 8), :]
                    m = jnp.concatenate([m, m], axis=0)
                    for kh in range(2):
                        pt[kh, j] = jnp.exp2(s_buf[pl.ds(r_ld + ((64 * kh + e) * 2 + j) * 16, 16), :] - m)
                us = [signed_sum(lambda *ix: pt[ix], terms) for _, terms, _ in PV]
                for j in range(2):
                    x = us[j][:8] + us[j][8:]
                    val["sum", a, p, j] = x if e == 0 else val["sum", a, p, j] + x
                val["p", a, p, e] = ([u.astype(bf16) for u in us], val["sum", a, p, 1])

            @at(slot_of(e) + T["PREP"], 0)
            def _(e=e):
                us, val["prep"] = val.pop(("p", a, p, e))
                for i, u in enumerate(us):
                    store(u_buf, i * 1024 + 16 * e, u)

        @at(slot_of(63) + T["PREP"] + 2, 0)
        def _():
            for j in range(2):
                l = jnp.broadcast_to(jnp.sum(val.pop(("sum", a, p, j)), axis=0, keepdims=True), (8, 128))
                r = pl.reciprocal(l, approx=True)
                ring(c_bufs, a, p)[pl.ds(r_st + 256 + 8 * j, 8), :] = r * (2.0 - l * r)

    def values(d):
        _, a, c = d
        p, i = divmod(c, 7)
        j0 = start[d]
        u_buf, c_buf = ring(u_bufs, a, p), ring(c_bufs, a, p)
        outs = updates([step[2] for step in PV])[i]
        for r in range(8):
            @at(j0 + r - T["U"], 1)
            def _(w=r // 4, rr=3 - r % 4):
                if rr == 3:
                    token(u_buf, 7 * 1024)
                for k in range(4 * w, 4 * w + 4):
                    val["u", d, k, rr] = load(u_buf, (8 * i + k) * 128 + 32 * rr, 32)

            @at(j0 + r - T["T"], 1)
            def _(r=r):
                if r == 0:
                    token(t_buf, 0, block=2 * G)
                val["t", d, r] = jnp.concatenate(
                    [load(t_buf, (8 * i + r // 4 * 4 + k) * 64 + r % 4 * 16, 16, (grp & 1) * G + a % G)
                     for k in range(4)], axis=1)
        for r in range(4):
            @at(j0 + 4 + r + POP - T["ACC"], 1)
            def _(r=r):
                for dh, j, _, first, last in outs:
                    if not first:
                        val["c", d, r, dh, j] = c_buf[pl.ds(r_ld + 128 * j + 64 * dh + 16 * r, 16), :]
                    if last:
                        val["scale", d, r, dh, j] = c_buf[pl.ds(r_ld + 256 + 8 * j, 8), :]

            @at(j0 + 4 + r + POP, 0)
            def _(r=r):
                x = result(d)[16 * r:16 * r + 16]
                for dh, j, sign, first, last in outs:
                    if first:
                        y = x if sign > 0 else -x
                    else:
                        y = val.pop(("c", d, r, dh, j))
                        y = y + x if sign > 0 else y - x
                    if last:
                        y = y * jnp.tile(val.pop(("scale", d, r, dh, j)), (2, 1))
                        store(u_buf, 7 * 1024 + 64 + 128 * j + 64 * dh + 16 * r, y.astype(bf16))
                    else:
                        c_buf[pl.ds(r_st + 128 * j + 64 * dh + 16 * r, 16), :] = y
                val["token"] = x[:8]
        for j in range(2 if i == 6 else 0):
            @at(j0 + 9 + POP + 4 * j, 1)
            def _(j=j):
                val["ot", d, j] = load(u_buf, 7 * 1024 + 64 + 128 * j, 128).T

            @at(j0 + 9 + POP + 4 * j + T["XPOSE"], 0)
            def _(j=j):
                store(q_buf, (2 * p + j) * 128, val.pop(("ot", d, j)), q_blocks[a])

    def projection(d):
        _, b, c = d
        j0 = start[d]
        assert j0 - T["O"] > start["pv", b // 2 * G + G - 1, b % 2 * 7 + 6] + 13 + POP + T["XPOSE"]
        extra = isinstance(OP[c], int)
        outs = [(i, 2 * j + u, u, sign, last)
                for i, j, sign, _, last in updates([((s_, 2, 1),) if isinstance(s_, int) else s_[2] for s_ in OP])[c]
                for u in range(1 if extra else 2)]
        rows = lambda z, i, r, k=0: pl.ds(z + row0 + (k * S + (2 * b + i) * 128 + 16 * r), 16)
        for r in range(8):
            @at(j0 + r - T["O"], 1)
            def _(r=r):
                token(q_buf, 0)
                get = lambda i, h: load(q_buf, (b % 2 * 2 + i) * 128 + 16 * r, 16, q_blocks[b // 2 * G + h])
                if extra:
                    tiles = [get(OP[c], h) for h in range(G)]
                elif len(OP[c][0]) == 1:
                    tiles = [get(OP[c][0][0][0], 2 * OP[c][0][0][1] + u) for u in range(2)]
                else:
                    tiles = [signed_sum(lambda i, k: get(i, 2 * k + u).astype(f32), OP[c][0]).astype(bf16)
                             for u in range(2)]
                val["o", d, r] = jnp.concatenate(tiles, axis=1)

            @at(j0 + r + POP - T["ACC"], 1)
            def _(r=r):
                if r % 2 == 0 and any(last for *_, last in outs):
                    x_token()
                for i, w, _, _, last in outs:
                    val["y", d, r, i, w] = y_bufs[w][rows(r_ld, i, r), :]
                    if last:
                        val["x", d, r, i, w] = [x_buf[rows(r_ld, i, r, k), pl.ds(128 * w, 128)].astype(f32)
                                                for k in range(2)]

            @at(j0 + r + POP - 1, 0)
            def _(r=r):
                for i, w, u, sign, last in outs:
                    x = result(d)[16 * r:16 * r + 16, 128 * u:128 * (u + 1)]
                    y = val.pop(("y", d, r, i, w))
                    y = y + x if sign > 0 else y - x
                    y_bufs[w][rows(r_st, i, r), :] = y
                    if last:
                        x, gate = val.pop(("x", d, r, i, w))
                        out_buf[rows(0, i, r), pl.ds(128 * w, 128)] = (x + y * gate).astype(bf16)
                val["token"] = y[:8]
                if r == 7 and c in (6, 8):
                    out_start(2 * b + (c == 8))

    for d in dots:
        {"qk": scores, "pv": values, "op": projection}[d[0]](d)

    density = {start[d] + POP + r: T["W_QK"] if d[0] == "qk" else T["W_OP"]
               for d in dots if d[0] != "pv" for r in range(8)}
    cum = np.concatenate([[0], np.cumsum([T["W_START"] if j < start["pv", 0, 0] else density.get(j - T["W_SHIFT"], 1.0)
                                          for j in range(8 * len(dots))])])
    earliest = [max(start["qk", g // 2, 15] + 9 + POP + T["STAT"] + T["STAT_STEP"] * (g % 2 * 2 + 1),
                    start["pv", (g - N_U) // 2, (g - N_U) % 2 * 7 + 6] + 8 if g >= N_U else 0) for g in range(2 * n)]
    latest = [start["pv", g // 2, g % 2 * 7] - T["U"] - T["PREP"] - 1 for g in range(2 * n)]
    edge = [cum[earliest[0]]] + [cum[j] for j in latest]
    for _ in range(200):
        for g in range(1, 2 * n):
            edge[g] = min(max((edge[g - 1] + edge[g + 1]) / 2, cum[earliest[g]]), cum[latest[g - 1]])
    for g in range(2 * n):
        assert g + N_S >= 2 * n or latest[g] < start["qk", (g + N_S) // 2, 0] + POP
        probabilities(g // 2, g % 2, lambda e: int(np.searchsorted(cum, edge[g] + (edge[g + 1] - edge[g]) * (e + 0.5) / 64)) - 1)

    step = (T["V_PREP"][1] - T["V_PREP"][0]) / 16
    for hh, k in ((hh, k) for hh in range(2) for k in range(8)):
        head = jnp.minimum(grp + 1, NG - 1) * G + 2 * half + hh
        j0 = T["V_PREP"][0] + step * (8 * hh + k)
        for kh in range(2):
            @at(j0 + step / 2 * kh, 2)
            def _(head=head, hh=hh, k=k, kh=kh):
                token(v_buf, 0, block=H)
                val["vt", hh, k, kh] = load(v_buf, (8 * kh + k) * 128, 128, head).T

            @at(j0 + step / 2 * kh + T["XPOSE"], 0)
            def _(hh=hh, k=k, kh=kh):
                store(vt_buf, 128 * kh, val.pop(("vt", hh, k, kh)))
        for r in range(4):
            @at(j0 + step / 2 + 1 + T["XPOSE"] + step / 9 * r, 2)
            def _(hh=hh, k=k, r=r):
                token(vt_buf, 256)
                vt = {(dh, kh): load(vt_buf, 128 * kh + 64 * dh + 16 * r, 16).astype(f32)
                      for dh in range(2) for kh in range(2)}
                val["vs", hh, k, r] = [signed_sum(lambda *ix: vt[ix], terms) for terms, _, _ in PV]

            @at(j0 + step / 2 + 3 + T["XPOSE"] + step / 9 * r, 0)
            def _(hh=hh, k=k, r=r):
                for i, x in enumerate(val.pop(("vs", hh, k, r))):
                    store(t_buf, (8 * i + k) * 64 + 16 * r, x.astype(bf16), ((grp + 1) & 1) * G + 2 * half + hh)
                token(q_buf, 32, x[:8])

    for k, r in ((k, r) for k in range(len(OP_SUMS)) for r in range(16)):
        slot = T["WO_PREP"][0] + T["WO_PREP"][1] * (16 * k + r)

        @at(slot, 2)
        def _(k=k, r=r):
            for u in range(2):
                def get(i, j):
                    w = pltpu.bitcast(wo_buf[grp, pl.ds(256 * i + 16 * r, 16), pl.ds(256 * j + 128 * u, 128)], f32)
                    return pltpu.bitcast(jnp.where(never, val["token"], w), bf16).astype(f32)
                x = signed_sum(get, OP[OP_SUMS[k]][1])
                store(ws_buf, (2 * k + u) * 256 + 16 * r, x.astype(bf16))
            val["ws", k, r] = x[:8]

        @at(slot + 3, 0)
        def _(k=k, r=r):
            token(q_buf, 48, val.pop(("ws", k, r)))

    for r, w in ((r, w) for r in range(8) for w in range(KT)):
        slot = T["GATE"][0] + T["GATE"][1] * (KT * r + w)
        assert slot + 4 < start["op", 3, 0]
        where = lambda z, r=r, w=w: (pl.ds(z + pl.multiple_of(t * 128, 128) + (S + 16 * r), 16), pl.ds(128 * w, 128))

        @at(slot, 2)
        def _(r=r, w=w, where=where):
            x_token()
            x = x_buf[where(r_ld)].astype(f32)
            val["gate", r, w] = x * sigmoid(x)

        @at(slot + 4, 0)
        def _(r=r, w=w, where=where):
            gate = val.pop(("gate", r, w))
            x_buf[where(r_st)] = gate.astype(bf16)
            token(q_buf, 64, gate[8:])

    for *_, fn in sorted(events, key=lambda e: e[:3]):
        fn()


def kernel(x_hbm, k_hbm, v_hbm, wq_hbm, wo_hbm, wr_hbm, wg_hbm, wu_hbm, wd_hbm, out_hbm,
           x_buf, xn_buf, q_buf, k_buf, v_buf, wq_buf, wo_buf, wg_buf, wu_buf, wd_buf, out_buf,
           vt_buf, t_buf, ws_buf, y_bufs, s_bufs, u_bufs, c_bufs, wr_buf, zero_ref,
           x_sem, wq_sem, kv_sem, w_sem, out_sem):
    x_edges = (0, 1, 2, 4, 6, 8)

    def x_copy(i):
        rows = pl.ds(x_edges[i] * BX, (x_edges[i + 1] - x_edges[i]) * BX)
        return pltpu.make_async_copy(x_hbm.at[rows], x_buf.at[rows], x_sem.at[i])

    def wq_copy(j):
        return pltpu.make_async_copy(wq_hbm.at[:, pl.ds(j * G * DH, G * DH)], wq_buf.at[j], wq_sem.at[j])

    def kv_copies(late):
        k_heads, v_heads = (pl.ds(n, H - n) if late else pl.ds(0, n) for n in (G, 2 * G))
        return [pltpu.make_async_copy(k_hbm.at[k_heads], k_buf.at[k_heads], kv_sem.at[2 * late]),
                pltpu.make_async_copy(v_hbm.at[v_heads], v_buf.at[v_heads], kv_sem.at[2 * late + 1])]

    def w_copy(i):
        src, dst = ((wr_hbm, wr_buf), (wg_hbm, wg_buf), (wu_hbm, wu_buf), (wd_hbm, wd_buf), (wo_hbm, wo_buf))[i]
        return pltpu.make_async_copy(src, dst, w_sem.at[i])

    def out_copy(i):
        rows = pl.ds(i * 128, 128)
        return pltpu.make_async_copy(out_buf.at[rows], out_hbm.at[rows], out_sem.at[i])

    lane = lax.broadcasted_iota(i32, (8, 128), 1)
    sublane = lax.broadcasted_iota(i32, (8, 128), 0)
    row16 = lax.broadcasted_iota(i32, (16, D), 0)

    def layernorm(r0, n):
        x = x_buf[pl.ds(r0, n), :].astype(f32)
        mean = jnp.sum(x, axis=-1, keepdims=True)
        yield
        mean = mean * (1.0 / D)
        mean_b = rb(mean)
        xc = x - mean_b
        dm = mean - mean_b
        sq = jnp.sum(xc * xc, axis=-1, keepdims=True)
        yield
        var = jnp.broadcast_to(sq * (1.0 / D) - dm * dm, (n, 128))
        dense = var[:8]
        for k in range(1, n // 8):
            dense = jnp.where(lane == k, var[8 * k:8 * k + 8], dense)
        inv = 1.0 / rb(jnp.sqrt(rb(rb(jnp.maximum(dense, 0.0)) + EPS)))
        inv = jnp.concatenate([jnp.broadcast_to(inv[:, k:k + 1], (8, 128)) for k in range(n // 8)], axis=0)
        yield
        xc = rb(xc)
        xn = jnp.concatenate([xc[:, 128 * w:128 * (w + 1)] * inv for w in range(KT)], axis=1).astype(bf16)
        xn_buf[pl.ds(r0, n), :] = xn
        x_buf[pl.ds(S + r0, n), :] = xn

    live, started = [], [0]

    def layernorm_until(row, available):
        while started[0] - 64 * len(live) < row:
            for piece in list(live):
                if next(piece, "done") == "done":
                    live.remove(piece)
            if started[0] < available:
                live.append(layernorm(started[0], 64))
                next(live[-1])
                started[0] += 64

    def store_q(head, block, half, q):
        q = q * (DH ** -0.5 * LOG2E)
        q_buf[1 + head * 4 + block, pl.ds(half * BX, BX), :] = q.astype(bf16)
        return q[:8]

    JL = NG - 3
    x_copy(0).start()
    w_copy(0).start()
    wq_copy(0).start()
    x_copy(1).start()
    zero_ref[0] = 0
    zero_ref[1] = 0
    for y_buf in y_bufs:
        y_buf[...] = jnp.zeros_like(y_buf)
    x_copy(0).wait()
    x_copy(2).start()
    w_copy(0).wait()
    layernorm_until(BX, BX)
    wq_copy(0).wait()
    x_copy(3).start()
    for i in range(NX):
        if i + 1 in x_edges[:-1]:
            part = x_edges.index(i + 1)
            if part == 1:
                x_copy(4).start()
            if part == 3:
                for j in range(1, JL + 1):
                    wq_copy(j).start()
            x_copy(part).wait()
        q = jnp.dot(xn_buf[pl.ds(i * BX, BX), :], wq_buf[0], preferred_element_type=f32)
        for h in range(G):
            store_q(h, i // 2, i % 2, q[:, h * DH:(h + 1) * DH])
        if i + 1 < NX:
            layernorm_until((i + 2) * BX, x_edges[part + 1] * BX)

    def project(j, p, sums, after=None):
        rows = lambda r: pl.ds((2 * p + r) * BX if isinstance(p, int) else pl.multiple_of((2 * p + r) * BX, BX), BX)
        xa = lambda r, k: xn_buf[rows(r), pl.ds(256 * k, 256)]
        wb = lambda k, c: wq_buf[j, pl.ds(256 * k, 256), pl.ds(256 * c, 256)]

        def operand(get, terms):
            if len(terms) == 1:
                return get(*terms[0][:2])
            return signed_sum(lambda *ix: get(*ix).astype(f32), terms).astype(bf16)

        def product(c):
            if len(OP[c][0]) > 1 and c not in sums:
                sums[c] = operand(xa, OP[c][0])
            a = sums[c] if c in sums else operand(xa, OP[c][0])
            return jnp.dot(a, operand(wb, OP[c][1]), preferred_element_type=f32)

        def rest(r, after=None):
            a = xn_buf[rows(r), pl.ds(512, 128)]
            if after is not None:
                head = jnp.where(lane > p + 1000, after, pltpu.bitcast(a[:16], f32))
                a = jnp.concatenate([pltpu.bitcast(head, bf16), a[16:]], axis=0)
            e = jnp.dot(a, wq_buf[j, pl.ds(512, 128), :], preferred_element_type=f32)
            return e[:, :256], e[:, 256:]

        def put(r, c, q):
            return [store_q(j * G + 2 * c + h, p, r, q[:, h * DH:(h + 1) * DH]) for h in range(2)][0]

        c00, c01 = rest(0, after)
        yield
        m = product(1)
        c00, c01 = c00 - m, c01 + m
        yield
        m = product(3)
        yield put(0, 1, c01 + m)
        c10, c11 = rest(1)
        c11 = c11 + m
        yield
        m = product(2)
        c10, c11 = c10 + m, c11 - m
        yield
        m = product(4)
        c00 = c00 + m
        yield put(1, 0, c10 + m)
        c00 = c00 + product(5)
        yield
        m = product(6)
        c11 = c11 + m
        yield put(0, 0, c00 + m)
        yield put(1, 1, c11 + product(7))

    def top_k(scores):
        keys = []
        for k, r in enumerate(scores):
            r = rb(r)
            r = jnp.where(r == 0.0, 0.0, r)
            bits = lax.shift_right_logical(pltpu.bitcast(r, i32), 16)
            rank = jnp.where(r != r, 0, jnp.where(bits >= 0x8000, 0xFFFF - bits, bits + 0x8000))
            tok = k * 1024 + lane * 8 + sublane
            keys.append(pltpu.bitcast(0x20000000 + rank * S + (S - 1 - tok), f32))
        chosen, rows = jnp.zeros((8, 128), i32), jnp.zeros((16, D), f32)
        for c in range(C):
            best = jnp.max(jnp.max(jnp.maximum(*keys), axis=0, keepdims=True), axis=1, keepdims=True)
            best = jnp.broadcast_to(best, (8, 128))
            keys = [jnp.where(key == best, 0.0, key) for key in keys]
            best = pltpu.bitcast(best, i32)
            chosen = jnp.where(sublane == c, best, chosen)
            tok = S - 1 - (best[0, 0] & (S - 1))
            block = xn_buf[pl.ds(pl.multiple_of(tok & -16, 16), 16), :].astype(f32)
            row = jnp.sum(jnp.where(row16 == (tok & 15), block, 0.0), axis=0, keepdims=True)
            rows = jnp.where(row16 == c, row, rows)
        return chosen, rows

    def half_of_rows(jj, carry):
        @pl.when(jj == 1)
        def _():
            for copy in kv_copies(0):
                copy.start()

        @pl.when(jj == 0)
        def _():
            for j in range(1, JL):
                wq_copy(j).wait()
            for j in range(JL + 1, NG):
                wq_copy(j).start()
            for i in range(1, 5):
                w_copy(i).start()
            wq_copy(JL).wait()

        wr = wr_buf[...].astype(f32).reshape(1, D)
        r0 = pl.multiple_of(jj * (S // 2), S // 2)
        never = lane > jj + 1000
        score, done, after = jnp.zeros((8, 128), f32), 0, None
        for unit in range(2 * JL):
            if unit % JL == 0:
                sums = {}
            for pace in project(1 + unit % JL, 2 * jj + unit // JL, sums, after if unit == 2 * JL - 1 else None):
                if pace is None or done == 64:
                    continue
                for k in (done, done + 1):
                    terms = []
                    for w in range(KT):
                        xn = pltpu.bitcast(xn_buf[pl.ds(r0 + 16 * k, 16), pl.ds(128 * w, 128)], f32)
                        xn = pltpu.bitcast(jnp.where(never, pace, xn), bf16).astype(f32)
                        terms.append(xn * wr[:, 128 * w:128 * (w + 1)])
                    r = jnp.sum(functools.reduce(lambda x, y: x + y, terms), axis=-1, keepdims=True)
                    r = jnp.broadcast_to(r, (16, 128))
                    score = jnp.where(lane == 2 * k, r[:8], jnp.where(lane == 2 * k + 1, r[8:], score))
                done += 2
                if done == 64:
                    scores = [jnp.where(jnp.full((8, 128), jj) == k, score, carry[0][k]) for k in range(2)]
                    chosen, rows = top_k(scores)
                    after = functools.reduce(lambda x, y: x + y, [rows[:8, 128 * w:128 * (w + 1)] for w in range(KT)])
        return scores, chosen, rows

    zeros = jnp.zeros((8, 128), f32)
    _, chosen, x_sel = lax.fori_loop(
        0, 2, half_of_rows, ([zeros, zeros], jnp.zeros((8, 128), i32), jnp.zeros((16, D), f32)))
    x_sel = x_sel[:8]

    for j in range(JL + 1, NG):
        wq_copy(j).wait()
    for i in range(1, 4):
        w_copy(i).wait()
    for copy in kv_copies(0):
        copy.wait()
    w_copy(4).wait()
    rank = lax.shift_right_logical(chosen - 0x20000000, 11)
    r_sel = pltpu.bitcast(lax.shift_left(jnp.where(rank >= 0x8000, rank - 0x8000, 0xFFFF - rank), 16), f32)[:, :1]
    xs = x_sel.astype(bf16)
    cols = [pl.ds(f0, min(128, F - f0)) for f0 in range(0, F, 128)]
    acc = {}

    def accumulate(key, x):
        acc[key] = acc[key] + x if key in acc else x

    def up_tile(w_buf, name, f, k):
        accumulate((name, f), lax.dot_general(xs[:, 128 * k:128 * (k + 1)], w_buf[cols[f], pl.ds(128 * k, 128)], NT,
                                              preferred_element_type=f32))

    def down_tile(f, w):
        if w == 0:
            gate = rb(acc.pop(("gate", f)))
            acc["hidden"] = (rb(gate * sigmoid(gate)) * rb(acc.pop(("up", f)))).astype(bf16)
        accumulate(w, jnp.dot(acc["hidden"], wd_buf[cols[f], pl.ds(128 * w, 128)], preferred_element_type=f32))

    tiles = [functools.partial(up_tile, w_buf, name, f, k) for f in range(len(cols))
             for name, w_buf in (("gate", wg_buf), ("up", wu_buf)) for k in range(KT)]
    tiles += [lambda: None] * 32
    tiles += [functools.partial(down_tile, f, w) for f in range(len(cols)) for w in range(KT)]
    for p in range(NX // 2):
        sums = {}
        for j in range(JL + 1, NG):
            for k, _ in enumerate(project(j, p, sums)):
                if k != 7:
                    for tile in tiles[:4]:
                        tile()
                    tiles = tiles[4:]
    assert not tiles
    y = rb(jnp.concatenate([acc[w] for w in range(KT)], axis=1))
    routed = rb(x_sel + rb(y * rb(sigmoid(r_sel))))
    for c in range(C):
        tok = S - 1 - (chosen[c, 0] & (S - 1))
        rows = pl.ds(S + pl.multiple_of(tok & -16, 16), 16)
        x_buf[rows, :] = jnp.where(row16 == (tok & 15), routed[c:c + 1, :], x_buf[rows, :].astype(f32)).astype(bf16)
    for copy in kv_copies(1):
        copy.start()
    for h in range(G):
        for k in range(8):
            vt = [v_buf[h, pl.ds((8 * kh + k) * 128, 128), :].T for kh in range(2)]
            for i, (terms, _, _) in enumerate(PV):
                x = signed_sum(lambda dh, kh: vt[kh][64 * dh:64 * (dh + 1)].astype(f32), terms)
                t_buf[h, pl.ds((8 * i + k) * 64, 64), :] = x.astype(bf16)

    z_st, z_ld = zero_ref[0], zero_ref[1]

    def step(t, _):
        @pl.when(t == 2)
        def _():
            for copy in kv_copies(1):
                copy.wait()

        def out_start(block):
            @pl.when(t >= 2 * NG - 2)
            def _():
                out_copy((t & 1) * 8 + block).start()

        attention_step(t, z_st, z_ld, q_buf, k_buf, v_buf, wo_buf, x_buf, out_buf, vt_buf, t_buf, ws_buf,
                       y_bufs, s_bufs, u_bufs, c_bufs, out_start)

    lax.fori_loop(0, 2 * NG, step, None)
    for i in range(S // 128):
        out_copy(i).wait()


@jax.jit
def pallas_recurrent_scan__mha_block_cached__moe_arch_mod__prompt_kernel(
    A_x: jax.Array,
    A_k_cache: jax.Array,
    A_v_cache: jax.Array,
    A_wq: jax.Array,
    A_wo: jax.Array,
    B_x: jax.Array,
    B_w_r: jax.Array,
    B_w_gate: jax.Array,
    B_w_up: jax.Array,
    B_w_down: jax.Array,
):
    del B_x
    vmem, dma = pltpu.VMEM, pltpu.SemaphoreType.DMA
    hbm = pl.BlockSpec(memory_space=pl.ANY)
    scratch = [
        vmem((2 * S + 64, D), bf16),
        vmem((S, D), bf16),
        vmem((1 + 4 * H, 512, DH), bf16),
        vmem((H + 1, SK, DH), bf16),
        vmem((H + 1, SK, DH), bf16),
        vmem((NG, D, G * DH), bf16),
        vmem((NG, G * DH, D), bf16),
        vmem((F, D), bf16),
        vmem((F, D), bf16),
        vmem((F, D), bf16),
        vmem((S, D), bf16),
        vmem((1, 320, 128), bf16),
        vmem((2 * G + 1, 56 * 64, 128), bf16),
        vmem((1, 2560, 128), bf16),
        [vmem((S, 128), f32)] * KT,
        [vmem((2 * SK + 32, 128), f32)] * N_S,
        [vmem((1, 7 * 1024 + 320, 128), bf16)] * N_U,
        [vmem((288, 128), f32)] * N_C,
        vmem((D,), bf16),
        pltpu.SMEM((2,), i32),
        dma((5,)), dma((NG,)), dma((4,)), dma((5,)), dma((S // 128,)),
    ]
    out = pl.pallas_call(
        kernel,
        in_specs=[hbm] * 9,
        out_specs=hbm,
        out_shape=jax.ShapeDtypeStruct((S, D), bf16),
        scratch_shapes=scratch,
        compiler_params=pltpu.CompilerParams(vmem_limit_bytes=126 * 1024 * 1024),
        name="fused_kernel",
    )(A_x.reshape(S, D), A_k_cache.reshape(H, SK, DH), A_v_cache.reshape(H, SK, DH), A_wq,
      A_wo.reshape(NG, G * DH, D), B_w_r, B_w_gate.T, B_w_up.T, B_w_down)
    return out.reshape(1, S, D)
```

```python
import functools

import jax
import jax.experimental.pallas as pl
import jax.experimental.pallas.tpu as pltpu
import jax.numpy as jnp
import numpy as np
from jax import lax

S, D, H, DH, SK, F, C = 2048, 640, 32, 128, 2048, 1728, 8
KT = D // 128
G = 4
NG = H // G
BX = 256
NX = S // BX
LOG2E = 1.4426950408889634
EPS = float(np.asarray(1e-5, dtype=jnp.bfloat16))
f32, bf16, i32 = jnp.float32, jnp.bfloat16, jnp.int32
NT = (((1,), (1,)), ((), ()))

PV = [
    (((1, 1, 1),), ((0, 0, 1), (1, 0, 1)), ((0, 0, -1), (1, 0, 1))),
    (((0, 0, 1),), ((0, 1, 1), (1, 1, 1)), ((0, 1, 1), (1, 1, -1))),
    (((1, 0, 1), (1, 1, -1)), ((0, 0, 1),), ((1, 0, 1), (1, 1, 1))),
    (((0, 1, 1), (0, 0, -1)), ((1, 1, 1),), ((0, 0, 1), (0, 1, 1))),
    (((0, 1, 1), (1, 1, 1)), ((1, 0, 1), (1, 1, -1)), ((0, 0, 1),)),
    (((0, 0, 1), (1, 1, 1)), ((0, 0, 1), (1, 1, 1)), ((0, 0, 1), (1, 1, 1))),
    (((0, 0, 1), (1, 0, 1)), ((0, 1, 1), (0, 0, -1)), ((1, 1, 1),)),
]
OP = [
    0,
    (((0, 0, 1), (0, 1, 1)), ((1, 1, 1),), ((0, 0, -1), (0, 1, 1))),
    (((1, 0, 1), (1, 1, 1)), ((0, 0, 1),), ((1, 0, 1), (1, 1, -1))),
    (((0, 0, 1),), ((0, 1, 1), (1, 1, -1)), ((0, 1, 1), (1, 1, 1))),
    (((1, 1, 1),), ((1, 0, 1), (0, 0, -1)), ((0, 0, 1), (1, 0, 1))),
    (((0, 1, 1), (1, 1, -1)), ((1, 0, 1), (1, 1, 1)), ((0, 0, 1),)),
    (((0, 0, 1), (1, 1, 1)), ((0, 0, 1), (1, 1, 1)), ((0, 0, 1), (1, 1, 1))),
    (((1, 0, 1), (0, 0, -1)), ((0, 0, 1), (0, 1, 1)), ((1, 1, 1),)),
    1,
]
OP_SUMS = [c for c, step in enumerate(OP) if not isinstance(step, int) and len(step[1]) > 1]

TIMING = dict(
    POP=10,
    K=3, Q=8, U=8, T=2, O=3,
    ACC=3,
    PREP=3,
    STAT=6, STAT_STEP=8, STAT_TOK=4,
    XPOSE=15,
    LAG=5,
    W_START=0.4, W_QK=0.7, W_OP=0.5, W_SHIFT=-1,
    OP_RATE=0.55,
    V_PREP=(330, 1300), WO_PREP=(14, 1.6), GATE=(1300, 8),
)
N_S, N_U, N_C = 7, 4, 8


def rb(x):
    return x.astype(bf16).astype(f32)


def sigmoid(x):
    return 1.0 / (1.0 + jnp.exp2(x * (-LOG2E)))


def signed_sum(get, terms):
    v = get(*terms[0][:2])
    for i, j, sign in terms[1:]:
        v = v + get(i, j) if sign > 0 else v - get(i, j)
    return v


def updates(outputs):
    result = []
    for c, outs in enumerate(outputs):
        users = lambda i, j: [k for k, other in enumerate(outputs) if any(o[:2] == (i, j) for o in other)]
        result.append([(i, j, sign, c == users(i, j)[0], c == users(i, j)[-1]) for i, j, sign in outs])
    return result


PV_UPDATES = updates([step[2] for step in PV])
OP_UPDATES = updates([((step, 2, 1),) if isinstance(step, int) else step[2] for step in OP])


def attention_step(t, z_st, z_ld, q_buf, k_buf, v_buf, wo_buf, x_buf, out_buf, vt_buf, t_buf, ws_buf,
                   y_bufs, s_bufs, u_bufs, c_bufs, out_start):
    T = TIMING
    POP = T["POP"]
    n = 2 * G
    grp, half = lax.shift_right_logical(t, 1), t & 1
    heads = [grp * G + a % G for a in range(n)]
    q_blocks = [1 + heads[a] * 4 + half * 2 + a // G for a in range(n)]
    q_ld, k_ld = [z_ld + i for i in q_blocks], [z_ld + h for h in heads]
    t_ld = [z_ld + (grp & 1) * G + h for h in range(G)]
    y_st, y_ld = z_st + half, z_ld + half
    row_st, row_ld = pl.multiple_of(z_st * 64, 64), pl.multiple_of(z_ld * 64, 64)
    row0 = pl.multiple_of(half * (S // 2), S // 2)
    never = lax.broadcasted_iota(i32, (8, 128), 1) > z_st + 1000

    dots, pending, seen = [], [("op", b, c) for b in range(2) for c in range(len(OP))], 0
    for hp in range(2 * n + T["LAG"]):
        for c in range(8):
            if hp < 2 * n and c % 2 == 0:
                dots += [("qk", hp // 2, 8 * (hp % 2) + c + e) for e in range(2)]
            if hp >= T["LAG"] and c < 7:
                dots.append(("pv", (hp - T["LAG"]) // 2, 7 * ((hp - T["LAG"]) % 2) + c))
            if hp > n + T["LAG"] and c < 7:
                seen += 1
                while pending and 2 * len(OP) - len(pending) < seen * T["OP_RATE"] and (c in (1, 3, 5, 6) or hp >= 2 * n):
                    dots.append(pending.pop(0))
    dots += pending + [("op", b, c) for b in range(2, 4) for c in range(len(OP))]
    start = {d: 8 * i for i, d in enumerate(dots)}

    events, val = [], {}

    def at(slot, order):
        return lambda fn: events.append((slot, order, len(events), fn))

    def load(ref, index, r, rows):
        return pltpu.bitcast(ref.bitcast(f32)[(*index, pl.ds(r // 2, rows // 2), slice(None))], bf16)

    def token(ref, index, v=None):
        v = val.get("token") if v is None else v
        if v is not None:
            ref.bitcast(f32)[(*index, pl.ds(0, 8), slice(None))] = v

    def x_token():
        x_buf.bitcast(f32)[pl.ds(row_st + S, 4), pl.ds(0, 128)] = val["token"][:4]

    ring = lambda bufs, a, p: bufs[(2 * a + p) % len(bufs)]

    def result(d):
        if d not in val:
            kind, a, c = d
            if kind == "qk" and c % 2:
                val[d] = result((kind, a, c - 1))[128:]
            elif kind == "qk":
                k = jnp.concatenate([val.pop(("k", a, 8 * c + r)) for r in range(16)], axis=0)
                q = jnp.concatenate([val.pop(("q", d, r)) for r in range(4)], axis=1).reshape(512, DH)
                val[d] = lax.dot_general(k, q, NT, preferred_element_type=f32)
            elif kind == "pv":
                vt, pt = (jnp.concatenate([jnp.concatenate([val.pop((name, d, w, r)) for r in range(4)], axis=1)
                                           for w in range(2)], axis=0) for name in "tu")
                vt, pt = jnp.concatenate([vt[k] for k in range(8)], axis=1), pt.reshape(1024, 128)
                val[d] = jnp.dot(vt, pt, preferred_element_type=f32)
            else:
                o = jnp.concatenate([val.pop(("o", d, r)) for r in range(8)], axis=0)
                if isinstance(OP[c], int):
                    w = wo_buf[grp, :, pl.ds(512, 128)]
                elif c in OP_SUMS:
                    w = jnp.concatenate([load(ws_buf, (z_ld, 2 * OP_SUMS.index(c) + u), 0, 256) for u in range(2)], axis=1)
                else:
                    w = wo_buf[grp, pl.ds(OP[c][1][0][0] * 256, 256), pl.ds(OP[c][1][0][1] * 256, 256)]
                val[d] = jnp.dot(o, w, preferred_element_type=f32)
        return val[d]

    def scores(d):
        _, a, c = d
        j0 = start[d]
        for r in range(4 if c % 2 == 0 else 0):
            @at(j0 + r - T["Q"], 1)
            def _(r=3 - r):
                token(q_buf, (z_st, 0))
                val["q", d, r] = load(q_buf, (q_ld[a], slice(None)), 32 * r, 32)
        for r in range(8):
            @at(min(j0 + r - T["K"], j0 - c % 2 * 8 + POP - 1), 1)
            def _(r=r):
                if r == 0:
                    token(k_buf, (z_st + H,))
                val["k", a, 8 * c + r] = load(k_buf, (k_ld[a],), 128 * c + 16 * r, 16)

            @at(j0 + r + POP, 0)
            def _(r=r):
                s = result(d)[16 * r:16 * r + 16]
                for p in range(2):
                    tiles = jnp.concatenate([s[:, 256 * p:256 * p + 128], s[:, 256 * p + 128:256 * p + 256]], axis=0)
                    ring(s_bufs, a, p)[z_st, pl.ds((((c % 8) * 8 + r) * 2 + c // 8) * 32, 32), :] = tiles
                x = jnp.maximum(s[:8], s[8:])
                x = val["max"] = x if r == 0 else jnp.maximum(x, val["max"])
                if r == 7:
                    if c == 0:
                        val["stat", a] = (x, jnp.ones_like(x))
                    else:
                        m0, e0 = val["stat", a]
                        m = jnp.maximum(m0, x)
                        val["stat", a] = (m, jnp.exp2(x - m) + e0 * jnp.exp2(m0 - m))
                    val["stat token", d] = val["stat", a][1][:, 384:]
                val["token"] = s[:8, 384:]

        @at(j0 + 7 + POP + T["STAT_TOK"], 0)
        def _():
            token(q_buf, (z_st, 1), val.pop(("stat token", d)))

        for j in range(4 if c == 15 else 0):
            @at(j0 + 8 + POP + T["STAT"] + T["STAT_STEP"] * j, 0)
            def _(j=j):
                m, e = (x[:, 128 * j:128 * (j + 1)] for x in val["stat", a])
                top = jnp.max(m, axis=0, keepdims=True)
                e = jnp.broadcast_to(jnp.sum(e * jnp.exp2(m - top), axis=0, keepdims=True), (8, 128))
                shift = (0.5 * np.log2(SK) / np.log2(SK / 16)) * jnp.log2(e)
                ring(s_bufs, a, j // 2)[z_st, pl.ds(2 * SK + 8 * (j % 2), 8), :] = top + shift

    def probabilities(a, p, slot_of):
        s_buf, u_buf = ring(s_bufs, a, p), ring(u_bufs, a, p)
        for e in range(64):
            @at(slot_of(e), 1)
            def _(e=e):
                pace = jnp.where(never, val.pop("prep"), val["token"]) if "prep" in val else val["token"]
                s_buf[z_st, pl.ds(2 * SK + 16, 8), :] = pace
                m = s_buf[z_ld, pl.ds(2 * SK, 16), :]
                m0, m1 = m[:8], m[8:]
                pt = jnp.exp2(s_buf[z_ld, pl.ds(64 * e, 64), :] - jnp.concatenate([m0, m0, m1, m1] * 2, axis=0))
                pt = {(kh, j): pt[32 * kh + 16 * j:32 * kh + 16 * j + 16] for kh in range(2) for j in range(2)}
                us = [signed_sum(lambda *ix: pt[ix], terms) for _, terms, _ in PV]
                for j in range(2):
                    x = us[j][:8] + us[j][8:]
                    val["sum", a, p, j] = x if e == 0 else val["sum", a, p, j] + x
                us = jnp.concatenate(us, axis=0).reshape(7, 16, 128).astype(bf16)
                val["p", a, p, e] = (us, val["sum", a, p, 1])

            @at(slot_of(e) + T["PREP"], 0)
            def _(e=e):
                us, val["prep"] = val.pop(("p", a, p, e))
                u_buf[z_st, pl.ds(0, 7), e // 8, pl.ds(e % 8 * 16, 16), :] = us

        @at(slot_of(63) + T["PREP"] + 2, 0)
        def _():
            for j in range(2):
                l = jnp.broadcast_to(jnp.sum(val.pop(("sum", a, p, j)), axis=0, keepdims=True), (8, 128))
                r = pl.reciprocal(l, approx=True)
                ring(c_bufs, a, p)[z_st, pl.ds(256 + 8 * j, 8), :] = r * (2.0 - l * r)

    def values(d):
        _, a, c = d
        p, i = divmod(c, 7)
        j0 = start[d]
        u_buf, c_buf = ring(u_bufs, a, p), ring(c_bufs, a, p)
        outs = PV_UPDATES[i]
        for r in range(8):
            @at(j0 + r - T["U"], 1)
            def _(w=r // 4, rr=3 - r % 4):
                if rr == 3:
                    token(u_buf, (z_st, 7, 2))
                val["u", d, w, rr] = load(u_buf, (z_ld, i, pl.ds(4 * w, 4)), 32 * rr, 32)

            @at(j0 + r - T["T"], 1)
            def _(r=r):
                if r == 0:
                    token(t_buf, (z_st + 2 * G, 0, 0))
                val["t", d, r // 4, r % 4] = load(t_buf, (t_ld[a % G], i, pl.ds(r // 4 * 4, 4)), r % 4 * 16, 16)
        for r in range(4):
            @at(j0 + 4 + r + POP - T["ACC"], 1)
            def _(r=r):
                for dh, j, _, first, last in outs:
                    if not first:
                        val["c", d, r, dh, j] = c_buf[z_ld, pl.ds(128 * j + 64 * dh + 16 * r, 16), :]
                    if last:
                        val["scale", d, r, dh, j] = c_buf[z_ld, pl.ds(256 + 8 * j, 8), :]

            @at(j0 + 4 + r + POP, 0)
            def _(r=r):
                x = result(d)[16 * r:16 * r + 16]
                for dh, j, sign, first, last in outs:
                    if first:
                        y = x if sign > 0 else -x
                    else:
                        y = val.pop(("c", d, r, dh, j))
                        y = y + x if sign > 0 else y - x
                    if last:
                        y = y * jnp.concatenate([val.pop(("scale", d, r, dh, j))] * 2, axis=0)
                        u_buf[z_st, 7, j, pl.ds(64 * dh + 16 * r, 16), :] = y.astype(bf16)
                    else:
                        c_buf[z_st, pl.ds(128 * j + 64 * dh + 16 * r, 16), :] = y
                val["token"] = x[:8]
        for j in range(2 if i == 6 else 0):
            @at(j0 + 9 + POP + 4 * j, 1)
            def _(j=j):
                val["ot", d, j] = load(u_buf, (z_ld, 7, j), 0, 128).T

            @at(j0 + 9 + POP + 4 * j + T["XPOSE"], 0)
            def _(j=j):
                q_buf[z_st + q_blocks[a], 2 * p + j] = val.pop(("ot", d, j))

    def projection(d):
        _, b, c = d
        j0 = start[d]
        assert j0 - T["O"] > start["pv", b // 2 * G + G - 1, b % 2 * 7 + 6] + 13 + POP + T["XPOSE"]
        extra = isinstance(OP[c], int)
        outs = [(i, 2 * j + u, u, sign, last) for i, j, sign, _, last in OP_UPDATES[c] for u in range(1 if extra else 2)]
        rows = lambda i, r, base=0: pl.ds(base + ((2 * b + i) * 128 + 16 * r), 16)
        for r in range(8):
            @at(j0 + r - T["O"], 1)
            def _(r=r):
                token(q_buf, (z_st, 0))
                get = lambda i, h: load(q_buf, (q_ld[b // 2 * G + h], b % 2 * 2 + i), 16 * r, 16)
                if extra:
                    tiles = [get(OP[c], h) for h in range(G)]
                elif len(OP[c][0]) == 1:
                    tiles = [get(OP[c][0][0][0], 2 * OP[c][0][0][1] + u) for u in range(2)]
                else:
                    tiles = [signed_sum(lambda i, k: get(i, 2 * k + u).astype(f32), OP[c][0]).astype(bf16)
                             for u in range(2)]
                val["o", d, r] = jnp.concatenate(tiles, axis=1)

            @at(j0 + r + POP - T["ACC"], 1)
            def _(r=r):
                if r % 2 == 0 and any(last for *_, last in outs):
                    x_token()
                for i, w, _, _, last in outs:
                    val["y", d, r, i, w] = y_bufs[w][y_ld, rows(i, r), :]
                    if last:
                        val["x", d, r, i, w] = [x_buf[rows(i, r, row_ld + row0 + k * S), pl.ds(128 * w, 128)].astype(f32)
                                                for k in range(2)]

            @at(j0 + r + POP - 1, 0)
            def _(r=r):
                for i, w, u, sign, last in outs:
                    x = result(d)[16 * r:16 * r + 16, 128 * u:128 * (u + 1)]
                    y = val.pop(("y", d, r, i, w))
                    y = y + x if sign > 0 else y - x
                    y_bufs[w][y_st, rows(i, r), :] = y
                    if last:
                        x, gate = val.pop(("x", d, r, i, w))
                        out_buf[rows(i, r, row0), pl.ds(128 * w, 128)] = (x + y * gate).astype(bf16)
                val["token"] = y[:8]
                if r == 7 and c in (6, 8):
                    out_start(2 * b + (c == 8))

    for d in dots:
        {"qk": scores, "pv": values, "op": projection}[d[0]](d)

    density = {start[d] + POP + r: T["W_QK"] if d[0] == "qk" else T["W_OP"]
               for d in dots if d[0] != "pv" for r in range(8)}
    cum = np.concatenate([[0], np.cumsum([T["W_START"] if j < start["pv", 0, 0] else density.get(j - T["W_SHIFT"], 1.0)
                                          for j in range(8 * len(dots))])])
    earliest = [max(start["qk", g // 2, 15] + 9 + POP + T["STAT"] + T["STAT_STEP"] * (g % 2 * 2 + 1),
                    start["pv", (g - N_U) // 2, (g - N_U) % 2 * 7 + 6] + 8 if g >= N_U else 0) for g in range(2 * n)]
    latest = [start["pv", g // 2, g % 2 * 7] - T["U"] - T["PREP"] - 1 for g in range(2 * n)]
    edge = [cum[earliest[0]]] + [cum[j] for j in latest]
    for _ in range(200):
        for g in range(1, 2 * n):
            edge[g] = min(max((edge[g - 1] + edge[g + 1]) / 2, cum[earliest[g]]), cum[latest[g - 1]])
    for g in range(2 * n):
        assert g + N_S >= 2 * n or latest[g] < start["qk", (g + N_S) // 2, 0] + POP
        probabilities(g // 2, g % 2, lambda e: int(np.searchsorted(cum, edge[g] + (edge[g + 1] - edge[g]) * (e + 0.5) / 64)) - 1)

    step = (T["V_PREP"][1] - T["V_PREP"][0]) / 16
    for hh, k in ((hh, k) for hh in range(2) for k in range(8)):
        head = jnp.minimum(grp + 1, NG - 1) * G + 2 * half + hh
        j0 = T["V_PREP"][0] + step * (8 * hh + k)
        for kh in range(2):
            @at(j0 + step / 2 * kh, 2)
            def _(head=head, hh=hh, k=k, kh=kh):
                token(v_buf, (z_st + H,))
                val["vt", hh, k, kh] = load(v_buf, (z_ld + head,), (8 * kh + k) * 128, 128).T

            @at(j0 + step / 2 * kh + T["XPOSE"], 0)
            def _(hh=hh, k=k, kh=kh):
                vt_buf[z_st, kh] = val.pop(("vt", hh, k, kh))
        for r in range(4):
            @at(j0 + step / 2 + 1 + T["XPOSE"] + step / 9 * r, 2)
            def _(hh=hh, k=k, r=r):
                token(vt_buf, (z_st, 2))
                vt = {(dh, kh): load(vt_buf, (z_ld, kh), 64 * dh + 16 * r, 16).astype(f32)
                      for dh in range(2) for kh in range(2)}
                val["vs", hh, k, r] = [signed_sum(lambda *ix: vt[ix], terms) for terms, _, _ in PV]

            @at(j0 + step / 2 + 3 + T["XPOSE"] + step / 9 * r, 0)
            def _(hh=hh, k=k, r=r):
                x = jnp.concatenate(val.pop(("vs", hh, k, r)), axis=0)
                block = z_st + ((grp + 1) & 1) * G + 2 * half + hh
                t_buf[block, :, k, pl.ds(16 * r, 16), :] = x.reshape(7, 16, 128).astype(bf16)
                token(q_buf, (z_st, 2), x[96:104])

    for k, r in ((k, r) for k in range(len(OP_SUMS)) for r in range(16)):
        slot = T["WO_PREP"][0] + T["WO_PREP"][1] * (16 * k + r)

        @at(slot, 2)
        def _(k=k, r=r):
            for u in range(2):
                def get(i, j):
                    w = pltpu.bitcast(wo_buf[grp, pl.ds(256 * i + 16 * r, 16), pl.ds(256 * j + 128 * u, 128)], f32)
                    return pltpu.bitcast(jnp.where(never, val["token"], w), bf16).astype(f32)
                x = signed_sum(get, OP[OP_SUMS[k]][1])
                ws_buf[z_st, 2 * k + u, pl.ds(16 * r, 16), :] = x.astype(bf16)
            val["ws", k, r] = x[:8]

        @at(slot + 3, 0)
        def _(k=k, r=r):
            token(q_buf, (z_st, 3), val.pop(("ws", k, r)))

    for r, w in ((r, w) for r in range(8) for w in range(KT)):
        slot = T["GATE"][0] + T["GATE"][1] * (KT * r + w)
        assert slot + 4 < start["op", 3, 0]
        where = lambda z, r=r, w=w: (pl.ds(z + pl.multiple_of(t * 128, 128) + (S + 16 * r), 16), pl.ds(128 * w, 128))

        @at(slot, 2)
        def _(r=r, w=w, where=where):
            x_token()
            x = x_buf[where(row_ld)].astype(f32)
            val["gate", r, w] = x * sigmoid(x)

        @at(slot + 4, 0)
        def _(r=r, w=w, where=where):
            gate = val.pop(("gate", r, w))
            x_buf[where(row_st)] = gate.astype(bf16)
            token(q_buf, (z_st, 3), gate[8:])

    for *_, fn in sorted(events, key=lambda e: e[:3]):
        fn()


def kernel(x_hbm, k_hbm, v_hbm, wq_hbm, wo_hbm, wr_hbm, wg_hbm, wu_hbm, wd_hbm, out_hbm,
           x_buf, xn_buf, q_buf, k_buf, v_buf, wq_buf, wo_buf, wg_buf, wu_buf, wd_buf, out_buf,
           vt_buf, t_buf, ws_buf, y_bufs, s_bufs, u_bufs, c_bufs, wr_buf, zero_ref,
           x_sem, wq_sem, kv_sem, w_sem, out_sem):
    x_edges = (0, 1, 2, 4, 6, 8)

    def x_copy(i):
        rows = pl.ds(x_edges[i] * BX, (x_edges[i + 1] - x_edges[i]) * BX)
        return pltpu.make_async_copy(x_hbm.at[rows], x_buf.at[rows], x_sem.at[i])

    def wq_copy(j):
        return pltpu.make_async_copy(wq_hbm.at[:, pl.ds(j * G * DH, G * DH)], wq_buf.at[j], wq_sem.at[j])

    def kv_copies(late):
        k_heads, v_heads = (pl.ds(n, H - n) if late else pl.ds(0, n) for n in (G, 2 * G))
        return [pltpu.make_async_copy(k_hbm.at[k_heads], k_buf.at[k_heads], kv_sem.at[2 * late]),
                pltpu.make_async_copy(v_hbm.at[v_heads], v_buf.at[v_heads], kv_sem.at[2 * late + 1])]

    def w_copy(i):
        src, dst = ((wr_hbm, wr_buf), (wg_hbm, wg_buf), (wu_hbm, wu_buf), (wd_hbm, wd_buf), (wo_hbm, wo_buf))[i]
        return pltpu.make_async_copy(src, dst, w_sem.at[i])

    def out_copy(i):
        rows = pl.ds(i * 128, 128)
        return pltpu.make_async_copy(out_buf.at[rows], out_hbm.at[rows], out_sem.at[i])

    lane = lax.broadcasted_iota(i32, (8, 128), 1)
    sublane = lax.broadcasted_iota(i32, (8, 128), 0)
    row16 = lax.broadcasted_iota(i32, (16, D), 0)

    def layernorm(r0, n):
        x = x_buf[pl.ds(r0, n), :].astype(f32)
        mean = jnp.sum(x, axis=-1, keepdims=True)
        yield
        mean = mean * (1.0 / D)
        mean_b = rb(mean)
        xc = x - mean_b
        dm = mean - mean_b
        sq = jnp.sum(xc * xc, axis=-1, keepdims=True)
        yield
        var = jnp.broadcast_to(sq * (1.0 / D) - dm * dm, (n, 128))
        dense = var[:8]
        for k in range(1, n // 8):
            dense = jnp.where(lane == k, var[8 * k:8 * k + 8], dense)
        inv = 1.0 / rb(jnp.sqrt(rb(rb(jnp.maximum(dense, 0.0)) + EPS)))
        inv = jnp.concatenate([jnp.broadcast_to(inv[:, k:k + 1], (8, 128)) for k in range(n // 8)], axis=0)
        yield
        xc = rb(xc)
        xn = jnp.concatenate([xc[:, 128 * w:128 * (w + 1)] * inv for w in range(KT)], axis=1).astype(bf16)
        xn_buf[pl.ds(r0, n), :] = xn
        x_buf[pl.ds(S + r0, n), :] = xn

    live, started = [], [0]

    def layernorm_until(row, available):
        while started[0] - 64 * len(live) < row:
            for piece in list(live):
                if next(piece, "done") == "done":
                    live.remove(piece)
            if started[0] < available:
                live.append(layernorm(started[0], 64))
                next(live[-1])
                started[0] += 64

    def store_q(head, block, half, q):
        q = q * (DH ** -0.5 * LOG2E)
        q_buf[1 + head * 4 + block, pl.ds(2 * half, 2)] = q.reshape(2, 128, DH).astype(bf16)
        return q[:8]

    JL = NG - 3
    x_copy(0).start()
    w_copy(0).start()
    wq_copy(0).start()
    x_copy(1).start()
    zero_ref[0] = 0
    zero_ref[1] = 0
    for y_buf in y_bufs:
        y_buf[...] = jnp.zeros_like(y_buf)
    x_copy(0).wait()
    x_copy(2).start()
    w_copy(0).wait()
    layernorm_until(BX, BX)
    wq_copy(0).wait()
    x_copy(3).start()
    for i in range(NX):
        if i + 1 in x_edges[:-1]:
            part = x_edges.index(i + 1)
            if part == 1:
                x_copy(4).start()
            if part == 3:
                for j in range(1, JL + 1):
                    wq_copy(j).start()
            x_copy(part).wait()
        q = jnp.dot(xn_buf[pl.ds(i * BX, BX), :], wq_buf[0], preferred_element_type=f32)
        for h in range(G):
            store_q(h, i // 2, i % 2, q[:, h * DH:(h + 1) * DH])
        if i + 1 < NX:
            layernorm_until((i + 2) * BX, x_edges[part + 1] * BX)

    def project(j, p, sums, after=None):
        rows = lambda r: pl.ds((2 * p + r) * BX if isinstance(p, int) else pl.multiple_of((2 * p + r) * BX, BX), BX)
        xa = lambda r, k: xn_buf[rows(r), pl.ds(256 * k, 256)]
        wb = lambda k, c: wq_buf[j, pl.ds(256 * k, 256), pl.ds(256 * c, 256)]

        def operand(get, terms):
            if len(terms) == 1:
                return get(*terms[0][:2])
            return signed_sum(lambda *ix: get(*ix).astype(f32), terms).astype(bf16)

        def product(c):
            if len(OP[c][0]) > 1 and c not in sums:
                sums[c] = operand(xa, OP[c][0])
            a = sums[c] if c in sums else operand(xa, OP[c][0])
            return jnp.dot(a, operand(wb, OP[c][1]), preferred_element_type=f32)

        def rest(r, after=None):
            a = xn_buf[rows(r), pl.ds(512, 128)]
            if after is not None:
                head = jnp.where(lane > p + 1000, after, pltpu.bitcast(a[:16], f32))
                a = jnp.concatenate([pltpu.bitcast(head, bf16), a[16:]], axis=0)
            e = jnp.dot(a, wq_buf[j, pl.ds(512, 128), :], preferred_element_type=f32)
            return e[:, :256], e[:, 256:]

        def put(r, c, q):
            return [store_q(j * G + 2 * c + h, p, r, q[:, h * DH:(h + 1) * DH]) for h in range(2)][0]

        c00, c01 = rest(0, after)
        yield
        m = product(1)
        c00, c01 = c00 - m, c01 + m
        yield
        m = product(3)
        yield put(0, 1, c01 + m)
        c10, c11 = rest(1)
        c11 = c11 + m
        yield
        m = product(2)
        c10, c11 = c10 + m, c11 - m
        yield
        m = product(4)
        c00 = c00 + m
        yield put(1, 0, c10 + m)
        c00 = c00 + product(5)
        yield
        m = product(6)
        c11 = c11 + m
        yield put(0, 0, c00 + m)
        yield put(1, 1, c11 + product(7))

    def top_k(scores):
        keys = []
        for k, r in enumerate(scores):
            r = rb(r)
            r = jnp.where(r == 0.0, 0.0, r)
            bits = lax.shift_right_logical(pltpu.bitcast(r, i32), 16)
            rank = jnp.where(r != r, 0, jnp.where(bits >= 0x8000, 0xFFFF - bits, bits + 0x8000))
            tok = k * 1024 + lane * 8 + sublane
            keys.append(pltpu.bitcast(0x20000000 + rank * S + (S - 1 - tok), f32))
        chosen, rows = jnp.zeros((8, 128), i32), jnp.zeros((16, D), f32)
        for c in range(C):
            best = jnp.max(jnp.max(jnp.maximum(*keys), axis=0, keepdims=True), axis=1, keepdims=True)
            best = jnp.broadcast_to(best, (8, 128))
            keys = [jnp.where(key == best, 0.0, key) for key in keys]
            best = pltpu.bitcast(best, i32)
            chosen = jnp.where(sublane == c, best, chosen)
            tok = S - 1 - (best[0, 0] & (S - 1))
            block = xn_buf[pl.ds(pl.multiple_of(tok & -16, 16), 16), :].astype(f32)
            row = jnp.sum(jnp.where(row16 == (tok & 15), block, 0.0), axis=0, keepdims=True)
            rows = jnp.where(row16 == c, row, rows)
        return chosen, rows

    def half_of_rows(jj, carry):
        @pl.when(jj == 1)
        def _():
            for copy in kv_copies(0):
                copy.start()

        @pl.when(jj == 0)
        def _():
            for j in range(1, JL):
                wq_copy(j).wait()
            for j in range(JL + 1, NG):
                wq_copy(j).start()
            for i in range(1, 5):
                w_copy(i).start()
            wq_copy(JL).wait()

        wr = wr_buf[...].astype(f32).reshape(1, D)
        r0 = pl.multiple_of(jj * (S // 2), S // 2)
        never = lane > jj + 1000
        score, done, after = jnp.zeros((8, 128), f32), 0, None
        for unit in range(2 * JL):
            if unit % JL == 0:
                sums = {}
            for pace in project(1 + unit % JL, 2 * jj + unit // JL, sums, after if unit == 2 * JL - 1 else None):
                if pace is None or done == 64:
                    continue
                for k in (done, done + 1):
                    terms = []
                    for w in range(KT):
                        xn = pltpu.bitcast(xn_buf[pl.ds(r0 + 16 * k, 16), pl.ds(128 * w, 128)], f32)
                        xn = pltpu.bitcast(jnp.where(never, pace, xn), bf16).astype(f32)
                        terms.append(xn * wr[:, 128 * w:128 * (w + 1)])
                    r = jnp.sum(functools.reduce(lambda x, y: x + y, terms), axis=-1, keepdims=True)
                    r = jnp.broadcast_to(r, (16, 128))
                    score = jnp.where(lane == 2 * k, r[:8], jnp.where(lane == 2 * k + 1, r[8:], score))
                done += 2
                if done == 64:
                    scores = [jnp.where(jnp.full((8, 128), jj) == k, score, carry[0][k]) for k in range(2)]
                    chosen, rows = top_k(scores)
                    after = functools.reduce(lambda x, y: x + y, [rows[:8, 128 * w:128 * (w + 1)] for w in range(KT)])
        return scores, chosen, rows

    zeros = jnp.zeros((8, 128), f32)
    _, chosen, x_sel = lax.fori_loop(
        0, 2, half_of_rows, ([zeros, zeros], jnp.zeros((8, 128), i32), jnp.zeros((16, D), f32)))
    x_sel = x_sel[:8]

    for j in range(JL + 1, NG):
        wq_copy(j).wait()
    for i in range(1, 4):
        w_copy(i).wait()
    for copy in kv_copies(0):
        copy.wait()
    w_copy(4).wait()
    rank = lax.shift_right_logical(chosen - 0x20000000, 11)
    r_sel = pltpu.bitcast(lax.shift_left(jnp.where(rank >= 0x8000, rank - 0x8000, 0xFFFF - rank), 16), f32)[:, :1]
    xs = x_sel.astype(bf16)
    cols = [pl.ds(f0, min(128, F - f0)) for f0 in range(0, F, 128)]
    acc = {}

    def accumulate(key, x):
        acc[key] = acc[key] + x if key in acc else x

    def up_tile(w_buf, name, f, k):
        accumulate((name, f), lax.dot_general(xs[:, 128 * k:128 * (k + 1)], w_buf[cols[f], pl.ds(128 * k, 128)], NT,
                                              preferred_element_type=f32))

    def down_tile(f, w):
        if w == 0:
            gate = rb(acc.pop(("gate", f)))
            acc["hidden"] = (rb(gate * sigmoid(gate)) * rb(acc.pop(("up", f)))).astype(bf16)
        accumulate(w, jnp.dot(acc["hidden"], wd_buf[cols[f], pl.ds(128 * w, 128)], preferred_element_type=f32))

    tiles = [functools.partial(up_tile, w_buf, name, f, k) for f in range(len(cols))
             for name, w_buf in (("gate", wg_buf), ("up", wu_buf)) for k in range(KT)]
    tiles += [lambda: None] * 32
    tiles += [functools.partial(down_tile, f, w) for f in range(len(cols)) for w in range(KT)]
    for p in range(NX // 2):
        sums = {}
        for j in range(JL + 1, NG):
            for k, _ in enumerate(project(j, p, sums)):
                if k != 7:
                    for tile in tiles[:4]:
                        tile()
                    tiles = tiles[4:]
    assert not tiles
    y = rb(jnp.concatenate([acc[w] for w in range(KT)], axis=1))
    routed = rb(x_sel + rb(y * rb(sigmoid(r_sel))))
    for c in range(C):
        tok = S - 1 - (chosen[c, 0] & (S - 1))
        rows = pl.ds(S + pl.multiple_of(tok & -16, 16), 16)
        x_buf[rows, :] = jnp.where(row16 == (tok & 15), routed[c:c + 1, :], x_buf[rows, :].astype(f32)).astype(bf16)
    for copy in kv_copies(1):
        copy.start()
    for h in range(G):
        for k in range(8):
            vt = [v_buf[h, pl.ds((8 * kh + k) * 128, 128), :].T for kh in range(2)]
            for i, (terms, _, _) in enumerate(PV):
                x = signed_sum(lambda dh, kh: vt[kh][64 * dh:64 * (dh + 1)].astype(f32), terms)
                t_buf[h, i, k] = x.astype(bf16)

    z_st, z_ld = zero_ref[0], zero_ref[1]

    def step(t, _):
        @pl.when(t == 2)
        def _():
            for copy in kv_copies(1):
                copy.wait()

        def out_start(block):
            @pl.when(t >= 2 * NG - 2)
            def _():
                out_copy((t & 1) * 8 + block).start()

        attention_step(t, z_st, z_ld, q_buf, k_buf, v_buf, wo_buf, x_buf, out_buf, vt_buf, t_buf, ws_buf,
                       y_bufs, s_bufs, u_bufs, c_bufs, out_start)

    lax.fori_loop(0, 2 * NG, step, None)
    for i in range(S // 128):
        out_copy(i).wait()


@jax.jit
def pallas_recurrent_scan__mha_block_cached__moe_arch_mod__prompt_kernel(
    A_x: jax.Array,
    A_k_cache: jax.Array,
    A_v_cache: jax.Array,
    A_wq: jax.Array,
    A_wo: jax.Array,
    B_x: jax.Array,
    B_w_r: jax.Array,
    B_w_gate: jax.Array,
    B_w_up: jax.Array,
    B_w_down: jax.Array,
):
    del B_x
    vmem, dma = pltpu.VMEM, pltpu.SemaphoreType.DMA
    hbm = pl.BlockSpec(memory_space=pl.ANY)
    scratch = [
        vmem((2 * S + 64, D), bf16),
        vmem((S, D), bf16),
        vmem((1 + 4 * H, 4, 128, DH), bf16),
        vmem((H + 1, SK, DH), bf16),
        vmem((H + 1, SK, DH), bf16),
        vmem((NG, D, G * DH), bf16),
        vmem((NG, G * DH, D), bf16),
        vmem((F, D), bf16),
        vmem((F, D), bf16),
        vmem((F, D), bf16),
        vmem((S, D), bf16),
        vmem((1, 3, 128, 128), bf16),
        vmem((2 * G + 1, 7, 8, 64, 128), bf16),
        vmem((1, 10, 256, 128), bf16),
        [vmem((2, S // 2, 128), f32)] * KT,
        [vmem((1, 2 * SK + 32, 128), f32)] * N_S,
        [vmem((1, 8, 8, 128, 128), bf16)] * N_U,
        [vmem((1, 288, 128), f32)] * N_C,
        vmem((D,), bf16),
        pltpu.SMEM((2,), i32),
        dma((5,)), dma((NG,)), dma((4,)), dma((5,)), dma((S // 128,)),
    ]
    out = pl.pallas_call(
        kernel,
        in_specs=[hbm] * 9,
        out_specs=hbm,
        out_shape=jax.ShapeDtypeStruct((S, D), bf16),
        scratch_shapes=scratch,
        compiler_params=pltpu.CompilerParams(vmem_limit_bytes=126 * 1024 * 1024),
        name="fused_kernel",
    )(A_x.reshape(S, D), A_k_cache.reshape(H, SK, DH), A_v_cache.reshape(H, SK, DH), A_wq,
      A_wo.reshape(NG, G * DH, D), B_w_r, B_w_gate.T, B_w_up.T, B_w_down)
    return out.reshape(1, S, D)
```

```python
import functools

import jax
import jax.experimental.pallas as pl
import jax.experimental.pallas.tpu as pltpu
import jax.numpy as jnp
import numpy as np
from jax import lax

S, D, H, DH, SK, F, C = 2048, 640, 32, 128, 2048, 1728, 8
KT = D // 128
G = 4
NG = H // G
BX = 256
NX = S // BX
LOG2E = 1.4426950408889634
EPS = float(np.asarray(1e-5, dtype=jnp.bfloat16))
f32, bf16, i32 = jnp.float32, jnp.bfloat16, jnp.int32
NT = (((1,), (1,)), ((), ()))

PV = [
    (((1, 1, 1),), ((0, 0, 1), (1, 0, 1)), ((0, 0, -1), (1, 0, 1))),
    (((0, 0, 1),), ((0, 1, 1), (1, 1, 1)), ((0, 1, 1), (1, 1, -1))),
    (((1, 0, 1), (1, 1, -1)), ((0, 0, 1),), ((1, 0, 1), (1, 1, 1))),
    (((0, 1, 1), (0, 0, -1)), ((1, 1, 1),), ((0, 0, 1), (0, 1, 1))),
    (((0, 1, 1), (1, 1, 1)), ((1, 0, 1), (1, 1, -1)), ((0, 0, 1),)),
    (((0, 0, 1), (1, 1, 1)), ((0, 0, 1), (1, 1, 1)), ((0, 0, 1), (1, 1, 1))),
    (((0, 0, 1), (1, 0, 1)), ((0, 1, 1), (0, 0, -1)), ((1, 1, 1),)),
]
OP = [
    0,
    (((0, 0, 1), (0, 1, 1)), ((1, 1, 1),), ((0, 0, -1), (0, 1, 1))),
    (((1, 0, 1), (1, 1, 1)), ((0, 0, 1),), ((1, 0, 1), (1, 1, -1))),
    (((0, 0, 1),), ((0, 1, 1), (1, 1, -1)), ((0, 1, 1), (1, 1, 1))),
    (((1, 1, 1),), ((1, 0, 1), (0, 0, -1)), ((0, 0, 1), (1, 0, 1))),
    (((0, 1, 1), (1, 1, -1)), ((1, 0, 1), (1, 1, 1)), ((0, 0, 1),)),
    (((0, 0, 1), (1, 1, 1)), ((0, 0, 1), (1, 1, 1)), ((0, 0, 1), (1, 1, 1))),
    (((1, 0, 1), (0, 0, -1)), ((0, 0, 1), (0, 1, 1)), ((1, 1, 1),)),
    1,
]

TIMING = dict(
    POP=10,
    K=3, Q=8, U=8, T=2, O=3, W=8,
    ACC=3,
    PREP=3,
    STAT=6, STAT_STEP=8, STAT_TOK=4,
    XPOSE=15,
    LAG=5,
    W_START=0.4, W_QK=0.7, W_OP=0.5, W_SHIFT=-1,
    OP_RATE=0.55,
    V_PREP=(330, 1300), WO_PREP=(14, 1.2), GATE=(1300, 8),
)
N_S, N_U, N_C = 7, 4, 8


def rb(x):
    return x.astype(bf16).astype(f32)


def sigmoid(x):
    return 1.0 / (1.0 + jnp.exp2(x * (-LOG2E)))


def signed_sum(get, terms):
    v = get(*terms[0][:2])
    for i, j, sign in terms[1:]:
        v = v + get(i, j) if sign > 0 else v - get(i, j)
    return v


def updates(outputs):
    result = []
    for c, outs in enumerate(outputs):
        users = lambda i, j: [k for k, other in enumerate(outputs) if any(o[:2] == (i, j) for o in other)]
        result.append([(i, j, sign, c == users(i, j)[0], c == users(i, j)[-1]) for i, j, sign in outs])
    return result


PV_UPDATES = updates([step[2] for step in PV])
OP_UPDATES = updates([((step, 2, 1),) if isinstance(step, int) else step[2] for step in OP])


def attention_step(t, z_st, z_ld, q_buf, k_buf, v_buf, wo_buf, x_buf, g_buf, out_buf, vt_buf, t_buf, ws_buf,
                   y_bufs, s_bufs, u_bufs, c_bufs, out_start):
    T = TIMING
    POP = T["POP"]
    n = 2 * G
    grp, half = lax.shift_right_logical(t, 1), t & 1
    heads = [grp * G + a % G for a in range(n)]
    q_blocks = [1 + heads[a] * 4 + half * 2 + a // G for a in range(n)]
    q_ld, k_ld = [z_ld + i for i in q_blocks], [z_ld + h for h in heads]
    t_ld = [z_ld + (grp & 1) * G + h for h in range(G)]
    y_st, y_ld = z_st + half, z_ld + half
    row_st, row_ld = pl.multiple_of(z_st * 64, 64), pl.multiple_of(z_ld * 64, 64)
    x_rows = row_ld + pl.multiple_of(half * (S // 2), S // 2)
    never = lax.broadcasted_iota(i32, (8, 128), 1) > z_st + 1000

    dots, pending, seen = [], [("op", b, c) for b in range(2) for c in range(len(OP))], 0
    for hp in range(2 * n + T["LAG"]):
        for c in range(8):
            if hp < 2 * n and c % 2 == 0:
                dots += [("qk", hp // 2, 8 * (hp % 2) + c + e) for e in range(2)]
            if hp >= T["LAG"] and c < 7:
                dots.append(("pv", (hp - T["LAG"]) // 2, 7 * ((hp - T["LAG"]) % 2) + c))
            if hp > n + T["LAG"] and c < 7:
                seen += 1
                while pending and 2 * len(OP) - len(pending) < seen * T["OP_RATE"] and (c in (1, 3, 5, 6) or hp >= 2 * n):
                    dots.append(pending.pop(0))
    dots += pending + [("op", b, c) for b in range(2, 4) for c in range(len(OP))]
    start = {d: 8 * i for i, d in enumerate(dots)}

    events, val = [], {}

    def at(slot, order):
        return lambda fn: events.append((slot, order, len(events), fn))

    def load(ref, index, r, rows):
        return pltpu.bitcast(ref.bitcast(f32)[(*index, pl.ds(r // 2, rows // 2), slice(None))], bf16)

    def token(ref, index, v=None):
        v = val.get("token") if v is None else v
        if v is not None:
            ref.bitcast(f32)[(*index, pl.ds(0, 8), slice(None))] = v

    def x_token():
        x_buf.bitcast(f32)[pl.ds(row_st + S // 2, 4), pl.ds(0, 128)] = val["token"][:4]
        token(g_buf, (z_st + 2, 0))

    ring = lambda bufs, a, p: bufs[(2 * a + p) % len(bufs)]

    def result(d):
        if d not in val:
            kind, a, c = d
            if kind == "qk" and c % 2:
                val[d] = result((kind, a, c - 1))[128:]
            elif kind == "qk":
                k = jnp.concatenate([val.pop(("k", a, 8 * c + r)) for r in range(16)], axis=0)
                q = jnp.concatenate([val.pop(("q", d, r)) for r in range(4)], axis=1).reshape(512, DH)
                val[d] = lax.dot_general(k, q, NT, preferred_element_type=f32)
            elif kind == "pv":
                vt, pt = (jnp.concatenate([jnp.concatenate([val.pop((name, d, w, r)) for r in range(4)], axis=1)
                                           for w in range(2)], axis=0) for name in "tu")
                vt, pt = jnp.concatenate([vt[k] for k in range(8)], axis=1), pt.reshape(1024, 128)
                val[d] = jnp.dot(vt, pt, preferred_element_type=f32)
            else:
                o = jnp.concatenate([val.pop(("o", d, r)) for r in range(8)], axis=0)
                w = jnp.concatenate([val.pop(("w", d, r)) for r in range(4)], axis=1)
                if isinstance(OP[c], int):
                    w = w.reshape(512, 128)
                else:
                    w = jnp.concatenate([w[2 * u:2 * u + 2].reshape(256, 128) for u in range(2)], axis=1)
                val[d] = jnp.dot(o, w, preferred_element_type=f32)
        return val[d]

    def scores(d):
        _, a, c = d
        j0 = start[d]
        for r in range(4 if c % 2 == 0 else 0):
            @at(j0 + r - T["Q"], 1)
            def _(r=3 - r):
                token(q_buf, (z_st, 0))
                val["q", d, r] = load(q_buf, (q_ld[a], slice(None)), 32 * r, 32)
        for r in range(8):
            @at(min(j0 + r - T["K"], j0 - c % 2 * 8 + POP - 1), 1)
            def _(r=r):
                if r == 0:
                    token(k_buf, (z_st + H,))
                val["k", a, 8 * c + r] = load(k_buf, (k_ld[a],), 128 * c + 16 * r, 16)

            @at(j0 + r + POP, 0)
            def _(r=r):
                s = result(d)[16 * r:16 * r + 16]
                for p in range(2):
                    tiles = jnp.concatenate([s[:, 256 * p:256 * p + 128], s[:, 256 * p + 128:256 * p + 256]], axis=0)
                    ring(s_bufs, a, p)[z_st, pl.ds((((c % 8) * 8 + r) * 2 + c // 8) * 32, 32), :] = tiles
                x = jnp.maximum(s[:8], s[8:])
                x = val["max"] = x if r == 0 else jnp.maximum(x, val["max"])
                if r == 7:
                    if c == 0:
                        val["stat", a] = (x, jnp.ones_like(x))
                    else:
                        m0, e0 = val["stat", a]
                        m = jnp.maximum(m0, x)
                        val["stat", a] = (m, jnp.exp2(x - m) + e0 * jnp.exp2(m0 - m))
                    val["stat token", d] = val["stat", a][1][:, 384:]
                val["token"] = s[:8, 384:]

        @at(j0 + 7 + POP + T["STAT_TOK"], 0)
        def _():
            token(q_buf, (z_st, 1), val.pop(("stat token", d)))

        for j in range(4 if c == 15 else 0):
            @at(j0 + 8 + POP + T["STAT"] + T["STAT_STEP"] * j, 0)
            def _(j=j):
                m, e = (x[:, 128 * j:128 * (j + 1)] for x in val["stat", a])
                top = jnp.max(m, axis=0, keepdims=True)
                e = jnp.broadcast_to(jnp.sum(e * jnp.exp2(m - top), axis=0, keepdims=True), (8, 128))
                shift = (0.5 * np.log2(SK) / np.log2(SK / 16)) * jnp.log2(e)
                ring(s_bufs, a, j // 2)[z_st, pl.ds(2 * SK + 8 * (j % 2), 8), :] = top + shift

    def probabilities(a, p, slot_of):
        s_buf, u_buf = ring(s_bufs, a, p), ring(u_bufs, a, p)
        for e in range(64):
            @at(slot_of(e), 1)
            def _(e=e):
                pace = jnp.where(never, val.pop("prep"), val["token"]) if "prep" in val else val["token"]
                s_buf[z_st, pl.ds(2 * SK + 16, 8), :] = pace
                m = s_buf[z_ld, pl.ds(2 * SK, 16), :]
                m0, m1 = m[:8], m[8:]
                pt = jnp.exp2(s_buf[z_ld, pl.ds(64 * e, 64), :] - jnp.concatenate([m0, m0, m1, m1] * 2, axis=0))
                pt = {(kh, j): pt[32 * kh + 16 * j:32 * kh + 16 * j + 16] for kh in range(2) for j in range(2)}
                us = [signed_sum(lambda *ix: pt[ix], terms) for _, terms, _ in PV]
                for j in range(2):
                    x = us[j][:8] + us[j][8:]
                    val["sum", a, p, j] = x if e == 0 else val["sum", a, p, j] + x
                us = jnp.concatenate(us, axis=0).reshape(7, 16, 128).astype(bf16)
                val["p", a, p, e] = (us, val["sum", a, p, 1])

            @at(slot_of(e) + T["PREP"], 0)
            def _(e=e):
                us, val["prep"] = val.pop(("p", a, p, e))
                u_buf[z_st, pl.ds(0, 7), e // 8, pl.ds(e % 8 * 16, 16), :] = us

        @at(slot_of(63) + T["PREP"] + 2, 0)
        def _():
            for j in range(2):
                l = jnp.broadcast_to(jnp.sum(val.pop(("sum", a, p, j)), axis=0, keepdims=True), (8, 128))
                r = pl.reciprocal(l, approx=True)
                ring(c_bufs, a, p)[z_st, pl.ds(256 + 8 * j, 8), :] = r * (2.0 - l * r)

    def values(d):
        _, a, c = d
        p, i = divmod(c, 7)
        j0 = start[d]
        u_buf, c_buf = ring(u_bufs, a, p), ring(c_bufs, a, p)
        outs = PV_UPDATES[i]
        for r in range(8):
            @at(j0 + r - T["U"], 1)
            def _(w=r // 4, rr=3 - r % 4):
                if rr == 3:
                    token(u_buf, (z_st, 7, 2))
                val["u", d, w, rr] = load(u_buf, (z_ld, i, pl.ds(4 * w, 4)), 32 * rr, 32)

            @at(j0 + r - T["T"], 1)
            def _(r=r):
                if r == 0:
                    token(t_buf, (z_st + 2 * G, 0, 0))
                val["t", d, r // 4, r % 4] = load(t_buf, (t_ld[a % G], i, pl.ds(r // 4 * 4, 4)), r % 4 * 16, 16)
        for r in range(4):
            @at(j0 + 4 + r + POP - T["ACC"], 1)
            def _(r=r):
                for dh, j, _, first, last in outs:
                    if not first:
                        val["c", d, r, dh, j] = c_buf[z_ld, pl.ds(128 * j + 64 * dh + 16 * r, 16), :]
                    if last:
                        val["scale", d, r, dh, j] = c_buf[z_ld, pl.ds(256 + 8 * j, 8), :]

            @at(j0 + 4 + r + POP, 0)
            def _(r=r):
                x = result(d)[16 * r:16 * r + 16]
                for dh, j, sign, first, last in outs:
                    if first:
                        y = x if sign > 0 else -x
                    else:
                        y = val.pop(("c", d, r, dh, j))
                        y = y + x if sign > 0 else y - x
                    if last:
                        y = y * jnp.concatenate([val.pop(("scale", d, r, dh, j))] * 2, axis=0)
                        u_buf[z_st, 7, j, pl.ds(64 * dh + 16 * r, 16), :] = y.astype(bf16)
                    else:
                        c_buf[z_st, pl.ds(128 * j + 64 * dh + 16 * r, 16), :] = y
                val["token"] = x[:8]
        for j in range(2 if i == 6 else 0):
            @at(j0 + 9 + POP + 4 * j, 1)
            def _(j=j):
                val["ot", d, j] = load(u_buf, (z_ld, 7, j), 0, 128).T

            @at(j0 + 9 + POP + 4 * j + T["XPOSE"], 0)
            def _(j=j):
                q_buf[z_st + q_blocks[a], 2 * p + j] = val.pop(("ot", d, j))

    def projection(d):
        _, b, c = d
        j0 = start[d]
        assert j0 - T["O"] > start["pv", b // 2 * G + G - 1, b % 2 * 7 + 6] + 13 + POP + T["XPOSE"]
        extra = isinstance(OP[c], int)
        outs = [(i, 2 * j + u, u, sign, last) for i, j, sign, _, last in OP_UPDATES[c] for u in range(1 if extra else 2)]
        rows = lambda i, r, base=0: pl.ds(base + ((2 * b + i) * 128 + 16 * r), 16)
        for r in range(4):
            @at(j0 + r - T["W"], 1)
            def _(r=3 - r):
                if r % 2 == 1:
                    token(ws_buf, (z_st, 8, 0))
                val["w", d, r] = load(ws_buf, (z_ld, c % 8, slice(None)), 32 * r, 32)
        for r in range(8):
            @at(j0 + r - T["O"], 1)
            def _(r=r):
                token(q_buf, (z_st, 0))
                get = lambda i, h: load(q_buf, (q_ld[b // 2 * G + h], b % 2 * 2 + i), 16 * r, 16)
                if extra:
                    tiles = [get(OP[c], h) for h in range(G)]
                elif len(OP[c][0]) == 1:
                    tiles = [get(OP[c][0][0][0], 2 * OP[c][0][0][1] + u) for u in range(2)]
                else:
                    tiles = [signed_sum(lambda i, k: get(i, 2 * k + u).astype(f32), OP[c][0]).astype(bf16)
                             for u in range(2)]
                val["o", d, r] = jnp.concatenate(tiles, axis=1)

            @at(j0 + r + POP - T["ACC"], 1)
            def _(r=r):
                if r % 2 == 0 and any(last for *_, last in outs):
                    x_token()
                for i, w, _, _, last in outs:
                    val["y", d, r, i, w] = y_bufs[w][y_ld, rows(i, r), :]
                    if last:
                        val["x", d, r, i, w] = (x_buf[rows(i, r, x_rows), pl.ds(128 * w, 128)].astype(f32),
                                                load(g_buf, (y_ld, w), (2 * b + i) * 128 + 16 * r, 16).astype(f32))

            @at(j0 + r + POP - 1, 0)
            def _(r=r):
                for i, w, u, sign, last in outs:
                    x = result(d)[16 * r:16 * r + 16, 128 * u:128 * (u + 1)]
                    y = val.pop(("y", d, r, i, w))
                    y = y + x if sign > 0 else y - x
                    y_bufs[w][y_st, rows(i, r), :] = y
                    if last:
                        x, gate = val.pop(("x", d, r, i, w))
                        out_buf[w, half * 8 + 2 * b + i, pl.ds(16 * r, 16), :] = (x + y * gate).astype(bf16)
                val["token"] = y[:8]
                if r == 7 and c in (6, 8):
                    out_start(2 * b + (c == 8))

    for d in dots:
        {"qk": scores, "pv": values, "op": projection}[d[0]](d)

    density = {start[d] + POP + r: T["W_QK"] if d[0] == "qk" else T["W_OP"]
               for d in dots if d[0] != "pv" for r in range(8)}
    cum = np.concatenate([[0], np.cumsum([T["W_START"] if j < start["pv", 0, 0] else density.get(j - T["W_SHIFT"], 1.0)
                                          for j in range(8 * len(dots))])])
    earliest = [max(start["qk", g // 2, 15] + 9 + POP + T["STAT"] + T["STAT_STEP"] * (g % 2 * 2 + 1),
                    start["pv", (g - N_U) // 2, (g - N_U) % 2 * 7 + 6] + 8 if g >= N_U else 0) for g in range(2 * n)]
    latest = [start["pv", g // 2, g % 2 * 7] - T["U"] - T["PREP"] - 1 for g in range(2 * n)]
    edge = [cum[earliest[0]]] + [cum[j] for j in latest]
    for _ in range(200):
        for g in range(1, 2 * n):
            edge[g] = min(max((edge[g - 1] + edge[g + 1]) / 2, cum[earliest[g]]), cum[latest[g - 1]])
    for g in range(2 * n):
        assert g + N_S >= 2 * n or latest[g] < start["qk", (g + N_S) // 2, 0] + POP
        probabilities(g // 2, g % 2, lambda e: int(np.searchsorted(cum, edge[g] + (edge[g + 1] - edge[g]) * (e + 0.5) / 64)) - 1)

    step = (T["V_PREP"][1] - T["V_PREP"][0]) / 16
    for hh, k in ((hh, k) for hh in range(2) for k in range(8)):
        head = jnp.minimum(grp + 1, NG - 1) * G + 2 * half + hh
        j0 = T["V_PREP"][0] + step * (8 * hh + k)
        for kh in range(2):
            @at(j0 + step / 2 * kh, 2)
            def _(head=head, hh=hh, k=k, kh=kh):
                token(v_buf, (z_st + H,))
                val["vt", hh, k, kh] = load(v_buf, (z_ld + head,), (8 * kh + k) * 128, 128).T

            @at(j0 + step / 2 * kh + T["XPOSE"], 0)
            def _(hh=hh, k=k, kh=kh):
                vt_buf[z_st, kh] = val.pop(("vt", hh, k, kh))
        for r in range(4):
            @at(j0 + step / 2 + 1 + T["XPOSE"] + step / 9 * r, 2)
            def _(hh=hh, k=k, r=r):
                token(vt_buf, (z_st, 2))
                vt = {(dh, kh): load(vt_buf, (z_ld, kh), 64 * dh + 16 * r, 16).astype(f32)
                      for dh in range(2) for kh in range(2)}
                val["vs", hh, k, r] = [signed_sum(lambda *ix: vt[ix], terms) for terms, _, _ in PV]

            @at(j0 + step / 2 + 3 + T["XPOSE"] + step / 9 * r, 0)
            def _(hh=hh, k=k, r=r):
                x = jnp.concatenate(val.pop(("vs", hh, k, r)), axis=0)
                block = z_st + ((grp + 1) & 1) * G + 2 * half + hh
                t_buf[block, :, k, pl.ds(16 * r, 16), :] = x.reshape(7, 16, 128).astype(bf16)
                token(q_buf, (z_st, 2), x[96:104])

    for k, r in ((k, r) for k in range(8) for r in range(16)):
        slot = T["WO_PREP"][0] + T["WO_PREP"][1] * (16 * k + r)

        @at(slot, 2)
        def _(k=k, r=r):
            def get(row, col):
                w = pltpu.bitcast(wo_buf[grp, pl.ds(row, 16), pl.ds(col, 128)], f32)
                return jnp.where(never, val["token"], w)
            for u in range(2):
                if k == 0 or len(OP[k][1]) == 1:
                    row, col = (256 * u, 512) if k == 0 else (256 * OP[k][1][0][0], 256 * OP[k][1][0][1] + 128 * u)
                    x = get(row + 16 * r, col)
                    ws_buf.bitcast(f32)[z_st, k, 2 * u + r // 8, pl.ds(r % 8 * 8, 8), :] = x
                else:
                    x = signed_sum(lambda i, j: pltpu.bitcast(get(256 * i + 16 * r, 256 * j + 128 * u), bf16).astype(f32),
                                   OP[k][1])
                    ws_buf[z_st, k, 2 * u + r // 8, pl.ds(r % 8 * 16, 16), :] = x.astype(bf16)
            val["ws", k, r] = x[:8]

        @at(slot + 3, 0)
        def _(k=k, r=r):
            token(q_buf, (z_st, 3), val.pop(("ws", k, r)))

    for r, w in ((r, w) for r in range(8) for w in range(KT)):
        slot = T["GATE"][0] + T["GATE"][1] * (KT * r + w)
        assert slot + 4 < start["op", 3, 0]
        where = lambda z, r=r, w=w: (z + lax.shift_right_logical(t, 3), w, pl.ds(pl.multiple_of((t & 7) * 128 + 16 * r, 16), 16))

        @at(slot, 2)
        def _(r=r, w=w, where=where):
            token(g_buf, (z_st + 2, 0))
            x = g_buf[where(z_ld)].astype(f32)
            val["gate", r, w] = x * sigmoid(x)

        @at(slot + 4, 0)
        def _(r=r, w=w, where=where):
            gate = val.pop(("gate", r, w))
            g_buf[where(z_st)] = gate.astype(bf16)
            token(q_buf, (z_st, 3), gate[8:])

    for *_, fn in sorted(events, key=lambda e: e[:3]):
        fn()


def kernel(x_hbm, k_hbm, v_hbm, wq_hbm, wo_hbm, wr_hbm, wg_hbm, wu_hbm, wd_hbm, out_hbm,
           x_buf, xn_buf, g_buf, q_buf, k_buf, v_buf, wq_buf, wo_buf, wg_buf, wu_buf, wd_buf, out_buf,
           vt_buf, t_buf, ws_buf, y_bufs, s_bufs, u_bufs, c_bufs, wr_buf, zero_ref,
           x_sem, wq_sem, kv_sem, w_sem, out_sem):
    x_edges = (0, 1, 2, 4, 6, 8)

    def x_copy(i):
        rows = pl.ds(x_edges[i] * BX, (x_edges[i + 1] - x_edges[i]) * BX)
        return pltpu.make_async_copy(x_hbm.at[rows], x_buf.at[rows], x_sem.at[i])

    def wq_copy(j):
        return pltpu.make_async_copy(wq_hbm.at[:, pl.ds(j * G * DH, G * DH)], wq_buf.at[j], wq_sem.at[j])

    def kv_copies(late):
        k_heads, v_heads = (pl.ds(n, H - n) if late else pl.ds(0, n) for n in (G, 2 * G))
        return [pltpu.make_async_copy(k_hbm.at[k_heads], k_buf.at[k_heads], kv_sem.at[2 * late]),
                pltpu.make_async_copy(v_hbm.at[v_heads], v_buf.at[v_heads], kv_sem.at[2 * late + 1])]

    def w_copy(i):
        src, dst = ((wr_hbm, wr_buf), (wg_hbm, wg_buf), (wu_hbm, wu_buf), (wd_hbm, wd_buf), (wo_hbm, wo_buf))[i]
        return pltpu.make_async_copy(src, dst, w_sem.at[i])

    def out_copy(i):
        return [pltpu.make_async_copy(out_buf.at[w, i], out_hbm.at[pl.ds(i * 128, 128), pl.ds(128 * w, 128)], out_sem.at[0])
                for w in range(KT)]

    lane = lax.broadcasted_iota(i32, (8, 128), 1)
    sublane = lax.broadcasted_iota(i32, (8, 128), 0)
    row16 = lax.broadcasted_iota(i32, (16, D), 0)

    def layernorm(r0, n):
        x = x_buf[pl.ds(r0, n), :].astype(f32)
        mean = jnp.sum(x, axis=-1, keepdims=True)
        yield
        mean = mean * (1.0 / D)
        mean_b = rb(mean)
        xc = x - mean_b
        dm = mean - mean_b
        sq = jnp.sum(xc * xc, axis=-1, keepdims=True)
        yield
        var = jnp.broadcast_to(sq * (1.0 / D) - dm * dm, (n, 128))
        dense = var[:8]
        for k in range(1, n // 8):
            dense = jnp.where(lane == k, var[8 * k:8 * k + 8], dense)
        inv = 1.0 / rb(jnp.sqrt(rb(rb(jnp.maximum(dense, 0.0)) + EPS)))
        inv = jnp.concatenate([jnp.broadcast_to(inv[:, k:k + 1], (8, 128)) for k in range(n // 8)], axis=0)
        yield
        xc = rb(xc)
        for w in range(KT):
            xn = (xc[:, 128 * w:128 * (w + 1)] * inv).astype(bf16)
            xn_buf[w, pl.ds(r0, n), :] = xn
            g_buf[r0 // 1024, w, pl.ds(r0 % 1024, n), :] = xn

    def load_xn(r0, n, tiles):
        rows = pl.ds(r0 // 2 if isinstance(r0, int) else pl.multiple_of(lax.shift_right_logical(r0, 1), 8), n // 2)
        return jnp.concatenate([pltpu.bitcast(xn_buf.bitcast(f32)[w, rows, :], bf16) for w in tiles], axis=1)

    live, started = [], [0]

    def layernorm_until(row, available):
        while started[0] - 64 * len(live) < row:
            for piece in list(live):
                if next(piece, "done") == "done":
                    live.remove(piece)
            if started[0] < available:
                live.append(layernorm(started[0], 64))
                next(live[-1])
                started[0] += 64

    def store_q(head, block, half, q):
        q = q * (DH ** -0.5 * LOG2E)
        q_buf[1 + head * 4 + block, pl.ds(2 * half, 2)] = q.reshape(2, 128, DH).astype(bf16)
        return q[:8]

    JL = NG - 3
    x_copy(0).start()
    w_copy(0).start()
    wq_copy(0).start()
    x_copy(1).start()
    zero_ref[0] = 0
    zero_ref[1] = 0
    for y_buf in y_bufs:
        y_buf[...] = jnp.zeros_like(y_buf)
    x_copy(0).wait()
    x_copy(2).start()
    w_copy(0).wait()
    layernorm_until(BX, BX)
    wq_copy(0).wait()
    x_copy(3).start()
    for i in range(NX):
        if i + 1 in x_edges[:-1]:
            part = x_edges.index(i + 1)
            if part == 1:
                x_copy(4).start()
            if part == 3:
                for j in range(1, JL + 1):
                    wq_copy(j).start()
            x_copy(part).wait()
        q = jnp.dot(load_xn(i * BX, BX, range(KT)), wq_buf[0], preferred_element_type=f32)
        for h in range(G):
            store_q(h, i // 2, i % 2, q[:, h * DH:(h + 1) * DH])
        if i + 1 < NX:
            layernorm_until((i + 2) * BX, x_edges[part + 1] * BX)

    def project(j, p, sums, after=None):
        xa = lambda r, k: load_xn((2 * p + r) * BX, BX, (2 * k, 2 * k + 1))
        wb = lambda k, c: wq_buf[j, pl.ds(256 * k, 256), pl.ds(256 * c, 256)]

        def operand(get, terms):
            if len(terms) == 1:
                return get(*terms[0][:2])
            return signed_sum(lambda *ix: get(*ix).astype(f32), terms).astype(bf16)

        def product(c):
            if len(OP[c][0]) > 1 and c not in sums:
                sums[c] = operand(xa, OP[c][0])
            a = sums[c] if c in sums else operand(xa, OP[c][0])
            return jnp.dot(a, operand(wb, OP[c][1]), preferred_element_type=f32)

        def rest(r, after=None):
            a = load_xn((2 * p + r) * BX, BX, (4,))
            if after is not None:
                head = jnp.where(lane > p + 1000, after, pltpu.bitcast(a[:16], f32))
                a = jnp.concatenate([pltpu.bitcast(head, bf16), a[16:]], axis=0)
            e = jnp.dot(a, wq_buf[j, pl.ds(512, 128), :], preferred_element_type=f32)
            return e[:, :256], e[:, 256:]

        def put(r, c, q):
            return [store_q(j * G + 2 * c + h, p, r, q[:, h * DH:(h + 1) * DH]) for h in range(2)][0]

        c00, c01 = rest(0, after)
        yield
        m = product(1)
        c00, c01 = c00 - m, c01 + m
        yield
        m = product(3)
        yield put(0, 1, c01 + m)
        c10, c11 = rest(1)
        c11 = c11 + m
        yield
        m = product(2)
        c10, c11 = c10 + m, c11 - m
        yield
        m = product(4)
        c00 = c00 + m
        yield put(1, 0, c10 + m)
        c00 = c00 + product(5)
        yield
        m = product(6)
        c11 = c11 + m
        yield put(0, 0, c00 + m)
        yield put(1, 1, c11 + product(7))

    def top_k(scores):
        keys = []
        for k, r in enumerate(scores):
            r = rb(r)
            r = jnp.where(r == 0.0, 0.0, r)
            bits = lax.shift_right_logical(pltpu.bitcast(r, i32), 16)
            rank = jnp.where(r != r, 0, jnp.where(bits >= 0x8000, 0xFFFF - bits, bits + 0x8000))
            tok = k * 1024 + lane * 8 + sublane
            keys.append(pltpu.bitcast(0x20000000 + rank * S + (S - 1 - tok), f32))
        chosen, rows = jnp.zeros((8, 128), i32), jnp.zeros((16, D), f32)
        for c in range(C):
            best = jnp.max(jnp.max(jnp.maximum(*keys), axis=0, keepdims=True), axis=1, keepdims=True)
            best = jnp.broadcast_to(best, (8, 128))
            keys = [jnp.where(key == best, 0.0, key) for key in keys]
            best = pltpu.bitcast(best, i32)
            chosen = jnp.where(sublane == c, best, chosen)
            tok = S - 1 - (best[0, 0] & (S - 1))
            block = load_xn(tok & -16, 16, range(KT)).astype(f32)
            row = jnp.sum(jnp.where(row16 == (tok & 15), block, 0.0), axis=0, keepdims=True)
            rows = jnp.where(row16 == c, row, rows)
        return chosen, rows

    def half_of_rows(jj, carry):
        @pl.when(jj == 1)
        def _():
            for copy in kv_copies(0):
                copy.start()

        @pl.when(jj == 0)
        def _():
            for j in range(1, JL):
                wq_copy(j).wait()
            for j in range(JL + 1, NG):
                wq_copy(j).start()
            for i in range(1, 5):
                w_copy(i).start()
            wq_copy(JL).wait()

        wr = wr_buf[...].astype(f32).reshape(1, D)
        r0 = pl.multiple_of(jj * (S // 4), S // 4)
        never = lane > jj + 1000
        score, done, after = jnp.zeros((8, 128), f32), 0, None
        for unit in range(2 * JL):
            if unit % JL == 0:
                sums = {}
            for pace in project(1 + unit % JL, 2 * jj + unit // JL, sums, after if unit == 2 * JL - 1 else None):
                if pace is None or done == 64:
                    continue
                for k in (done, done + 1):
                    terms = []
                    for w in range(KT):
                        xn = xn_buf.bitcast(f32)[w, pl.ds(r0 + 8 * k, 8), :]
                        xn = pltpu.bitcast(jnp.where(never, pace, xn), bf16).astype(f32)
                        terms.append(xn * wr[:, 128 * w:128 * (w + 1)])
                    r = jnp.sum(functools.reduce(lambda x, y: x + y, terms), axis=-1, keepdims=True)
                    r = jnp.broadcast_to(r, (16, 128))
                    score = jnp.where(lane == 2 * k, r[:8], jnp.where(lane == 2 * k + 1, r[8:], score))
                done += 2
                if done == 64:
                    scores = [jnp.where(jnp.full((8, 128), jj) == k, score, carry[0][k]) for k in range(2)]
                    chosen, rows = top_k(scores)
                    after = functools.reduce(lambda x, y: x + y, [rows[:8, 128 * w:128 * (w + 1)] for w in range(KT)])
        return scores, chosen, rows

    zeros = jnp.zeros((8, 128), f32)
    _, chosen, x_sel = lax.fori_loop(
        0, 2, half_of_rows, ([zeros, zeros], jnp.zeros((8, 128), i32), jnp.zeros((16, D), f32)))
    x_sel = x_sel[:8]

    for j in range(JL + 1, NG):
        wq_copy(j).wait()
    for i in range(1, 4):
        w_copy(i).wait()
    for copy in kv_copies(0):
        copy.wait()
    w_copy(4).wait()
    rank = lax.shift_right_logical(chosen - 0x20000000, 11)
    r_sel = pltpu.bitcast(lax.shift_left(jnp.where(rank >= 0x8000, rank - 0x8000, 0xFFFF - rank), 16), f32)[:, :1]
    xs = x_sel.astype(bf16)
    cols = [pl.ds(f0, min(128, F - f0)) for f0 in range(0, F, 128)]
    acc = {}

    def accumulate(key, x):
        acc[key] = acc[key] + x if key in acc else x

    def up_tile(w_buf, name, f, k):
        accumulate((name, f), lax.dot_general(xs[:, 128 * k:128 * (k + 1)], w_buf[cols[f], pl.ds(128 * k, 128)], NT,
                                              preferred_element_type=f32))

    def down_tile(f, w):
        if w == 0:
            gate = rb(acc.pop(("gate", f)))
            acc["hidden"] = (rb(gate * sigmoid(gate)) * rb(acc.pop(("up", f)))).astype(bf16)
        accumulate(w, jnp.dot(acc["hidden"], wd_buf[cols[f], pl.ds(128 * w, 128)], preferred_element_type=f32))

    tiles = [functools.partial(up_tile, w_buf, name, f, k) for f in range(len(cols))
             for name, w_buf in (("gate", wg_buf), ("up", wu_buf)) for k in range(KT)]
    tiles += [lambda: None] * 32
    tiles += [functools.partial(down_tile, f, w) for f in range(len(cols)) for w in range(KT)]
    for p in range(NX // 2):
        sums = {}
        for j in range(JL + 1, NG):
            for k, _ in enumerate(project(j, p, sums)):
                if k != 7:
                    for tile in tiles[:4]:
                        tile()
                    tiles = tiles[4:]
    assert not tiles
    y = rb(jnp.concatenate([acc[w] for w in range(KT)], axis=1))
    routed = rb(x_sel + rb(y * rb(sigmoid(r_sel))))
    for c in range(C):
        tok = S - 1 - (chosen[c, 0] & (S - 1))
        for w in range(KT):
            rows = (lax.shift_right_logical(tok, 10), w, pl.ds(pl.multiple_of(tok & 1008, 16), 16))
            row = routed[c:c + 1, 128 * w:128 * (w + 1)]
            g_buf[rows] = jnp.where(row16[:, :128] == (tok & 15), row, g_buf[rows].astype(f32)).astype(bf16)
    for copy in kv_copies(1):
        copy.start()
    for h in range(G):
        for k in range(8):
            vt = [v_buf[h, pl.ds((8 * kh + k) * 128, 128), :].T for kh in range(2)]
            for i, (terms, _, _) in enumerate(PV):
                x = signed_sum(lambda dh, kh: vt[kh][64 * dh:64 * (dh + 1)].astype(f32), terms)
                t_buf[h, i, k] = x.astype(bf16)

    z_st, z_ld = zero_ref[0], zero_ref[1]

    def step(t, _):
        @pl.when(t == 2)
        def _():
            for copy in kv_copies(1):
                copy.wait()

        def out_start(block):
            @pl.when(t >= 2 * NG - 2)
            def _():
                for copy in out_copy((t & 1) * 8 + block):
                    copy.start()

        attention_step(t, z_st, z_ld, q_buf, k_buf, v_buf, wo_buf, x_buf, g_buf, out_buf, vt_buf, t_buf, ws_buf,
                       y_bufs, s_bufs, u_bufs, c_bufs, out_start)

    lax.fori_loop(0, 2 * NG, step, None)
    pltpu.make_async_copy(out_buf, out_buf, out_sem.at[0]).wait()


@jax.jit
def pallas_recurrent_scan__mha_block_cached__moe_arch_mod__prompt_kernel(
    A_x: jax.Array,
    A_k_cache: jax.Array,
    A_v_cache: jax.Array,
    A_wq: jax.Array,
    A_wo: jax.Array,
    B_x: jax.Array,
    B_w_r: jax.Array,
    B_w_gate: jax.Array,
    B_w_up: jax.Array,
    B_w_down: jax.Array,
):
    del B_x
    vmem, dma = pltpu.VMEM, pltpu.SemaphoreType.DMA
    hbm = pl.BlockSpec(memory_space=pl.ANY)
    scratch = [
        vmem((S + 64, D), bf16),
        vmem((KT, S, 128), bf16),
        vmem((3, KT, S // 2, 128), bf16),
        vmem((1 + 4 * H, 4, 128, DH), bf16),
        vmem((H + 1, SK, DH), bf16),
        vmem((H + 1, SK, DH), bf16),
        vmem((NG, D, G * DH), bf16),
        vmem((NG, G * DH, D), bf16),
        vmem((F, D), bf16),
        vmem((F, D), bf16),
        vmem((F, D), bf16),
        vmem((KT, S // 128, 128, 128), bf16),
        vmem((1, 3, 128, 128), bf16),
        vmem((2 * G + 1, 7, 8, 64, 128), bf16),
        vmem((1, 9, 4, 128, 128), bf16),
        [vmem((2, S // 2, 128), f32)] * KT,
        [vmem((1, 2 * SK + 32, 128), f32)] * N_S,
        [vmem((1, 8, 8, 128, 128), bf16)] * N_U,
        [vmem((1, 288, 128), f32)] * N_C,
        vmem((D,), bf16),
        pltpu.SMEM((2,), i32),
        dma((5,)), dma((NG,)), dma((4,)), dma((5,)), dma((1,)),
    ]
    out = pl.pallas_call(
        kernel,
        in_specs=[hbm] * 9,
        out_specs=hbm,
        out_shape=jax.ShapeDtypeStruct((S, D), bf16),
        scratch_shapes=scratch,
        compiler_params=pltpu.CompilerParams(vmem_limit_bytes=126 * 1024 * 1024),
        name="fused_kernel",
    )(A_x.reshape(S, D), A_k_cache.reshape(H, SK, DH), A_v_cache.reshape(H, SK, DH), A_wq,
      A_wo.reshape(NG, G * DH, D), B_w_r, B_w_gate.T, B_w_up.T, B_w_down)
    return out.reshape(1, S, D)
```

```python
import functools

import jax
import jax.experimental.pallas as pl
import jax.experimental.pallas.tpu as pltpu
import jax.numpy as jnp
import numpy as np
from jax import lax

S, D, H, DH, SK, F, C = 2048, 640, 32, 128, 2048, 1728, 8
KT = D // 128
G = 4
NG = H // G
BX = 256
NX = S // BX
LOG2E = 1.4426950408889634
EPS = float(np.asarray(1e-5, dtype=jnp.bfloat16))
f32, bf16, i32 = jnp.float32, jnp.bfloat16, jnp.int32
NT = (((1,), (1,)), ((), ()))

PV = [
    (((0, 0, 1), (1, 1, 1)), ((0, 0, 1), (1, 1, 1)), ((0, 0, 1), (1, 1, 1))),
    (((0, 1, 1), (1, 1, 1)), ((1, 0, 1), (1, 1, -1)), ((0, 0, 1),)),
    (((0, 0, 1), (1, 0, 1)), ((0, 1, 1), (0, 0, -1)), ((1, 1, 1),)),
    (((0, 0, 1),), ((0, 1, 1), (1, 1, 1)), ((0, 1, 1), (1, 1, -1))),
    (((1, 1, 1),), ((0, 0, 1), (1, 0, 1)), ((0, 0, -1), (1, 0, 1))),
    (((0, 1, 1), (0, 0, -1)), ((1, 1, 1),), ((0, 0, 1), (0, 1, 1))),
    (((1, 0, 1), (1, 1, -1)), ((0, 0, 1),), ((1, 0, 1), (1, 1, 1))),
]
OP = [
    0,
    (((0, 0, 1), (0, 1, 1)), ((1, 1, 1),), ((0, 0, -1), (0, 1, 1))),
    (((1, 0, 1), (1, 1, 1)), ((0, 0, 1),), ((1, 0, 1), (1, 1, -1))),
    (((0, 0, 1),), ((0, 1, 1), (1, 1, -1)), ((0, 1, 1), (1, 1, 1))),
    (((1, 1, 1),), ((1, 0, 1), (0, 0, -1)), ((0, 0, 1), (1, 0, 1))),
    (((0, 1, 1), (1, 1, -1)), ((1, 0, 1), (1, 1, 1)), ((0, 0, 1),)),
    (((0, 0, 1), (1, 1, 1)), ((0, 0, 1), (1, 1, 1)), ((0, 0, 1), (1, 1, 1))),
    (((1, 0, 1), (0, 0, -1)), ((0, 0, 1), (0, 1, 1)), ((1, 1, 1),)),
    1,
]

TIMING = dict(
    POP=10,
    K=3, Q=8, U=8, T=2, O=3, W=8,
    ACC=3,
    PREP=3,
    STAT=7, STAT_STEP=7, STAT_TOK=4,
    XPOSE=15,
    LAG=5,
    W_START=0.4, W_QK=0.7, W_OP=0.55, W_SHIFT=-1,
    OP_RATE=0.58,
    V_PREP=(330, 1300), WO_PREP=(14, 1.2), GATE=(170, 4),
)
N_S, N_U, N_C = 7, 4, 8


def rb(x):
    return x.astype(bf16).astype(f32)


def sigmoid(x):
    return 1.0 / (1.0 + jnp.exp2(x * (-LOG2E)))


def signed_sum(get, terms):
    v = get(*terms[0][:2])
    for i, j, sign in terms[1:]:
        v = v + get(i, j) if sign > 0 else v - get(i, j)
    return v


def updates(outputs):
    result = []
    for c, outs in enumerate(outputs):
        users = lambda i, j: [k for k, other in enumerate(outputs) if any(o[:2] == (i, j) for o in other)]
        result.append([(i, j, sign, c == users(i, j)[0], c == users(i, j)[-1]) for i, j, sign in outs])
    return result


PV_UPDATES = updates([step[2] for step in PV])
OP_UPDATES = updates([((step, 2, 1),) if isinstance(step, int) else step[2] for step in OP])


def attention_step(t, z_st, z_ld, q_buf, k_buf, v_buf, wo_buf, x_buf, g_buf, out_buf, vt_buf, t_buf, ws_buf,
                   y_bufs, s_bufs, u_bufs, c_bufs, out_start):
    T = TIMING
    POP = T["POP"]
    n = 2 * G
    grp, half = lax.shift_right_logical(t, 1), t & 1
    heads = [grp * G + a % G for a in range(n)]
    q_blocks = [1 + heads[a] * 4 + half * 2 + a // G for a in range(n)]
    q_ld, k_ld = [z_ld + i for i in q_blocks], [z_ld + h for h in heads]
    t_ld = [z_ld + (grp & 1) * G + h for h in range(G)]
    y_st, y_ld = z_st + half, z_ld + half
    row_st, row_ld = pl.multiple_of(z_st * 64, 64), pl.multiple_of(z_ld * 64, 64)
    x_rows = row_ld + pl.multiple_of(half * (S // 2), S // 2)
    never = lax.broadcasted_iota(i32, (8, 128), 1) > z_st + 1000

    dots, pending, seen = [], [("op", b, c) for b in range(2) for c in range(len(OP))], 0
    for hp in range(2 * n + T["LAG"]):
        for c in range(8):
            if hp < 2 * n and c % 2 == 0:
                dots += [("qk", hp // 2, 8 * (hp % 2) + c + e) for e in range(2)]
            if hp >= T["LAG"] and c < 7:
                dots.append(("pv", (hp - T["LAG"]) // 2, 7 * ((hp - T["LAG"]) % 2) + c))
            if hp > n + T["LAG"] and c < 7:
                seen += 1
                while pending and 2 * len(OP) - len(pending) < seen * T["OP_RATE"] and (c in (1, 3, 5, 6) or hp >= 2 * n):
                    dots.append(pending.pop(0))
    dots += pending + [("op", b, c) for b in range(2, 4) for c in range(len(OP))]
    start = {d: 8 * i for i, d in enumerate(dots)}

    events, val = [], {}

    def at(slot, order):
        return lambda fn: events.append((slot, order, len(events), fn))

    def load(ref, index, r, rows):
        return pltpu.bitcast(ref.bitcast(f32)[(*index, pl.ds(r // 2, rows // 2), slice(None))], bf16)

    def token(ref, index, v=None):
        v = val.get("token") if v is None else v
        if v is not None:
            ref.bitcast(f32)[(*index, pl.ds(0, 8), slice(None))] = v

    def x_token():
        x_buf.bitcast(f32)[pl.ds(row_st + S // 2, 4), pl.ds(0, 128)] = val["token"][:4]
        token(g_buf, (z_st + 2, 0))

    ring = lambda bufs, a, p: bufs[(2 * a + p) % len(bufs)]

    def result(d):
        if d not in val:
            kind, a, c = d
            if kind == "qk" and c % 2:
                val[d] = result((kind, a, c - 1))[128:]
            elif kind == "qk":
                k = jnp.concatenate([val.pop(("k", a, 8 * c + r)) for r in range(16)], axis=0)
                q = jnp.concatenate([val.pop(("q", d, r)) for r in range(4)], axis=1).reshape(512, DH)
                val[d] = lax.dot_general(k, q, NT, preferred_element_type=f32)
            elif kind == "pv":
                vt, pt = (jnp.concatenate([jnp.concatenate([val.pop((name, d, w, r)) for r in range(4)], axis=1)
                                           for w in range(2)], axis=0) for name in "tu")
                vt, pt = jnp.concatenate([vt[k] for k in range(8)], axis=1), pt.reshape(1024, 128)
                val[d] = jnp.dot(vt, pt, preferred_element_type=f32)
            else:
                o = jnp.concatenate([val.pop(("o", d, r)) for r in range(8)], axis=0)
                w = jnp.concatenate([val.pop(("w", d, r)) for r in range(4)], axis=1)
                if isinstance(OP[c], int):
                    w = w.reshape(512, 128)
                else:
                    w = jnp.concatenate([w[2 * u:2 * u + 2].reshape(256, 128) for u in range(2)], axis=1)
                val[d] = jnp.dot(o, w, preferred_element_type=f32)
        return val[d]

    def scores(d):
        _, a, c = d
        j0 = start[d]
        for r in range(4 if c % 2 == 0 else 0):
            @at(j0 + r - T["Q"], 1)
            def _(r=3 - r):
                token(q_buf, (z_st, 0))
                val["q", d, r] = load(q_buf, (q_ld[a], slice(None)), 32 * r, 32)
        for r in range(8):
            @at(min(j0 + r - T["K"], j0 - c % 2 * 8 + POP - 1), 1)
            def _(r=r):
                if r == 0:
                    token(k_buf, (z_st + H,))
                val["k", a, 8 * c + r] = load(k_buf, (k_ld[a],), 128 * c + 16 * r, 16)

            @at(j0 + r + POP, 0)
            def _(r=r):
                s = result(d)[16 * r:16 * r + 16]
                for p in range(2):
                    tiles = jnp.concatenate([s[:, 256 * p:256 * p + 128], s[:, 256 * p + 128:256 * p + 256]], axis=0)
                    ring(s_bufs, a, p)[z_st, pl.ds((((c % 8) * 8 + r) * 2 + c // 8) * 32, 32), :] = tiles
                x = jnp.maximum(s[:8], s[8:])
                x = val["max"] = x if r == 0 else jnp.maximum(x, val["max"])
                if r == 7:
                    if c == 0:
                        val["stat", a] = (x, jnp.ones_like(x))
                    else:
                        m0, e0 = val["stat", a]
                        m = jnp.maximum(m0, x)
                        val["stat", a] = (m, jnp.exp2(x - m) + e0 * jnp.exp2(m0 - m))
                    val["stat token", d] = val["stat", a][1][:, 384:]
                val["token"] = s[:8, 384:]

        @at(j0 + 7 + POP + T["STAT_TOK"], 0)
        def _():
            token(q_buf, (z_st, 1), val.pop(("stat token", d)))

        for j in range(4 if c == 15 else 0):
            @at(j0 + 8 + POP + T["STAT"] + T["STAT_STEP"] * j, 0)
            def _(j=j):
                m, e = (x[:, 128 * j:128 * (j + 1)] for x in val["stat", a])
                top = jnp.max(m, axis=0, keepdims=True)
                e = jnp.broadcast_to(jnp.sum(e * jnp.exp2(m - top), axis=0, keepdims=True), (8, 128))
                shift = (0.5 * np.log2(SK) / np.log2(SK / 16)) * jnp.log2(e)
                ring(s_bufs, a, j // 2)[z_st, pl.ds(2 * SK + 8 * (j % 2), 8), :] = top + shift

    def probabilities(a, p, slot_of):
        s_buf, u_buf = ring(s_bufs, a, p), ring(u_bufs, a, p)
        for e in range(64):
            @at(slot_of(e), 1)
            def _(e=e):
                pace = jnp.where(never, val.pop("prep"), val["token"]) if "prep" in val else val["token"]
                s_buf[z_st, pl.ds(2 * SK + 16, 8), :] = pace
                m = s_buf[z_ld, pl.ds(2 * SK, 16), :]
                m0, m1 = m[:8], m[8:]
                pt = jnp.exp2(s_buf[z_ld, pl.ds(64 * e, 64), :] - jnp.concatenate([m0, m0, m1, m1] * 2, axis=0))
                pt = {(kh, j): pt[32 * kh + 16 * j:32 * kh + 16 * j + 16] for kh in range(2) for j in range(2)}
                us = [signed_sum(lambda *ix: pt[ix], terms) for _, terms, _ in PV]
                for j in range(2):
                    x = us[[terms for _, terms, _ in PV].index(((0, j, 1), (1, j, 1)))]
                    x = x[:8] + x[8:]
                    val["sum", a, p, j] = x if e == 0 else val["sum", a, p, j] + x
                us = jnp.concatenate(us, axis=0).reshape(7, 16, 128).astype(bf16)
                val["p", a, p, e] = (us, val["sum", a, p, 1])

            @at(slot_of(e) + T["PREP"], 0)
            def _(e=e):
                us, val["prep"] = val.pop(("p", a, p, e))
                u_buf[z_st, pl.ds(0, 7), e // 8, pl.ds(e % 8 * 16, 16), :] = us

        @at(slot_of(63) + T["PREP"] + 2, 0)
        def _():
            for j in range(2):
                l = jnp.broadcast_to(jnp.sum(val.pop(("sum", a, p, j)), axis=0, keepdims=True), (8, 128))
                r = pl.reciprocal(l, approx=True)
                ring(c_bufs, a, p)[z_st, pl.ds(256 + 8 * j, 8), :] = r * (2.0 - l * r)

    def values(d):
        _, a, c = d
        p, i = divmod(c, 7)
        j0 = start[d]
        u_buf, c_buf = ring(u_bufs, a, p), ring(c_bufs, a, p)
        outs = PV_UPDATES[i]
        for r in range(8):
            @at(j0 + r - T["U"], 1)
            def _(w=r // 4, rr=3 - r % 4):
                if rr == 3:
                    token(u_buf, (z_st, 7, 2))
                val["u", d, w, rr] = load(u_buf, (z_ld, i, pl.ds(4 * w, 4)), 32 * rr, 32)

            @at(j0 + r - T["T"], 1)
            def _(r=r):
                if r == 0:
                    token(t_buf, (z_st + 2 * G, 0, 0))
                val["t", d, r // 4, r % 4] = load(t_buf, (t_ld[a % G], i, pl.ds(r // 4 * 4, 4)), r % 4 * 16, 16)
        for r in range(4):
            @at(j0 + 4 + r + POP - T["ACC"], 1)
            def _(r=r):
                for dh, j, _, first, last in outs:
                    if not first:
                        val["c", d, r, dh, j] = c_buf[z_ld, pl.ds(128 * j + 64 * dh + 16 * r, 16), :]
                    if last:
                        val["scale", d, r, dh, j] = c_buf[z_ld, pl.ds(256 + 8 * j, 8), :]

            @at(j0 + 4 + r + POP, 0)
            def _(r=r):
                x = result(d)[16 * r:16 * r + 16]
                for dh, j, sign, first, last in outs:
                    if first:
                        y = x if sign > 0 else -x
                    else:
                        y = val.pop(("c", d, r, dh, j))
                        y = y + x if sign > 0 else y - x
                    if last:
                        y = y * jnp.concatenate([val.pop(("scale", d, r, dh, j))] * 2, axis=0)
                        u_buf[z_st, 7, j, pl.ds(64 * dh + 16 * r, 16), :] = y.astype(bf16)
                    else:
                        c_buf[z_st, pl.ds(128 * j + 64 * dh + 16 * r, 16), :] = y
                val["token"] = x[:8]
        for j in range(2 if i == 6 else 0):
            @at(j0 + 9 + POP + 4 * j, 1)
            def _(j=j):
                val["ot", d, j] = load(u_buf, (z_ld, 7, j), 0, 128).T

            @at(j0 + 9 + POP + 4 * j + T["XPOSE"], 0)
            def _(j=j):
                q_buf[z_st + q_blocks[a], 2 * p + j] = val.pop(("ot", d, j))

    def projection(d):
        _, b, c = d
        j0 = start[d]
        assert j0 - T["O"] > start["pv", b // 2 * G + G - 1, b % 2 * 7 + 6] + 13 + POP + T["XPOSE"]
        extra = isinstance(OP[c], int)
        outs = [(i, 2 * j + u, u, sign, last) for i, j, sign, _, last in OP_UPDATES[c] for u in range(1 if extra else 2)]
        rows = lambda i, r, base=0: pl.ds(base + ((2 * b + i) * 128 + 16 * r), 16)
        for r in range(4):
            @at(j0 + r - T["W"], 1)
            def _(r=3 - r):
                if r % 2 == 1:
                    token(ws_buf, (z_st, 8, 0))
                val["w", d, r] = load(ws_buf, (z_ld, c % 8, slice(None)), 32 * r, 32)
        for r in range(8):
            @at(j0 + r - T["O"], 1)
            def _(r=r):
                token(q_buf, (z_st, 0))
                get = lambda i, h: load(q_buf, (q_ld[b // 2 * G + h], b % 2 * 2 + i), 16 * r, 16)
                if extra:
                    tiles = [get(OP[c], h) for h in range(G)]
                elif len(OP[c][0]) == 1:
                    tiles = [get(OP[c][0][0][0], 2 * OP[c][0][0][1] + u) for u in range(2)]
                else:
                    tiles = [signed_sum(lambda i, k: get(i, 2 * k + u).astype(f32), OP[c][0]).astype(bf16)
                             for u in range(2)]
                val["o", d, r] = jnp.concatenate(tiles, axis=1)

            @at(j0 + r + POP - T["ACC"], 1)
            def _(r=r):
                if r % 2 == 0 and any(last for *_, last in outs):
                    x_token()
                for i, w, _, _, last in outs:
                    val["y", d, r, i, w] = y_bufs[w][y_ld, rows(i, r), :]
                    if last:
                        val["x", d, r, i, w] = (x_buf[rows(i, r, x_rows), pl.ds(128 * w, 128)].astype(f32),
                                                load(g_buf, (y_ld, w), (2 * b + i) * 128 + 16 * r, 16).astype(f32))

            @at(j0 + r + POP - 1, 0)
            def _(r=r):
                for i, w, u, sign, last in outs:
                    x = result(d)[16 * r:16 * r + 16, 128 * u:128 * (u + 1)]
                    y = val.pop(("y", d, r, i, w))
                    y = y + x if sign > 0 else y - x
                    y_bufs[w][y_st, rows(i, r), :] = y
                    if last:
                        x, gate = val.pop(("x", d, r, i, w))
                        out_buf[w, half * 8 + 2 * b + i, pl.ds(16 * r, 16), :] = (x + y * gate).astype(bf16)
                val["token"] = y[:8]
                if r == 7 and c in (6, 8):
                    out_start(2 * b + (c == 8))

    for d in dots:
        {"qk": scores, "pv": values, "op": projection}[d[0]](d)

    density = {start[d] + POP + r: T["W_QK"] if d[0] == "qk" else T["W_OP"]
               for d in dots if d[0] != "pv" for r in range(8)}
    cum = np.concatenate([[0], np.cumsum([T["W_START"] if j < start["pv", 0, 0] else density.get(j - T["W_SHIFT"], 1.0)
                                          for j in range(8 * len(dots))])])
    earliest = [max(start["qk", g // 2, 15] + 9 + POP + T["STAT"] + T["STAT_STEP"] * (g % 2 * 2 + 1),
                    start["pv", (g - N_U) // 2, (g - N_U) % 2 * 7 + 6] + 8 if g >= N_U else 0) for g in range(2 * n)]
    latest = [start["pv", g // 2, g % 2 * 7] - T["U"] - T["PREP"] - 1 for g in range(2 * n)]
    edge = [cum[earliest[0]]] + [cum[j] for j in latest]
    for _ in range(200):
        for g in range(1, 2 * n):
            edge[g] = min(max((edge[g - 1] + edge[g + 1]) / 2, cum[earliest[g]]), cum[latest[g - 1]])
    for g in range(2 * n):
        assert g + N_S >= 2 * n or latest[g] < start["qk", (g + N_S) // 2, 0] + POP
        probabilities(g // 2, g % 2, lambda e: int(np.searchsorted(cum, edge[g] + (edge[g + 1] - edge[g]) * (e + 0.5) / 64)) - 1)

    step = (T["V_PREP"][1] - T["V_PREP"][0]) / 16
    for hh, k in ((hh, k) for hh in range(2) for k in range(8)):
        head = jnp.minimum(grp + 1, NG - 1) * G + 2 * half + hh
        j0 = T["V_PREP"][0] + step * (8 * hh + k)
        for kh in range(2):
            @at(j0 + step / 2 * kh, 2)
            def _(head=head, hh=hh, k=k, kh=kh):
                token(v_buf, (z_st + H,))
                val["vt", hh, k, kh] = load(v_buf, (z_ld + head,), (8 * kh + k) * 128, 128).T

            @at(j0 + step / 2 * kh + T["XPOSE"], 0)
            def _(hh=hh, k=k, kh=kh):
                vt_buf[z_st, kh] = val.pop(("vt", hh, k, kh))
        for r in range(4):
            @at(j0 + step / 2 + 1 + T["XPOSE"] + step / 9 * r, 2)
            def _(hh=hh, k=k, r=r):
                token(vt_buf, (z_st, 2))
                vt = {(dh, kh): load(vt_buf, (z_ld, kh), 64 * dh + 16 * r, 16).astype(f32)
                      for dh in range(2) for kh in range(2)}
                val["vs", hh, k, r] = [signed_sum(lambda *ix: vt[ix], terms) for terms, _, _ in PV]

            @at(j0 + step / 2 + 3 + T["XPOSE"] + step / 9 * r, 0)
            def _(hh=hh, k=k, r=r):
                x = jnp.concatenate(val.pop(("vs", hh, k, r)), axis=0)
                block = z_st + ((grp + 1) & 1) * G + 2 * half + hh
                t_buf[block, :, k, pl.ds(16 * r, 16), :] = x.reshape(7, 16, 128).astype(bf16)
                token(q_buf, (z_st, 2), x[96:104])

    for k, r in ((k, r) for k in range(8) for r in range(16)):
        slot = T["WO_PREP"][0] + T["WO_PREP"][1] * (16 * k + r)

        @at(slot, 2)
        def _(k=k, r=r):
            def get(row, col):
                w = pltpu.bitcast(wo_buf[grp, pl.ds(row, 16), pl.ds(col, 128)], f32)
                return jnp.where(never, val["token"], w)
            for u in range(2):
                if k == 0 or len(OP[k][1]) == 1:
                    row, col = (256 * u, 512) if k == 0 else (256 * OP[k][1][0][0], 256 * OP[k][1][0][1] + 128 * u)
                    x = get(row + 16 * r, col)
                    ws_buf.bitcast(f32)[z_st, k, 2 * u + r // 8, pl.ds(r % 8 * 8, 8), :] = x
                else:
                    x = signed_sum(lambda i, j: pltpu.bitcast(get(256 * i + 16 * r, 256 * j + 128 * u), bf16).astype(f32),
                                   OP[k][1])
                    ws_buf[z_st, k, 2 * u + r // 8, pl.ds(r % 8 * 16, 16), :] = x.astype(bf16)
            val["ws", k, r] = x[:8]

        @at(slot + 3, 0)
        def _(k=k, r=r):
            token(q_buf, (z_st, 3), val.pop(("ws", k, r)))

    for r, w in ((r, w) for r in range(8) for w in range(KT)):
        slot = T["GATE"][0] + T["GATE"][1] * (KT * r + w)
        assert slot + 4 < start["op", 3, 0]
        where = lambda z, r=r, w=w: (z + lax.shift_right_logical(t, 3), w, pl.ds(pl.multiple_of((t & 7) * 128 + 16 * r, 16), 16))

        @at(slot, 2)
        def _(r=r, w=w, where=where):
            token(g_buf, (z_st + 2, 0))
            x = g_buf[where(z_ld)].astype(f32)
            val["gate", r, w] = x * sigmoid(x)

        @at(slot + 4, 0)
        def _(r=r, w=w, where=where):
            gate = val.pop(("gate", r, w))
            g_buf[where(z_st)] = gate.astype(bf16)
            token(q_buf, (z_st, 3), gate[8:])

    for *_, fn in sorted(events, key=lambda e: e[:3]):
        fn()


def kernel(x_hbm, k_hbm, v_hbm, wq_hbm, wo_hbm, wr_hbm, wg_hbm, wu_hbm, wd_hbm, out_hbm,
           x_buf, xn_buf, g_buf, q_buf, k_buf, v_buf, wq_buf, wo_buf, wg_buf, wu_buf, wd_buf, out_buf,
           vt_buf, t_buf, ws_buf, y_bufs, s_bufs, u_bufs, c_bufs, wr_buf, zero_ref,
           x_sem, wq_sem, kv_sem, w_sem, out_sem):
    x_edges = (0, 1, 2, 4, 6, 8)

    def x_copy(i):
        rows = pl.ds(x_edges[i] * BX, (x_edges[i + 1] - x_edges[i]) * BX)
        return pltpu.make_async_copy(x_hbm.at[rows], x_buf.at[rows], x_sem.at[i])

    def wq_copy(j):
        return pltpu.make_async_copy(wq_hbm.at[:, pl.ds(j * G * DH, G * DH)], wq_buf.at[j], wq_sem.at[j])

    def kv_copies(late):
        k_heads, v_heads = (pl.ds(n, H - n) if late else pl.ds(0, n) for n in (G, 2 * G))
        return [pltpu.make_async_copy(k_hbm.at[k_heads], k_buf.at[k_heads], kv_sem.at[2 * late]),
                pltpu.make_async_copy(v_hbm.at[v_heads], v_buf.at[v_heads], kv_sem.at[2 * late + 1])]

    def w_copy(i):
        src, dst = ((wr_hbm, wr_buf), (wg_hbm, wg_buf), (wu_hbm, wu_buf), (wd_hbm, wd_buf), (wo_hbm, wo_buf))[i]
        return pltpu.make_async_copy(src, dst, w_sem.at[i])

    def out_copy(i):
        return [pltpu.make_async_copy(out_buf.at[w, i], out_hbm.at[pl.ds(i * 128, 128), pl.ds(128 * w, 128)], out_sem.at[0])
                for w in range(KT)]

    lane = lax.broadcasted_iota(i32, (8, 128), 1)
    sublane = lax.broadcasted_iota(i32, (8, 128), 0)
    row16 = lax.broadcasted_iota(i32, (16, D), 0)

    def layernorm(r0, n):
        x = x_buf[pl.ds(r0, n), :].astype(f32)
        mean = jnp.sum(x, axis=-1, keepdims=True)
        yield
        mean = mean * (1.0 / D)
        mean_b = rb(mean)
        xc = x - mean_b
        dm = mean - mean_b
        sq = jnp.sum(xc * xc, axis=-1, keepdims=True)
        yield
        var = jnp.broadcast_to(sq * (1.0 / D) - dm * dm, (n, 128))
        dense = var[:8]
        for k in range(1, n // 8):
            dense = jnp.where(lane == k, var[8 * k:8 * k + 8], dense)
        inv = 1.0 / rb(jnp.sqrt(rb(rb(jnp.maximum(dense, 0.0)) + EPS)))
        inv = jnp.concatenate([jnp.broadcast_to(inv[:, k:k + 1], (8, 128)) for k in range(n // 8)], axis=0)
        yield
        xc = rb(xc)
        for w in range(KT):
            xn = (xc[:, 128 * w:128 * (w + 1)] * inv).astype(bf16)
            xn_buf[w, pl.ds(r0, n), :] = xn
            g_buf[r0 // 1024, w, pl.ds(r0 % 1024, n), :] = xn

    def load_xn(r0, n, tiles):
        rows = pl.ds(r0 // 2 if isinstance(r0, int) else pl.multiple_of(lax.shift_right_logical(r0, 1), 8), n // 2)
        return jnp.concatenate([pltpu.bitcast(xn_buf.bitcast(f32)[w, rows, :], bf16) for w in tiles], axis=1)

    live, started = [], [0]

    def layernorm_until(row, available):
        while started[0] - 64 * len(live) < row:
            for piece in list(live):
                if next(piece, "done") == "done":
                    live.remove(piece)
            if started[0] < available:
                live.append(layernorm(started[0], 64))
                next(live[-1])
                started[0] += 64

    def store_q(head, block, half, q):
        q = q * (DH ** -0.5 * LOG2E)
        q_buf[1 + head * 4 + block, pl.ds(2 * half, 2)] = q.reshape(2, 128, DH).astype(bf16)
        return q[:8]

    JL = NG - 3
    x_copy(0).start()
    w_copy(0).start()
    wq_copy(0).start()
    x_copy(1).start()
    zero_ref[0] = 0
    zero_ref[1] = 0
    for y_buf in y_bufs:
        y_buf[...] = jnp.zeros_like(y_buf)
    x_copy(0).wait()
    x_copy(2).start()
    w_copy(0).wait()
    layernorm_until(BX, BX)
    wq_copy(0).wait()
    x_copy(3).start()
    for i in range(NX):
        if i + 1 in x_edges[:-1]:
            part = x_edges.index(i + 1)
            if part == 1:
                x_copy(4).start()
            if part == 3:
                for j in range(1, JL + 1):
                    wq_copy(j).start()
            x_copy(part).wait()
        q = jnp.dot(load_xn(i * BX, BX, range(KT)), wq_buf[0], preferred_element_type=f32)
        for h in range(G):
            store_q(h, i // 2, i % 2, q[:, h * DH:(h + 1) * DH])
        if i + 1 < NX:
            layernorm_until((i + 2) * BX, x_edges[part + 1] * BX)

    def project(j, p, sums, after=None):
        xa = lambda r, k: load_xn((2 * p + r) * BX, BX, (2 * k, 2 * k + 1))
        wb = lambda k, c: wq_buf[j, pl.ds(256 * k, 256), pl.ds(256 * c, 256)]

        def operand(get, terms):
            if len(terms) == 1:
                return get(*terms[0][:2])
            return signed_sum(lambda *ix: get(*ix).astype(f32), terms).astype(bf16)

        def product(c):
            if len(OP[c][0]) > 1 and c not in sums:
                sums[c] = operand(xa, OP[c][0])
            a = sums[c] if c in sums else operand(xa, OP[c][0])
            return jnp.dot(a, operand(wb, OP[c][1]), preferred_element_type=f32)

        def rest(r, after=None):
            a = load_xn((2 * p + r) * BX, BX, (4,))
            if after is not None:
                head = jnp.where(lane > p + 1000, after, pltpu.bitcast(a[:16], f32))
                a = jnp.concatenate([pltpu.bitcast(head, bf16), a[16:]], axis=0)
            e = jnp.dot(a, wq_buf[j, pl.ds(512, 128), :], preferred_element_type=f32)
            return e[:, :256], e[:, 256:]

        def put(r, c, q):
            return [store_q(j * G + 2 * c + h, p, r, q[:, h * DH:(h + 1) * DH]) for h in range(2)][0]

        c00, c01 = rest(0, after)
        yield
        m = product(1)
        c00, c01 = c00 - m, c01 + m
        yield
        m = product(3)
        yield put(0, 1, c01 + m)
        c10, c11 = rest(1)
        c11 = c11 + m
        yield
        m = product(2)
        c10, c11 = c10 + m, c11 - m
        yield
        m = product(4)
        c00 = c00 + m
        yield put(1, 0, c10 + m)
        c00 = c00 + product(5)
        yield
        m = product(6)
        c11 = c11 + m
        yield put(0, 0, c00 + m)
        yield put(1, 1, c11 + product(7))

    def top_k(scores):
        keys = []
        for k, r in enumerate(scores):
            r = rb(r)
            r = jnp.where(r == 0.0, 0.0, r)
            bits = lax.shift_right_logical(pltpu.bitcast(r, i32), 16)
            rank = jnp.where(r != r, 0, jnp.where(bits >= 0x8000, 0xFFFF - bits, bits + 0x8000))
            tok = k * 1024 + lane * 8 + sublane
            keys.append(pltpu.bitcast(0x20000000 + rank * S + (S - 1 - tok), f32))
        chosen, rows = jnp.zeros((8, 128), i32), jnp.zeros((16, D), f32)
        for c in range(C):
            best = jnp.max(jnp.max(jnp.maximum(*keys), axis=0, keepdims=True), axis=1, keepdims=True)
            best = jnp.broadcast_to(best, (8, 128))
            keys = [jnp.where(key == best, 0.0, key) for key in keys]
            best = pltpu.bitcast(best, i32)
            chosen = jnp.where(sublane == c, best, chosen)
            tok = S - 1 - (best[0, 0] & (S - 1))
            block = load_xn(tok & -16, 16, range(KT)).astype(f32)
            row = jnp.sum(jnp.where(row16 == (tok & 15), block, 0.0), axis=0, keepdims=True)
            rows = jnp.where(row16 == c, row, rows)
        return chosen, rows

    def half_of_rows(jj, carry):
        @pl.when(jj == 1)
        def _():
            for copy in kv_copies(0):
                copy.start()

        @pl.when(jj == 0)
        def _():
            for j in range(1, JL):
                wq_copy(j).wait()
            for j in range(JL + 1, NG):
                wq_copy(j).start()
            for i in range(1, 5):
                w_copy(i).start()
            wq_copy(JL).wait()

        wr = wr_buf[...].astype(f32).reshape(1, D)
        r0 = pl.multiple_of(jj * (S // 4), S // 4)
        never = lane > jj + 1000
        score, done, after = jnp.zeros((8, 128), f32), 0, None
        for unit in range(2 * JL):
            if unit % JL == 0:
                sums = {}
            for pace in project(1 + unit % JL, 2 * jj + unit // JL, sums, after if unit == 2 * JL - 1 else None):
                if pace is None or done == 64:
                    continue
                for k in (done, done + 1):
                    terms = []
                    for w in range(KT):
                        xn = xn_buf.bitcast(f32)[w, pl.ds(r0 + 8 * k, 8), :]
                        xn = pltpu.bitcast(jnp.where(never, pace, xn), bf16).astype(f32)
                        terms.append(xn * wr[:, 128 * w:128 * (w + 1)])
                    r = jnp.sum(functools.reduce(lambda x, y: x + y, terms), axis=-1, keepdims=True)
                    r = jnp.broadcast_to(r, (16, 128))
                    score = jnp.where(lane == 2 * k, r[:8], jnp.where(lane == 2 * k + 1, r[8:], score))
                done += 2
                if done == 64:
                    scores = [jnp.where(jnp.full((8, 128), jj) == k, score, carry[0][k]) for k in range(2)]
                    chosen, rows = top_k(scores)
                    after = functools.reduce(lambda x, y: x + y, [rows[:8, 128 * w:128 * (w + 1)] for w in range(KT)])
        return scores, chosen, rows

    zeros = jnp.zeros((8, 128), f32)
    _, chosen, x_sel = lax.fori_loop(
        0, 2, half_of_rows, ([zeros, zeros], jnp.zeros((8, 128), i32), jnp.zeros((16, D), f32)))
    x_sel = x_sel[:8]

    for j in range(JL + 1, NG):
        wq_copy(j).wait()
    for i in range(1, 4):
        w_copy(i).wait()
    for copy in kv_copies(0):
        copy.wait()
    w_copy(4).wait()
    rank = lax.shift_right_logical(chosen - 0x20000000, 11)
    r_sel = pltpu.bitcast(lax.shift_left(jnp.where(rank >= 0x8000, rank - 0x8000, 0xFFFF - rank), 16), f32)[:, :1]
    xs = x_sel.astype(bf16)
    cols = [pl.ds(f0, min(128, F - f0)) for f0 in range(0, F, 128)]
    acc = {}

    def accumulate(key, x):
        acc[key] = acc[key] + x if key in acc else x

    def up_tile(w_buf, name, f, k):
        accumulate((name, f), lax.dot_general(xs[:, 128 * k:128 * (k + 1)], w_buf[cols[f], pl.ds(128 * k, 128)], NT,
                                              preferred_element_type=f32))

    def down_tile(f, w):
        if w == 0:
            gate = rb(acc.pop(("gate", f)))
            acc["hidden"] = (rb(gate * sigmoid(gate)) * rb(acc.pop(("up", f)))).astype(bf16)
        accumulate(w, jnp.dot(acc["hidden"], wd_buf[cols[f], pl.ds(128 * w, 128)], preferred_element_type=f32))

    tiles = [functools.partial(up_tile, w_buf, name, f, k) for f in range(len(cols))
             for name, w_buf in (("gate", wg_buf), ("up", wu_buf)) for k in range(KT)]
    tiles += [lambda: None] * 32
    tiles += [functools.partial(down_tile, f, w) for f in range(len(cols)) for w in range(KT)]
    for p in range(NX // 2):
        sums = {}
        for j in range(JL + 1, NG):
            for k, _ in enumerate(project(j, p, sums)):
                if k != 7:
                    for tile in tiles[:4]:
                        tile()
                    tiles = tiles[4:]
    assert not tiles
    y = rb(jnp.concatenate([acc[w] for w in range(KT)], axis=1))
    routed = rb(x_sel + rb(y * rb(sigmoid(r_sel))))
    for c in range(C):
        tok = S - 1 - (chosen[c, 0] & (S - 1))
        for w in range(KT):
            rows = (lax.shift_right_logical(tok, 10), w, pl.ds(pl.multiple_of(tok & 1008, 16), 16))
            row = routed[c:c + 1, 128 * w:128 * (w + 1)]
            g_buf[rows] = jnp.where(row16[:, :128] == (tok & 15), row, g_buf[rows].astype(f32)).astype(bf16)
    for copy in kv_copies(1):
        copy.start()
    for h in range(G):
        for k in range(8):
            vt = [v_buf[h, pl.ds((8 * kh + k) * 128, 128), :].T for kh in range(2)]
            for i, (terms, _, _) in enumerate(PV):
                x = signed_sum(lambda dh, kh: vt[kh][64 * dh:64 * (dh + 1)].astype(f32), terms)
                t_buf[h, i, k] = x.astype(bf16)

    z_st, z_ld = zero_ref[0], zero_ref[1]

    def step(t, _):
        @pl.when(t == 2)
        def _():
            for copy in kv_copies(1):
                copy.wait()

        def out_start(block):
            @pl.when(t >= 2 * NG - 2)
            def _():
                for copy in out_copy((t & 1) * 8 + block):
                    copy.start()

        attention_step(t, z_st, z_ld, q_buf, k_buf, v_buf, wo_buf, x_buf, g_buf, out_buf, vt_buf, t_buf, ws_buf,
                       y_bufs, s_bufs, u_bufs, c_bufs, out_start)

    lax.fori_loop(0, 2 * NG, step, None)
    pltpu.make_async_copy(out_buf, out_buf, out_sem.at[0]).wait()


@jax.jit
def pallas_recurrent_scan__mha_block_cached__moe_arch_mod__prompt_kernel(
    A_x: jax.Array,
    A_k_cache: jax.Array,
    A_v_cache: jax.Array,
    A_wq: jax.Array,
    A_wo: jax.Array,
    B_x: jax.Array,
    B_w_r: jax.Array,
    B_w_gate: jax.Array,
    B_w_up: jax.Array,
    B_w_down: jax.Array,
):
    del B_x
    vmem, dma = pltpu.VMEM, pltpu.SemaphoreType.DMA
    hbm = pl.BlockSpec(memory_space=pl.ANY)
    scratch = [
        vmem((S + 64, D), bf16),
        vmem((KT, S, 128), bf16),
        vmem((3, KT, S // 2, 128), bf16),
        vmem((1 + 4 * H, 4, 128, DH), bf16),
        vmem((H + 1, SK, DH), bf16),
        vmem((H + 1, SK, DH), bf16),
        vmem((NG, D, G * DH), bf16),
        vmem((NG, G * DH, D), bf16),
        vmem((F, D), bf16),
        vmem((F, D), bf16),
        vmem((F, D), bf16),
        vmem((KT, S // 128, 128, 128), bf16),
        vmem((1, 3, 128, 128), bf16),
        vmem((2 * G + 1, 7, 8, 64, 128), bf16),
        vmem((1, 9, 4, 128, 128), bf16),
        [vmem((2, S // 2, 128), f32)] * KT,
        [vmem((1, 2 * SK + 32, 128), f32)] * N_S,
        [vmem((1, 8, 8, 128, 128), bf16)] * N_U,
        [vmem((1, 288, 128), f32)] * N_C,
        vmem((D,), bf16),
        pltpu.SMEM((2,), i32),
        dma((5,)), dma((NG,)), dma((4,)), dma((5,)), dma((1,)),
    ]
    out = pl.pallas_call(
        kernel,
        in_specs=[hbm] * 9,
        out_specs=hbm,
        out_shape=jax.ShapeDtypeStruct((S, D), bf16),
        scratch_shapes=scratch,
        compiler_params=pltpu.CompilerParams(vmem_limit_bytes=126 * 1024 * 1024),
        name="fused_kernel",
    )(A_x.reshape(S, D), A_k_cache.reshape(H, SK, DH), A_v_cache.reshape(H, SK, DH), A_wq,
      A_wo.reshape(NG, G * DH, D), B_w_r, B_w_gate.T, B_w_up.T, B_w_down)
    return out.reshape(1, S, D)
```
